```python
import jax
import jax.numpy as jnp

def _softmax(x, axis=-1):
    return jax.nn.softmax(x, axis=axis)
def _gelu(x):
    return jax.nn.gelu(x, approximate=True)
def _silu(x):
    return jax.nn.silu(x)
def _sigmoid(x):
    return jax.nn.sigmoid(x)
def _layernorm(x, axis=-1, eps=1e-5):
    m = jnp.mean(x, axis=axis, keepdims=True)
    v = jnp.var(x, axis=axis, keepdims=True)
    return (x - m) / jnp.sqrt(v + eps)
def _scatter_add(tgt, idx, src, axis=0):
    return tgt.at[idx].add(src)
def _segment_sum(src, seg, n):
    return jax.ops.segment_sum(src, seg, n)
class _Rng:
    def __init__(self, key):
        self._k = key
    def _next(self):
        self._k, sub = jax.random.split(self._k)
        return sub
    def normal(self, shape):
        return jax.random.normal(self._next(), shape, dtype=jnp.bfloat16)
    def randint(self, lo, hi, shape):
        return jax.random.randint(self._next(), shape, lo, hi, dtype=jnp.int32)
    def uniform(self, shape, lo=0.0, hi=1.0):
        return jax.random.uniform(self._next(), shape, jnp.bfloat16, lo, hi)
    def permutation(self, n):
        return jax.random.permutation(self._next(), n)


kernel_name = 'gated_mix__sliding_local_dilated__glu_gated_reglu__prompt'

def setup_inputs():
    _rng = _Rng(jax.random.key(int.from_bytes(__import__("os").urandom(4), "little")))
    _w = (lambda a: (lambda t: t.astype(jnp.bfloat16) if jnp.issubdtype(t.dtype, jnp.floating) else t)(jnp.asarray(a)))
    def _A_setup():
        B, S, D = 1, 2048, 1024
        return {
            "x": _w((lambda *s: _rng.normal(s) * 0.05)(B, S, D)),
            "wqkv": _w((lambda *s: _rng.normal(s) * 0.05)(D, 3 * D)),
            "wo": _w((lambda *s: _rng.normal(s) * 0.05)(D, D)),
        }
    _A_in = _A_setup()

    def _B_setup():
        B, S, D, F = 1, 2048, 1024, 3584
        return {
            "x": _w((lambda *s: _rng.normal(s) * 0.05)(B, S, D)),
            "W_gate": _w((lambda *s: _rng.normal(s) * 0.05)(D, F) * (2.0 / D) ** 0.5),
            "W_up": _w((lambda *s: _rng.normal(s) * 0.05)(D, F) * (2.0 / D) ** 0.5),
            "W_down": _w((lambda *s: _rng.normal(s) * 0.05)(F, D) * (1.0 / F) ** 0.5),
        }
    _B_in = _B_setup()

    return {
        "A_x": _A_in["x"],
        "A_wqkv": _A_in["wqkv"],
        "A_wo": _A_in["wo"],
        "B_x": _B_in["x"],
        "B_W_gate": _B_in["W_gate"],
        "B_W_up": _B_in["W_up"],
        "B_W_down": _B_in["W_down"],
        "gate_w": _w((lambda *s: _rng.normal(s) * 0.05)(1024)),
    }

def reference(A_x, A_wqkv, A_wo, B_x, B_W_gate, B_W_up, B_W_down, gate_w):
    def _A_ref(x, wqkv, wo):
        B, S, D = x.shape
        H = 32; Dh = D // H
        W, dil = 8, 2
        qkv = (lambda x, *d: x.transpose(*d))((x @ wqkv).reshape(B, S, 3, H, Dh), 2, 0, 3, 1, 4)
        q, k, v = qkv[0], qkv[1], qkv[2]
        scale = Dh ** -0.5
        pos = jnp.arange(S)
        off = jnp.arange(W) * dil
        idx = pos[:, None] - off[None, :]
        mask = idx >= 0
        idx_c = jnp.where(mask, idx, 0).reshape(-1)
        kg = k[:, :, idx_c, :].reshape(B, H, S, W, Dh)
        vg = v[:, :, idx_c, :].reshape(B, H, S, W, Dh)
        logits = jnp.einsum("bhsd,bhswd->bhsw", q, kg) * scale
        logits = jnp.where(mask[None, None, :, :], logits, -1e9)
        attn = _softmax(logits, axis=-1)
        o = jnp.einsum("bhsw,bhswd->bhsd", attn, vg)
        return (lambda x, *d: x.transpose(*d))(o, 0, 2, 1, 3).reshape(B, S, D) @ wo

    def _B_ref(x, W_gate, W_up, W_down):
        gate = jnp.einsum("bsd,df->bsf", x, W_gate)
        up = jnp.einsum("bsd,df->bsf", x, W_up)
        gate = gate * (lambda x, dt: x.astype(dt))(gate > 0, gate.dtype)
        h = gate * up
        return jnp.einsum("bsf,fd->bsd", h, W_down)

    x = A_x
    g = _sigmoid((x * gate_w).sum(-1, keepdims=True))
    a = _A_ref(x, A_wqkv, A_wo)
    b = _B_ref(x, B_W_gate, B_W_up, B_W_down)
    return g * a + (1 - g) * b
```

```python
import functools
import math

import jax
import jax.numpy as jnp
from jax import lax
import jax.experimental.pallas as pl
import jax.experimental.pallas.tpu as pltpu

H = 32
DH = 32
W = 8
DIL = 2
LANES = 128
NT = 8
HALO = 16

TM = 512
TM0 = 256
F0 = 512
TF = 768
UNIT = 16
PB = 4

_F32 = jnp.float32
_BF16 = jnp.bfloat16


def _dot(a, b):
    return jnp.dot(a, b, preferred_element_type=_F32)


def _kernel(x_hbm, wqkv_hbm, wo_hbm, wg_hbm, wu_hbm, wd_hbm, gw_ref, out_hbm,
            x_v, wq_raw, wq_p, wo_raw, wo_f, wo_p, wg0, wu0, wd0, wg, wu, wd,
            acc, q_s, k_s, v_s, g_s, o_s, out_st,
            sem_x, sem_w0, sem_q, sem_rest, sem_out,
            *, S, D, F):
    NR = S // TM
    NR0 = S // TM0
    NC = (F - F0) // TF
    NSL = 6
    HR = D // 2

    def x_copy(t):
        return pltpu.make_async_copy(
            x_hbm.at[pl.ds(t * TM0, TM0), :], x_v.at[pl.ds(t * TM0, TM0), :],
            sem_x.at[t])

    def w0_copies():
        return (
            pltpu.make_async_copy(wg_hbm.at[:, pl.ds(0, F0)], wg0, sem_w0.at[0]),
            pltpu.make_async_copy(wu_hbm.at[:, pl.ds(0, F0)], wu0, sem_w0.at[1]),
            pltpu.make_async_copy(wd_hbm.at[pl.ds(0, F0), :], wd0, sem_w0.at[2]),
        )

    def wq_copy(a):
        sec = a // 2
        half = a % 2
        return pltpu.make_async_copy(
            wqkv_hbm.at[pl.ds(half * HR, HR), pl.ds(sec * D, D)],
            wq_raw.at[a], sem_q.at[a])

    def rest_copies():
        cps = [pltpu.make_async_copy(wo_hbm, wo_raw, sem_rest.at[0])]
        for c in range(NC):
            lo = F0 + c * TF
            cps.append(pltpu.make_async_copy(
                wg_hbm.at[:, pl.ds(lo, TF)], wg.at[c], sem_rest.at[1]))
            cps.append(pltpu.make_async_copy(
                wu_hbm.at[:, pl.ds(lo, TF)], wu.at[c], sem_rest.at[1]))
            cps.append(pltpu.make_async_copy(
                wd_hbm.at[pl.ds(lo, TF), :], wd.at[c], sem_rest.at[1]))
        return cps

    def out_copy(r):
        return pltpu.make_async_copy(
            out_st.at[r], out_hbm.at[pl.ds(r * TM, TM), :], sem_out.at[r])

    x_copy(0).start()
    for cp in w0_copies():
        cp.start()
    for t in range(1, NR0):
        x_copy(t).start()
        if t - 1 < NSL:
            wq_copy(t - 1).start()
    for cp in rest_copies():
        cp.start()

    zeros_halo = jnp.zeros((HALO, LANES), _F32)
    for j in range(NT):
        k_s[j, pl.ds(0, HALO), :] = zeros_halo
        v_s[j, pl.ds(0, HALO), :] = zeros_halo

    def permute_slice(a):
        rows = PB * 8
        lane = lax.broadcasted_iota(jnp.int32, (rows, LANES), 1)
        bits = [((lane >> (2 + b)) & 1) == 1 for b in range(3)]
        base_pat = NT * 4 * (lane & 3) + (lane >> 5) + 4 * ((lane >> 2) & 7)
        pats = [(base_pat + 4 * j) & (LANES - 1) for j in range(NT)]
        for g in range(HR // (16 * PB)):
            rs = pl.ds(g * 16 * PB, 16 * PB)
            z = []
            for i in range(NT):
                w = pltpu.bitcast(wq_raw[a, rs, pl.ds(i * LANES, LANES)],
                                  jnp.uint32)
                z.append(w if i == 0 else pltpu.roll(w, 4 * i, 1))
            for b in range(3):
                z = [jnp.where(bits[b], z[(k + (1 << b)) % NT], z[k])
                     for k in range(NT)]
            for j in range(NT):
                y = jnp.take_along_axis(z[(-j) % NT], pats[j], axis=1)
                wq_p[a, rs, pl.ds(j * LANES, LANES)] = pltpu.bitcast(y, _BF16)

    def phase0(t, carry):
        x_copy(t).wait()

        @pl.when(t == 0)
        def _():
            for cp in w0_copies():
                cp.wait()

        real = jnp.logical_and(t >= 1, t <= NSL)

        @pl.when(real)
        def _():
            wq_copy(t - 1).wait()

        rows = pl.ds(pl.multiple_of(t * TM0, TM0), TM0)
        xv = x_v[rows, :]
        gt = _dot(xv, wg0[...])
        up = _dot(xv, wu0[...])
        hh = (jnp.maximum(gt, 0.0) * up).astype(_BF16)
        acc[rows, :] = _dot(hh, wd0[...])
        permute_slice(jnp.where(real, t - 1, NSL))
        return carry

    lax.fori_loop(0, NR0, phase0, 0)

    c_exp = (DH ** -0.5) * math.log2(math.e)
    neg = -1e9 / (DH ** -0.5)

    def attn_unit(r, row0, masked):
        base = r * TM + row0
        qs = [q_s[j, pl.ds(row0, UNIT), :] for j in range(NT)]
        logits = []
        for w in range(W):
            st = base + (HALO - DIL * w)
            s = qs[0] * k_s[0, pl.ds(st, UNIT), :]
            for j in range(1, NT):
                s = s + qs[j] * k_s[j, pl.ds(st, UNIT), :]
            s = s + pltpu.roll(s, 64, 1)
            s = s + pltpu.roll(s, 32, 1)
            if masked and w > 0:
                pos = base + lax.broadcasted_iota(jnp.int32, (UNIT, LANES), 0)
                s = jnp.where(pos >= DIL * w, s, neg)
            logits.append(s)
        m = logits[0]
        for w in range(1, W):
            m = jnp.maximum(m, logits[w])
        ps = [jnp.exp2((logits[w] - m) * c_exp) for w in range(W)]
        den = ps[0]
        for w in range(1, W):
            den = den + ps[w]
        rinv = 1.0 / den
        for j in range(NT):
            o = ps[0] * v_s[j, pl.ds(base + HALO, UNIT), :]
            for w in range(1, W):
                o = o + ps[w] * v_s[j, pl.ds(base + (HALO - DIL * w), UNIT), :]
            o_s[pl.ds(row0, UNIT), pl.ds(j * LANES, LANES)] = (
                o * rinv).astype(_BF16)

    def row_block(r, carry):
        @pl.when(r == 0)
        def _():
            for cp in rest_copies():
                cp.wait()

        rows = pl.ds(pl.multiple_of(r * TM, TM), TM)
        krows = pl.ds(pl.multiple_of(r * TM + HALO, HALO), TM)
        xv = x_v[rows, :]
        for sec, dst in enumerate((q_s, k_s, v_s)):
            wsec = wq_p[pl.ds(2 * sec, 2)].reshape(D, D)
            res = _dot(xv, wsec)
            for j in range(NT):
                piece = res[:, j * LANES:(j + 1) * LANES]
                if sec == 0:
                    dst[j] = piece
                else:
                    dst[j, krows, :] = piece
        z = jnp.sum(xv.astype(_F32) * gw_ref[...].astype(_F32), axis=-1,
                    keepdims=True)
        g_s[...] = jnp.broadcast_to(jax.nn.sigmoid(z), (TM, LANES))
        for j in range(NT):
            wo_f[j] = wo_raw[:, pl.ds(j * LANES, LANES)].astype(_F32)
        for j in range(NT):
            for d in range(DH):
                wo_p[pl.ds(d * H, H), pl.ds(j * LANES, LANES)] = (
                    wo_f[j, pl.ds(d, H, stride=DH), :].astype(_BF16))

        AR = TM // NC

        def fa(c, carry2):
            xv2 = x_v[rows, :]
            gt = _dot(xv2, wg[c])
            up = _dot(xv2, wu[c])
            hh = (jnp.maximum(gt, 0.0) * up).astype(_BF16)
            acc[rows, :] += _dot(hh, wd[c])
            for un in range(AR // UNIT):
                row0 = pl.multiple_of(c * AR + un * UNIT, UNIT)
                attn_unit(r, row0, masked=(un * UNIT < HALO))
            return carry2

        lax.fori_loop(0, NC, fa, 0)

        a = _dot(o_s[...], wo_p[...])
        b = acc[rows, :]
        g = g_s[...]
        for j in range(NT):
            cols = slice(j * LANES, (j + 1) * LANES)
            bj = b[:, cols]
            out_st[r, :, cols] = (bj + g * (a[:, cols] - bj)).astype(_BF16)
        out_copy(r).start()
        return carry

    lax.fori_loop(0, NR, row_block, 0)
    for r in range(NR):
        out_copy(r).wait()


@jax.jit
def pallas_gated_mix__sliding_local_dilated__glu_gated_reglu__prompt_kernel(
    A_x: jax.Array,
    A_wqkv: jax.Array,
    A_wo: jax.Array,
    B_x: jax.Array,
    B_W_gate: jax.Array,
    B_W_up: jax.Array,
    B_W_down: jax.Array,
    gate_w: jax.Array,
):
    del B_x
    B, S, D = A_x.shape
    F = B_W_gate.shape[1]
    assert B == 1 and D == H * DH == NT * LANES
    assert S % TM == 0 and (F - F0) % TF == 0
    NR = S // TM
    NC = (F - F0) // TF
    assert TM % (NC * UNIT) == 0 and S // TM0 >= 8

    any_spec = pl.BlockSpec(memory_space=pl.ANY)
    out = pl.pallas_call(
        functools.partial(_kernel, S=S, D=D, F=F),
        out_shape=jax.ShapeDtypeStruct((S, D), _BF16),
        in_specs=[any_spec] * 6 + [pl.BlockSpec(memory_space=pltpu.VMEM)],
        out_specs=any_spec,
        scratch_shapes=[
            pltpu.VMEM((S, D), _BF16),
            pltpu.VMEM((7, D // 2, D), _BF16),
            pltpu.VMEM((7, D // 2, D), _BF16),
            pltpu.VMEM((D, D), _BF16),
            pltpu.VMEM((NT, D, LANES), _F32),
            pltpu.VMEM((D, D), _BF16),
            pltpu.VMEM((D, F0), _BF16),
            pltpu.VMEM((D, F0), _BF16),
            pltpu.VMEM((F0, D), _BF16),
            pltpu.VMEM((NC, D, TF), _BF16),
            pltpu.VMEM((NC, D, TF), _BF16),
            pltpu.VMEM((NC, TF, D), _BF16),
            pltpu.VMEM((S, D), _F32),
            pltpu.VMEM((NT, TM, LANES), _F32),
            pltpu.VMEM((NT, HALO + S, LANES), _F32),
            pltpu.VMEM((NT, HALO + S, LANES), _F32),
            pltpu.VMEM((TM, LANES), _F32),
            pltpu.VMEM((TM, D), _BF16),
            pltpu.VMEM((NR, TM, D), _BF16),
            pltpu.SemaphoreType.DMA((S // TM0,)),
            pltpu.SemaphoreType.DMA((3,)),
            pltpu.SemaphoreType.DMA((6,)),
            pltpu.SemaphoreType.DMA((2,)),
            pltpu.SemaphoreType.DMA((NR,)),
        ],
        compiler_params=pltpu.CompilerParams(
            vmem_limit_bytes=120 * 1024 * 1024),
        name="gated_mix",
    )(A_x.reshape(S, D), A_wqkv, A_wo, B_W_gate, B_W_up, B_W_down,
      gate_w.reshape(1, D))
    return out.reshape(B, S, D)
```

```python
import functools
import math

import jax
import jax.numpy as jnp
from jax import lax
import jax.experimental.pallas as pl
import jax.experimental.pallas.tpu as pltpu

H = 32
DH = 32
W = 8
DIL = 2
LANES = 128
NT = 8
HALO = 16

TM = 512
TM0 = 256
F0 = 512
TF = 768
UNIT = 16
PB = 4

_F32 = jnp.float32
_BF16 = jnp.bfloat16


def _dot(a, b):
    return jnp.dot(a, b, preferred_element_type=_F32)


def _kernel(x_hbm, wqkv_hbm, wo_hbm, wg_hbm, wu_hbm, wd_hbm, gw_hbm, out_hbm,
            x_v, wq_raw, wq_p, wo_raw, wo_f, wo_p, wg0, wu0, wd0, wg, wu, wd,
            acc, q_s, k_s, v_s, g_s, o_s, out_st, gw_ref,
            sems, sem_out,
            *, S, D, F):
    NR = S // TM
    NR0 = S // TM0
    NC = (F - F0) // TF
    NSL = 6
    HR = D // 2

    SX, SW0, SQ, SR = 0, NR0, NR0 + 3, NR0 + 3 + NSL

    def x_copy(t):
        return pltpu.make_async_copy(
            x_hbm.at[pl.ds(t * TM0, TM0), :], x_v.at[pl.ds(t * TM0, TM0), :],
            sems.at[SX + t])

    def w0_copies():
        return (
            pltpu.make_async_copy(wg_hbm.at[:, pl.ds(0, F0)], wg0, sems.at[SW0 + 0]),
            pltpu.make_async_copy(wu_hbm.at[:, pl.ds(0, F0)], wu0, sems.at[SW0 + 1]),
            pltpu.make_async_copy(wd_hbm.at[pl.ds(0, F0), :], wd0, sems.at[SW0 + 2]),
        )

    def wq_copy(a):
        sec = a // 2
        half = a % 2
        return pltpu.make_async_copy(
            wqkv_hbm.at[pl.ds(half * HR, HR), pl.ds(sec * D, D)],
            wq_raw.at[a], sems.at[SQ + a])

    def misc_copies():
        return (pltpu.make_async_copy(gw_hbm, gw_ref, sems.at[SR]),
                pltpu.make_async_copy(wo_hbm, wo_raw, sems.at[SR]))

    def ffn_copies(c):
        lo = F0 + c * TF
        if not isinstance(c, int):
            lo = pl.multiple_of(lo, LANES)
        sem = sems.at[SR + 1 + c]
        return (
            pltpu.make_async_copy(wg_hbm.at[:, pl.ds(lo, TF)], wg.at[c], sem),
            pltpu.make_async_copy(wu_hbm.at[:, pl.ds(lo, TF)], wu.at[c], sem),
            pltpu.make_async_copy(wd_hbm.at[pl.ds(lo, TF), :], wd.at[c], sem),
        )

    def out_copy(r):
        return pltpu.make_async_copy(
            out_st.at[r], out_hbm.at[pl.ds(r * TM, TM), :], sem_out.at[r])

    x_copy(0).start()
    for cp in w0_copies():
        cp.start()
    for t in range(1, NR0):
        x_copy(t).start()
        if t - 1 < NSL:
            wq_copy(t - 1).start()
    for cp in misc_copies():
        cp.start()
    for c in range(NC):
        for cp in ffn_copies(c):
            cp.start()

    zeros_halo = jnp.zeros((HALO, LANES), _F32)
    for j in range(NT):
        k_s[j, pl.ds(0, HALO), :] = zeros_halo
        v_s[j, pl.ds(0, HALO), :] = zeros_halo

    def permute_slice(a):
        rows = PB * 8
        lane = lax.broadcasted_iota(jnp.int32, (rows, LANES), 1)
        bits = [((lane >> (2 + b)) & 1) == 1 for b in range(3)]
        base_pat = NT * 4 * (lane & 3) + (lane >> 5) + 4 * ((lane >> 2) & 7)
        pats = [(base_pat + 4 * j) & (LANES - 1) for j in range(NT)]
        for g in range(HR // (16 * PB)):
            rs = pl.ds(g * 16 * PB, 16 * PB)
            z = []
            for i in range(NT):
                w = pltpu.bitcast(wq_raw[a, rs, pl.ds(i * LANES, LANES)],
                                  jnp.uint32)
                z.append(w if i == 0 else pltpu.roll(w, 4 * i, 1))
            for b in range(3):
                z = [jnp.where(bits[b], z[(k + (1 << b)) % NT], z[k])
                     for k in range(NT)]
            for j in range(NT):
                y = jnp.take_along_axis(z[(-j) % NT], pats[j], axis=1)
                wq_p[a, rs, pl.ds(j * LANES, LANES)] = pltpu.bitcast(y, _BF16)

    def phase0(t, carry):
        x_copy(t).wait()

        @pl.when(t == 0)
        def _():
            for cp in w0_copies():
                cp.wait()

        real = jnp.logical_and(t >= 1, t <= NSL)

        @pl.when(real)
        def _():
            wq_copy(t - 1).wait()

        rows = pl.ds(pl.multiple_of(t * TM0, TM0), TM0)
        xv = x_v[rows, :]
        gt = _dot(xv, wg0[...])
        up = _dot(xv, wu0[...])
        hh = (jnp.maximum(gt, 0.0) * up).astype(_BF16)
        acc[rows, :] = _dot(hh, wd0[...])
        permute_slice(jnp.where(real, t - 1, NSL))
        return carry

    lax.fori_loop(0, NR0, phase0, 0)

    c_exp = (DH ** -0.5) * math.log2(math.e)
    neg = -1e9 / (DH ** -0.5)

    def attn_unit(r, row0, masked):
        base = r * TM + row0
        qs = [q_s[j, pl.ds(row0, UNIT), :] for j in range(NT)]
        logits = []
        for w in range(W):
            st = base + (HALO - DIL * w)
            s = qs[0] * k_s[0, pl.ds(st, UNIT), :]
            for j in range(1, NT):
                s = s + qs[j] * k_s[j, pl.ds(st, UNIT), :]
            s = s + pltpu.roll(s, 64, 1)
            s = s + pltpu.roll(s, 32, 1)
            if masked and w > 0:
                pos = base + lax.broadcasted_iota(jnp.int32, (UNIT, LANES), 0)
                s = jnp.where(pos >= DIL * w, s, neg)
            logits.append(s)
        m = logits[0]
        for w in range(1, W):
            m = jnp.maximum(m, logits[w])
        ps = [jnp.exp2((logits[w] - m) * c_exp) for w in range(W)]
        den = ps[0]
        for w in range(1, W):
            den = den + ps[w]
        rinv = 1.0 / den
        for j in range(NT):
            o = ps[0] * v_s[j, pl.ds(base + HALO, UNIT), :]
            for w in range(1, W):
                o = o + ps[w] * v_s[j, pl.ds(base + (HALO - DIL * w), UNIT), :]
            o_s[pl.ds(row0, UNIT), pl.ds(j * LANES, LANES)] = (
                o * rinv).astype(_BF16)

    def row_block(r, carry):
        @pl.when(r == 0)
        def _():
            for cp in misc_copies():
                cp.wait()

        rows = pl.ds(pl.multiple_of(r * TM, TM), TM)
        krows = pl.ds(pl.multiple_of(r * TM + HALO, HALO), TM)
        xv = x_v[rows, :]
        for sec, dst in enumerate((q_s, k_s, v_s)):
            wsec = wq_p[pl.ds(2 * sec, 2)].reshape(D, D)
            res = _dot(xv, wsec)
            for j in range(NT):
                piece = res[:, j * LANES:(j + 1) * LANES]
                if sec == 0:
                    dst[j] = piece
                else:
                    dst[j, krows, :] = piece
        z = jnp.sum(xv.astype(_F32) * gw_ref[...].astype(_F32).reshape(1, D), axis=-1,
                    keepdims=True)
        g_s[...] = jnp.broadcast_to(jax.nn.sigmoid(z), (TM, LANES))
        for j in range(NT):
            cols = pl.ds(j * LANES, LANES)
            for h in range(H):
                blk = wo_raw[pl.ds(h * DH, DH), cols].astype(_F32)
                for a in range(4):
                    wo_f[j, (h // 8) * 4 + a, pl.ds((h % 8) * 8, 8), :] = (
                        blk[a * 8:(a + 1) * 8])
            for d in range(DH):
                rws = [wo_f[j, b * 4 + d // 8, pl.ds(d % 8, 8, stride=8), :]
                       for b in range(4)]
                wo_p[pl.ds(d * H, H), cols] = jnp.concatenate(
                    rws, axis=0).astype(_BF16)

        AR = TM // NC

        def fa(c, carry2):
            @pl.when(r == 0)
            def _():
                for cp in ffn_copies(c):
                    cp.wait()

            xv2 = x_v[rows, :]
            gt = _dot(xv2, wg[c])
            up = _dot(xv2, wu[c])
            hh = (jnp.maximum(gt, 0.0) * up).astype(_BF16)
            acc[rows, :] += _dot(hh, wd[c])
            for un in range(AR // UNIT):
                row0 = pl.multiple_of(c * AR + un * UNIT, UNIT)
                attn_unit(r, row0, masked=(un * UNIT < HALO))
            return carry2

        lax.fori_loop(0, NC, fa, 0)

        a = _dot(o_s[...], wo_p[...])
        b = acc[rows, :]
        g = g_s[...]
        for j in range(NT):
            cols = slice(j * LANES, (j + 1) * LANES)
            bj = b[:, cols]
            out_st[r, :, cols] = (bj + g * (a[:, cols] - bj)).astype(_BF16)
        out_copy(r).start()
        return carry

    lax.fori_loop(0, NR, row_block, 0)
    for r in range(NR):
        out_copy(r).wait()


@jax.jit
def pallas_gated_mix__sliding_local_dilated__glu_gated_reglu__prompt_kernel(
    A_x: jax.Array,
    A_wqkv: jax.Array,
    A_wo: jax.Array,
    B_x: jax.Array,
    B_W_gate: jax.Array,
    B_W_up: jax.Array,
    B_W_down: jax.Array,
    gate_w: jax.Array,
):
    del B_x
    B, S, D = A_x.shape
    F = B_W_gate.shape[1]
    assert B == 1 and D == H * DH == NT * LANES
    assert S % TM == 0 and (F - F0) % TF == 0
    NR = S // TM
    NC = (F - F0) // TF
    assert TM % (NC * UNIT) == 0 and S // TM0 >= 8

    any_spec = pl.BlockSpec(memory_space=pl.ANY)
    out = pl.pallas_call(
        functools.partial(_kernel, S=S, D=D, F=F),
        out_shape=jax.ShapeDtypeStruct((S, D), _BF16),
        in_specs=[any_spec] * 7,
        out_specs=any_spec,
        scratch_shapes=[
            pltpu.VMEM((S, D), _BF16),
            pltpu.VMEM((7, D // 2, D), _BF16),
            pltpu.VMEM((7, D // 2, D), _BF16),
            pltpu.VMEM((D, D), _BF16),
            pltpu.VMEM((NT, 16, 64, LANES), _F32),
            pltpu.VMEM((D, D), _BF16),
            pltpu.VMEM((D, F0), _BF16),
            pltpu.VMEM((D, F0), _BF16),
            pltpu.VMEM((F0, D), _BF16),
            pltpu.VMEM((NC, D, TF), _BF16),
            pltpu.VMEM((NC, D, TF), _BF16),
            pltpu.VMEM((NC, TF, D), _BF16),
            pltpu.VMEM((S, D), _F32),
            pltpu.VMEM((NT, TM, LANES), _F32),
            pltpu.VMEM((NT, HALO + S, LANES), _F32),
            pltpu.VMEM((NT, HALO + S, LANES), _F32),
            pltpu.VMEM((TM, LANES), _F32),
            pltpu.VMEM((TM, D), _BF16),
            pltpu.VMEM((NR, TM, D), _BF16),
            pltpu.VMEM((D,), _BF16),
            pltpu.SemaphoreType.DMA((S // TM0 + 10 + NC,)),
            pltpu.SemaphoreType.DMA((NR,)),
        ],
        compiler_params=pltpu.CompilerParams(
            vmem_limit_bytes=120 * 1024 * 1024),
        name="gated_mix",
    )(A_x.reshape(S, D), A_wqkv, A_wo, B_W_gate, B_W_up, B_W_down,
      gate_w)
    return out.reshape(B, S, D)
```

```python
import functools
import math

import jax
import jax.numpy as jnp
from jax import lax
import jax.experimental.pallas as pl
import jax.experimental.pallas.tpu as pltpu

H = 32
DH = 32
W = 8
DIL = 2
LANES = 128
NT = 8
HALO = 16

TM = 512
TM0 = 256
F0 = 512
TF = 768
UNIT = 16
WOC = 256
WOP = 33
PB = 4

_F32 = jnp.float32
_BF16 = jnp.bfloat16


def _dot(a, b):
    return jnp.dot(a, b, preferred_element_type=_F32)


def _kernel(x_hbm, wqkv_hbm, wo_hbm, wg_hbm, wu_hbm, wd_hbm, gw_hbm, out_hbm,
            x_v, wq_raw, wq_p, wo_raw, wo_f, wo_p, wg0, wu0, wd0, wg, wu, wd,
            acc, q_s, k_s, v_s, g_s, o_s, out_st, gw_ref,
            sems, sem_out,
            *, S, D, F):
    NR = S // TM
    NR0 = S // TM0
    NC = (F - F0) // TF
    NSL = 6
    HR = D // 2

    NWO = D // WOC
    SX = 0
    SW0 = SX + NR0
    SQ = SW0 + 4
    SO = SQ + NSL
    SR = SO + NWO

    def x_copy(t):
        return pltpu.make_async_copy(
            x_hbm.at[pl.ds(t * TM0, TM0), :], x_v.at[pl.ds(t * TM0, TM0), :],
            sems.at[SX + t])

    def w0_copies():
        return (
            pltpu.make_async_copy(wg_hbm.at[:, pl.ds(0, F0)], wg0, sems.at[SW0 + 0]),
            pltpu.make_async_copy(wu_hbm.at[:, pl.ds(0, F0)], wu0, sems.at[SW0 + 1]),
            pltpu.make_async_copy(wd_hbm.at[pl.ds(0, F0), :], wd0, sems.at[SW0 + 2]),
            pltpu.make_async_copy(gw_hbm, gw_ref, sems.at[SW0 + 3]),
        )

    def wq_copy(a):
        sec = a // 2
        half = a % 2
        return pltpu.make_async_copy(
            wqkv_hbm.at[pl.ds(half * HR, HR), pl.ds(sec * D, D)],
            wq_raw.at[a], sems.at[SQ + a])

    def wo_copy(n):
        lo = n * WOC
        if not isinstance(n, int):
            lo = pl.multiple_of(lo, LANES)
        return pltpu.make_async_copy(
            wo_hbm.at[:, pl.ds(lo, WOC)], wo_raw.at[n], sems.at[SO + n])

    def ffn_copies(c):
        lo = F0 + c * TF
        if not isinstance(c, int):
            lo = pl.multiple_of(lo, LANES)
        sem = sems.at[SR + c]
        return (
            pltpu.make_async_copy(wg_hbm.at[:, pl.ds(lo, TF)], wg.at[c], sem),
            pltpu.make_async_copy(wu_hbm.at[:, pl.ds(lo, TF)], wu.at[c], sem),
            pltpu.make_async_copy(wd_hbm.at[pl.ds(lo, TF), :], wd.at[c], sem),
        )

    def out_copy(r):
        return pltpu.make_async_copy(
            out_st.at[r], out_hbm.at[pl.ds(r * TM, TM), :], sem_out.at[r])

    x_copy(0).start()
    for cp in w0_copies():
        cp.start()
    for t in range(1, NR0):
        x_copy(t).start()
        if t - 1 < NSL:
            wq_copy(t - 1).start()
        if t >= NR0 - NWO:
            wo_copy(t - (NR0 - NWO)).start()
    for c in range(NC):
        for cp in ffn_copies(c):
            cp.start()

    zeros_halo = jnp.zeros((HALO, LANES), _F32)
    for j in range(NT):
        k_s[j, pl.ds(0, HALO), :] = zeros_halo
        v_s[j, pl.ds(0, HALO), :] = zeros_halo

    def permute_slice(a):
        rows = PB * 8
        lane = lax.broadcasted_iota(jnp.int32, (rows, LANES), 1)
        bits = [((lane >> (2 + b)) & 1) == 1 for b in range(3)]
        base_pat = NT * 4 * (lane & 3) + (lane >> 5) + 4 * ((lane >> 2) & 7)
        pats = [(base_pat + 4 * j) & (LANES - 1) for j in range(NT)]
        for g in range(HR // (16 * PB)):
            rs = pl.ds(g * 16 * PB, 16 * PB)
            z = []
            for i in range(NT):
                w = pltpu.bitcast(wq_raw[a, rs, pl.ds(i * LANES, LANES)],
                                  jnp.uint32)
                z.append(w if i == 0 else pltpu.roll(w, 4 * i, 1))
            for b in range(3):
                z = [jnp.where(bits[b], z[(k + (1 << b)) % NT], z[k])
                     for k in range(NT)]
            for j in range(NT):
                y = jnp.take_along_axis(z[(-j) % NT], pats[j], axis=1)
                wq_p[a, rs, pl.ds(j * LANES, LANES)] = pltpu.bitcast(y, _BF16)

    def permute_wo(n):
        nj = WOC // LANES
        for h in range(H):
            blk = wo_raw[n, pl.ds(h * DH, DH), :].astype(_F32)
            for j in range(nj):
                wo_f[j, pl.ds(h * WOP, DH), :] = (
                    blk[:, j * LANES:(j + 1) * LANES])
        for d in range(DH):
            rws = [wo_f[j, pl.ds(d, H, stride=WOP), :] for j in range(nj)]
            wo_p[n, pl.ds(d * H, H), :] = jnp.concatenate(
                rws, axis=1).astype(_BF16)

    def phase0(t, carry):
        x_copy(t).wait()

        @pl.when(t == 0)
        def _():
            for cp in w0_copies():
                cp.wait()

        real = jnp.logical_and(t >= 1, t <= NSL)

        @pl.when(real)
        def _():
            wq_copy(t - 1).wait()

        real_o = t >= NR0 - NWO

        @pl.when(real_o)
        def _():
            wo_copy(t - (NR0 - NWO)).wait()

        rows = pl.ds(pl.multiple_of(t * TM0, TM0), TM0)
        xv = x_v[rows, :]
        gt = _dot(xv, wg0[...])
        up = _dot(xv, wu0[...])
        hh = (jnp.maximum(gt, 0.0) * up).astype(_BF16)
        acc[rows, :] = _dot(hh, wd0[...])
        permute_slice(jnp.where(real, t - 1, NSL))
        permute_wo(jnp.where(real_o, t - (NR0 - NWO), NWO))
        return carry

    lax.fori_loop(0, NR0, phase0, 0)

    c_exp = (DH ** -0.5) * math.log2(math.e)
    neg = -1e9 / (DH ** -0.5)

    def attn_unit(r, row0, gw, masked):
        base = r * TM + row0
        qs = [q_s[j, pl.ds(row0, UNIT), :] for j in range(NT)]
        logits = []
        for w in range(W):
            st = base + (HALO - DIL * w)
            s = qs[0] * k_s[0, pl.ds(st, UNIT), :]
            for j in range(1, NT):
                s = s + qs[j] * k_s[j, pl.ds(st, UNIT), :]
            s = s + pltpu.roll(s, 64, 1)
            s = s + pltpu.roll(s, 32, 1)
            if masked and w > 0:
                pos = base + lax.broadcasted_iota(jnp.int32, (UNIT, LANES), 0)
                s = jnp.where(pos >= DIL * w, s, neg)
            logits.append(s)
        m = logits[0]
        for w in range(1, W):
            m = jnp.maximum(m, logits[w])
        ps = [jnp.exp2((logits[w] - m) * c_exp) for w in range(W)]
        den = ps[0]
        for w in range(1, W):
            den = den + ps[w]
        xg = x_v[pl.ds(pl.multiple_of(base, UNIT), UNIT), :].astype(_F32) * gw
        gate = jax.nn.sigmoid(jnp.sum(xg, axis=-1, keepdims=True))
        gate = jnp.broadcast_to(gate, (UNIT, LANES))
        g_s[pl.ds(row0, UNIT), :] = 1.0 - gate
        rinv = gate / den
        for j in range(NT):
            o = ps[0] * v_s[j, pl.ds(base + HALO, UNIT), :]
            for w in range(1, W):
                o = o + ps[w] * v_s[j, pl.ds(base + (HALO - DIL * w), UNIT), :]
            o_s[pl.ds(row0, UNIT), pl.ds(j * LANES, LANES)] = (
                o * rinv).astype(_BF16)

    def row_block(r, carry):
        rows = pl.ds(pl.multiple_of(r * TM, TM), TM)
        krows = pl.ds(pl.multiple_of(r * TM + HALO, HALO), TM)
        xv = x_v[rows, :]
        for sec, dst in enumerate((q_s, k_s, v_s)):
            wsec = wq_p[pl.ds(2 * sec, 2)].reshape(D, D)
            res = _dot(xv, wsec)
            for j in range(NT):
                piece = res[:, j * LANES:(j + 1) * LANES]
                if sec == 0:
                    dst[j] = piece
                else:
                    dst[j, krows, :] = piece
        AR = TM // NC

        def fa(c, carry2):
            @pl.when(r == 0)
            def _():
                for cp in ffn_copies(c):
                    cp.wait()

            xv2 = x_v[rows, :]
            gt = _dot(xv2, wg[c])
            up = _dot(xv2, wu[c])
            hh = (jnp.maximum(gt, 0.0) * up).astype(_BF16)
            acc[rows, :] += _dot(hh, wd[c])
            gw = gw_ref[...].astype(_F32).reshape(1, D)
            for un in range(AR // UNIT):
                row0 = pl.multiple_of(c * AR + un * UNIT, UNIT)
                attn_unit(r, row0, gw, masked=(un * UNIT < HALO))
            return carry2

        lax.fori_loop(0, NC, fa, 0)

        ov = o_s[...]
        g1 = g_s[...]
        g1 = jnp.concatenate([g1] * (WOC // LANES), axis=1)
        for n in range(NWO):
            cols = pl.ds(n * WOC, WOC)
            a = _dot(ov, wo_p[n])
            out_st[r, :, cols] = (a + g1 * acc[rows, cols]).astype(_BF16)
        out_copy(r).start()
        return carry

    lax.fori_loop(0, NR, row_block, 0)
    for r in range(NR):
        out_copy(r).wait()


@jax.jit
def pallas_gated_mix__sliding_local_dilated__glu_gated_reglu__prompt_kernel(
    A_x: jax.Array,
    A_wqkv: jax.Array,
    A_wo: jax.Array,
    B_x: jax.Array,
    B_W_gate: jax.Array,
    B_W_up: jax.Array,
    B_W_down: jax.Array,
    gate_w: jax.Array,
):
    del B_x
    B, S, D = A_x.shape
    F = B_W_gate.shape[1]
    assert B == 1 and D == H * DH == NT * LANES
    assert S % TM == 0 and (F - F0) % TF == 0
    NR = S // TM
    NC = (F - F0) // TF
    assert TM % (NC * UNIT) == 0 and S // TM0 >= 8

    any_spec = pl.BlockSpec(memory_space=pl.ANY)
    out = pl.pallas_call(
        functools.partial(_kernel, S=S, D=D, F=F),
        out_shape=jax.ShapeDtypeStruct((S, D), _BF16),
        in_specs=[any_spec] * 7,
        out_specs=any_spec,
        scratch_shapes=[
            pltpu.VMEM((S, D), _BF16),
            pltpu.VMEM((7, D // 2, D), _BF16),
            pltpu.VMEM((7, D // 2, D), _BF16),
            pltpu.VMEM((D // WOC + 1, D, WOC), _BF16),
            pltpu.VMEM((WOC // LANES, H * (WOP + 1), LANES), _F32),
            pltpu.VMEM((D // WOC + 1, D, WOC), _BF16),
            pltpu.VMEM((D, F0), _BF16),
            pltpu.VMEM((D, F0), _BF16),
            pltpu.VMEM((F0, D), _BF16),
            pltpu.VMEM((NC, D, TF), _BF16),
            pltpu.VMEM((NC, D, TF), _BF16),
            pltpu.VMEM((NC, TF, D), _BF16),
            pltpu.VMEM((S, D), _F32),
            pltpu.VMEM((NT, TM, LANES), _F32),
            pltpu.VMEM((NT, HALO + S, LANES), _F32),
            pltpu.VMEM((NT, HALO + S, LANES), _F32),
            pltpu.VMEM((TM, LANES), _F32),
            pltpu.VMEM((TM, D), _BF16),
            pltpu.VMEM((NR, TM, D), _BF16),
            pltpu.VMEM((D,), _BF16),
            pltpu.SemaphoreType.DMA((S // TM0 + 10 + D // WOC + NC,)),
            pltpu.SemaphoreType.DMA((NR,)),
        ],
        compiler_params=pltpu.CompilerParams(
            vmem_limit_bytes=120 * 1024 * 1024),
        name="gated_mix",
    )(A_x.reshape(S, D), A_wqkv, A_wo, B_W_gate, B_W_up, B_W_down,
      gate_w)
    return out.reshape(B, S, D)
```

```python
import functools
import math

import jax
import jax.numpy as jnp
from jax import lax
import jax.experimental.pallas as pl
import jax.experimental.pallas.tpu as pltpu

H = 32
DH = 32
W = 8
DIL = 2
LANES = 128
NT = 8
HALO = 16

TM = 512
TM0 = 256
F0 = 512
TF = 768
UNIT = 8
WOC = 256
WOP = 9
CHAIN_QK = True
CHAIN_PV = True
CHAIN_UNITS = 2
WO_P2 = 3
PB = 4

_F32 = jnp.float32
_BF16 = jnp.bfloat16


def _dot(a, b):
    return jnp.dot(a, b, preferred_element_type=_F32)


def _kernel(x_hbm, wqkv_hbm, wo_hbm, wg_hbm, wu_hbm, wd_hbm, gw_hbm, out_hbm,
            x_v, wq_raw, wq_p, wo_raw, wo_f, wo_p, wg0, wu0, wd0, wg, wu, wd,
            acc, q_s, k_s, v_s, g_s, o_s, out_st, gw_ref,
            sems, sem_out,
            *, S, D, F):
    NR = S // TM
    NR0 = S // TM0
    NC = (F - F0) // TF
    NSL = 6
    HR = D // 2

    NWO = D // WOC
    SX = 0
    SW0 = SX + NR0
    SQ = SW0 + 4
    SO = SQ + NSL
    SR = SO + NWO

    def x_copy(t):
        return pltpu.make_async_copy(
            x_hbm.at[pl.ds(t * TM0, TM0), :], x_v.at[pl.ds(t * TM0, TM0), :],
            sems.at[SX + t])

    def w0_copies():
        return (
            pltpu.make_async_copy(wg_hbm.at[:, pl.ds(0, F0)], wg0, sems.at[SW0 + 0]),
            pltpu.make_async_copy(wu_hbm.at[:, pl.ds(0, F0)], wu0, sems.at[SW0 + 1]),
            pltpu.make_async_copy(wd_hbm.at[pl.ds(0, F0), :], wd0, sems.at[SW0 + 2]),
            pltpu.make_async_copy(gw_hbm, gw_ref, sems.at[SW0 + 3]),
        )

    def wq_copy(a):
        sec = a // 2
        half = a % 2
        return pltpu.make_async_copy(
            wqkv_hbm.at[pl.ds(half * HR, HR), pl.ds(sec * D, D)],
            wq_raw.at[a], sems.at[SQ + a])

    def wo_copy(n):
        lo = n * WOC
        if not isinstance(n, int):
            lo = pl.multiple_of(lo, LANES)
        return pltpu.make_async_copy(
            wo_hbm.at[:, pl.ds(lo, WOC)], wo_raw.at[n], sems.at[SO + n])

    def ffn_copies(c):
        lo = F0 + c * TF
        if not isinstance(c, int):
            lo = pl.multiple_of(lo, LANES)
        sem = sems.at[SR + c]
        return (
            pltpu.make_async_copy(wg_hbm.at[:, pl.ds(lo, TF)], wg.at[c], sem),
            pltpu.make_async_copy(wu_hbm.at[:, pl.ds(lo, TF)], wu.at[c], sem),
            pltpu.make_async_copy(wd_hbm.at[pl.ds(lo, TF), :], wd.at[c], sem),
        )

    def out_copy(r):
        return pltpu.make_async_copy(
            out_st.at[r], out_hbm.at[pl.ds(r * TM, TM), :], sem_out.at[r])

    x_copy(0).start()
    for cp in w0_copies():
        cp.start()
    for t in range(1, NR0):
        x_copy(t).start()
        if t - 1 < NSL:
            wq_copy(t - 1).start()
        if t >= NR0 - NWO:
            wo_copy(t - (NR0 - NWO)).start()
    for c in range(NC):
        for cp in ffn_copies(c):
            cp.start()

    zeros_halo = jnp.zeros((HALO, LANES), _F32)
    for j in range(NT):
        k_s[j, pl.ds(0, HALO), :] = zeros_halo
        v_s[j, pl.ds(0, HALO), :] = zeros_halo

    def permute_slice(a):
        rows = PB * 8
        lane = lax.broadcasted_iota(jnp.int32, (rows, LANES), 1)
        bits = [((lane >> (2 + b)) & 1) == 1 for b in range(3)]
        base_pat = NT * 4 * (lane & 3) + (lane >> 5) + 4 * ((lane >> 2) & 7)
        pats = [(base_pat + 4 * j) & (LANES - 1) for j in range(NT)]
        for g in range(HR // (16 * PB)):
            rs = pl.ds(g * 16 * PB, 16 * PB)
            z = []
            for i in range(NT):
                w = pltpu.bitcast(wq_raw[a, rs, pl.ds(i * LANES, LANES)],
                                  jnp.uint32)
                z.append(w if i == 0 else pltpu.roll(w, 4 * i, 1))
            for b in range(3):
                z = [jnp.where(bits[b], z[(k + (1 << b)) % NT], z[k])
                     for k in range(NT)]
            for j in range(NT):
                y = jnp.take_along_axis(z[(-j) % NT], pats[j], axis=1)
                wq_p[a, rs, pl.ds(j * LANES, LANES)] = pltpu.bitcast(y, _BF16)

    def permute_wo(n, never, pace1, pace2):
        nj = WOC // LANES
        i = 0
        for h in range(H):
            blk = wo_raw[n, pl.ds(h * DH, DH), :].astype(_F32)
            for a in range(DH // 8):
                for j in range(nj):
                    pc = blk[a * 8:(a + 1) * 8, j * LANES:(j + 1) * LANES]
                    pc = jnp.where(never, pace1[i], pc)
                    i += 1
                    wo_f[a * nj + j][pl.ds(h * WOP, 8), :] = pc
        i = 0
        for d in range(DH):
            for b in range(H // 8):
                rws = []
                for j in range(nj):
                    pc = wo_f[(d // 8) * nj + j][
                        pl.ds(b * 8 * WOP + d % 8, 8, stride=WOP), :]
                    pc = jnp.where(never, pace2[i], pc)
                    i += 1
                    rws.append(pc)
                wo_p[n, pl.ds(d * H + b * 8, 8), :] = jnp.concatenate(
                    rws, axis=1).astype(_BF16)

    def vregs(v):
        return [v[i * 8:(i + 1) * 8, n * LANES:(n + 1) * LANES]
                for n in range(v.shape[1] // LANES)
                for i in range(v.shape[0] // 8)]

    def phase0(t, carry):
        x_copy(t).wait()

        @pl.when(t == 0)
        def _():
            for cp in w0_copies():
                cp.wait()

        real = jnp.logical_and(t >= 1, t <= NSL)

        @pl.when(real)
        def _():
            wq_copy(t - 1).wait()

        real_o = t >= NR0 - NWO

        @pl.when(real_o)
        def _():
            wo_copy(t - (NR0 - NWO)).wait()

        rows = pl.ds(pl.multiple_of(t * TM0, TM0), TM0)
        xv = x_v[rows, :]
        gt = _dot(xv, wg0[...])
        up = _dot(xv, wu0[...])
        hh = (jnp.maximum(gt, 0.0) * up).astype(_BF16)
        dn = _dot(hh, wd0[...])
        acc[rows, :] = dn
        permute_slice(jnp.where(real, t - 1, NSL))
        never = lax.broadcasted_iota(jnp.int32, (8, LANES), 1) < -1 - t
        p2 = vregs(dn)
        p2 = [p2[i * WO_P2 // 4] for i in range(len(p2))]
        permute_wo(jnp.where(real_o, t - (NR0 - NWO), NWO), never,
                   vregs(gt) + vregs(up), p2)
        return carry

    lax.fori_loop(0, NR0, phase0, 0)

    c_exp = (DH ** -0.5) * math.log2(math.e)
    neg = -1e9 / (DH ** -0.5)

    def attn_unit(r, row0, gw, never, link, masked):
        def tie(a, b):
            return a if b is None else jnp.where(never, b, a)

        base = r * TM + row0
        qs = [q_s[j, pl.ds(row0, UNIT), :] for j in range(NT)]
        logits = []
        for w in range(W):
            st = base + (HALO - DIL * w)
            q0 = tie(qs[0], link) if CHAIN_QK else qs[0]
            s = q0 * k_s[0, pl.ds(st, UNIT), :]
            for j in range(1, NT):
                s = s + qs[j] * k_s[j, pl.ds(st, UNIT), :]
            link = s
            s = s + pltpu.roll(s, 64, 1)
            s = s + pltpu.roll(s, 32, 1)
            if masked and w > 0:
                pos = base + lax.broadcasted_iota(jnp.int32, (UNIT, LANES), 0)
                s = jnp.where(pos >= DIL * w, s, neg)
            logits.append(s)
        m = logits[0]
        for w in range(1, W):
            m = jnp.maximum(m, logits[w])
        ps = [jnp.exp2((logits[w] - m) * c_exp) for w in range(W)]
        den = ps[0]
        for w in range(1, W):
            den = den + ps[w]
        xg = x_v[pl.ds(pl.multiple_of(base, UNIT), UNIT), :].astype(_F32) * gw
        gate = jax.nn.sigmoid(jnp.sum(xg, axis=-1, keepdims=True))
        gate = jnp.broadcast_to(gate, (UNIT, LANES))
        g_s[pl.ds(row0, UNIT), :] = 1.0 - gate
        rinv = gate / den
        olink = None
        for j in range(NT):
            p0 = tie(ps[0], olink) if CHAIN_PV else ps[0]
            o = p0 * v_s[j, pl.ds(base + HALO, UNIT), :]
            for w in range(1, W):
                o = o + ps[w] * v_s[j, pl.ds(base + (HALO - DIL * w), UNIT), :]
            olink = o
            o_s[pl.ds(row0, UNIT), pl.ds(j * LANES, LANES)] = (
                o * rinv).astype(_BF16)
        return olink if CHAIN_UNITS == 2 else (link if CHAIN_UNITS else None)

    def row_block(r, carry):
        rows = pl.ds(pl.multiple_of(r * TM, TM), TM)
        krows = pl.ds(pl.multiple_of(r * TM + HALO, HALO), TM)
        xv = x_v[rows, :]
        for sec, dst in enumerate((q_s, k_s, v_s)):
            wsec = wq_p[pl.ds(2 * sec, 2)].reshape(D, D)
            res = _dot(xv, wsec)
            for j in range(NT):
                piece = res[:, j * LANES:(j + 1) * LANES]
                if sec == 0:
                    dst[j] = piece
                else:
                    dst[j, krows, :] = piece
        AR = TM // NC

        def fa(c, carry2):
            @pl.when(r == 0)
            def _():
                for cp in ffn_copies(c):
                    cp.wait()

            gw = gw_ref[...].astype(_F32).reshape(1, D)
            nun = AR // UNIT

            never = lax.broadcasted_iota(jnp.int32, (UNIT, LANES), 1) < -1 - c
            link = None
            for un in range(nun):
                row0 = pl.multiple_of(c * AR + un * UNIT, UNIT)
                link = attn_unit(r, row0, gw, never, link,
                                 masked=(un * UNIT < HALO))
            xv2 = x_v[rows, :]
            gt = _dot(xv2, wg[c])
            up = _dot(xv2, wu[c])
            hh = (jnp.maximum(gt, 0.0) * up).astype(_BF16)
            acc[rows, :] += _dot(hh, wd[c])
            return carry2

        lax.fori_loop(0, NC, fa, 0)

        ov = o_s[...]
        g1 = g_s[...]
        g1 = jnp.concatenate([g1] * (WOC // LANES), axis=1)
        for n in range(NWO):
            cols = pl.ds(n * WOC, WOC)
            a = _dot(ov, wo_p[n])
            out_st[r, :, cols] = (a + g1 * acc[rows, cols]).astype(_BF16)
        out_copy(r).start()
        return carry

    lax.fori_loop(0, NR, row_block, 0)
    for r in range(NR):
        out_copy(r).wait()


@jax.jit
def pallas_gated_mix__sliding_local_dilated__glu_gated_reglu__prompt_kernel(
    A_x: jax.Array,
    A_wqkv: jax.Array,
    A_wo: jax.Array,
    B_x: jax.Array,
    B_W_gate: jax.Array,
    B_W_up: jax.Array,
    B_W_down: jax.Array,
    gate_w: jax.Array,
):
    del B_x
    B, S, D = A_x.shape
    F = B_W_gate.shape[1]
    assert B == 1 and D == H * DH == NT * LANES
    assert S % TM == 0 and (F - F0) % TF == 0
    NR = S // TM
    NC = (F - F0) // TF
    assert TM % (NC * UNIT) == 0 and S // TM0 >= 8

    any_spec = pl.BlockSpec(memory_space=pl.ANY)
    out = pl.pallas_call(
        functools.partial(_kernel, S=S, D=D, F=F),
        out_shape=jax.ShapeDtypeStruct((S, D), _BF16),
        in_specs=[any_spec] * 7,
        out_specs=any_spec,
        scratch_shapes=[
            pltpu.VMEM((S, D), _BF16),
            pltpu.VMEM((7, D // 2, D), _BF16),
            pltpu.VMEM((7, D // 2, D), _BF16),
            pltpu.VMEM((D // WOC + 1, D, WOC), _BF16),
            [pltpu.VMEM((H * WOP, LANES), _F32)] * (WOC // LANES * DH // 8),
            pltpu.VMEM((D // WOC + 1, D, WOC), _BF16),
            pltpu.VMEM((D, F0), _BF16),
            pltpu.VMEM((D, F0), _BF16),
            pltpu.VMEM((F0, D), _BF16),
            pltpu.VMEM((NC, D, TF), _BF16),
            pltpu.VMEM((NC, D, TF), _BF16),
            pltpu.VMEM((NC, TF, D), _BF16),
            pltpu.VMEM((S, D), _F32),
            pltpu.VMEM((NT, TM, LANES), _F32),
            pltpu.VMEM((NT, HALO + S, LANES), _F32),
            pltpu.VMEM((NT, HALO + S, LANES), _F32),
            pltpu.VMEM((TM, LANES), _F32),
            pltpu.VMEM((TM, D), _BF16),
            pltpu.VMEM((NR, TM, D), _BF16),
            pltpu.VMEM((D,), _BF16),
            pltpu.SemaphoreType.DMA((S // TM0 + 10 + D // WOC + NC,)),
            pltpu.SemaphoreType.DMA((NR,)),
        ],
        compiler_params=pltpu.CompilerParams(
            vmem_limit_bytes=120 * 1024 * 1024),
        name="gated_mix",
    )(A_x.reshape(S, D), A_wqkv, A_wo, B_W_gate, B_W_up, B_W_down,
      gate_w)
    return out.reshape(B, S, D)
```

```python
import functools
import math

import jax
import jax.numpy as jnp
from jax import lax
import jax.experimental.pallas as pl
import jax.experimental.pallas.tpu as pltpu

H = 32
DH = 32
W = 8
DIL = 2
LANES = 128
NT = 8
HALO = 16

TM = 512
TM0 = 256
F0 = 512
TF = 768
UNIT = 8
WOC = 256
WOP = 9
CHAIN_QK = True
CHAIN_PV = True
CHAIN_UNITS = 2
WO_P2 = 3
G_SPLIT = (256, 256)
U_SPLIT = (256, 256)
D_SPLIT = (512, 512)
PB = 4

_F32 = jnp.float32
_BF16 = jnp.bfloat16


def _splits(sizes):
    out, lo = [], 0
    for n in sizes:
        out.append((lo, lo + n))
        lo += n
    return out


def _dot(a, b):
    return jnp.dot(a, b, preferred_element_type=_F32)


def _kernel(x_hbm, wqkv_hbm, wo_hbm, wg_hbm, wu_hbm, wd_hbm, gw_hbm, out_hbm,
            x_v, wq_raw, wq_p, wo_raw, wo_f, wo_p, wg0, wu0, wd0, wg, wu, wd,
            acc, q_s, k_s, v_s, g_s, o_s, out_st, gw_ref,
            sems, sem_out,
            *, S, D, F):
    NR = S // TM
    NR0 = S // TM0
    NC = (F - F0) // TF
    NSL = 6
    HR = D // 2

    NWO = D // WOC
    pieces = ([(0, lo, hi) for lo, hi in _splits(G_SPLIT)]
              + [(1, lo, hi) for lo, hi in _splits(U_SPLIT)]
              + [(2, lo, hi) for lo, hi in _splits(D_SPLIT)])
    SX = 0
    SW0 = SX + NR0
    SG = SW0 + len(pieces)
    SQ = SG + 1
    SO = SQ + NSL
    SR = SO + NWO

    def x_copy(t):
        return pltpu.make_async_copy(
            x_hbm.at[pl.ds(t * TM0, TM0), :], x_v.at[pl.ds(t * TM0, TM0), :],
            sems.at[SX + t])

    def w0_copy(i):
        kind, lo, hi = pieces[i]
        cols = pl.ds(lo, hi - lo)
        src = (wg_hbm.at[:, cols], wu_hbm.at[:, cols],
               wd_hbm.at[pl.ds(0, F0), cols])[kind]
        dst = (wg0, wu0, wd0)[kind].at[:, cols]
        return pltpu.make_async_copy(src, dst, sems.at[SW0 + i])

    def gw_copy():
        return pltpu.make_async_copy(gw_hbm, gw_ref, sems.at[SG])

    def wq_copy(a):
        sec = a // 2
        half = a % 2
        return pltpu.make_async_copy(
            wqkv_hbm.at[pl.ds(half * HR, HR), pl.ds(sec * D, D)],
            wq_raw.at[a], sems.at[SQ + a])

    def wo_copy(n):
        lo = n * WOC
        if not isinstance(n, int):
            lo = pl.multiple_of(lo, LANES)
        return pltpu.make_async_copy(
            wo_hbm.at[:, pl.ds(lo, WOC)], wo_raw.at[n], sems.at[SO + n])

    def ffn_copies(c):
        lo = F0 + c * TF
        if not isinstance(c, int):
            lo = pl.multiple_of(lo, LANES)
        sem = sems.at[SR + c]
        return (
            pltpu.make_async_copy(wg_hbm.at[:, pl.ds(lo, TF)], wg.at[c], sem),
            pltpu.make_async_copy(wu_hbm.at[:, pl.ds(lo, TF)], wu.at[c], sem),
            pltpu.make_async_copy(wd_hbm.at[pl.ds(lo, TF), :], wd.at[c], sem),
        )

    def out_copy(r, n):
        return pltpu.make_async_copy(
            out_st[n].at[r],
            out_hbm.at[pl.ds(r * TM, TM), pl.ds(n * WOC, WOC)],
            sem_out.at[n])

    x_copy(0).start()
    for i in range(len(pieces)):
        w0_copy(i).start()
    for t in range(1, NR0):
        x_copy(t).start()
        if t - 1 < NSL:
            wq_copy(t - 1).start()
        if t >= NR0 - NWO:
            wo_copy(t - (NR0 - NWO)).start()
    gw_copy().start()
    for c in range(NC):
        for cp in ffn_copies(c):
            cp.start()

    zeros_halo = jnp.zeros((HALO, LANES), _F32)
    for j in range(NT):
        k_s[j, pl.ds(0, HALO), :] = zeros_halo
        v_s[j, pl.ds(0, HALO), :] = zeros_halo

    def permute_slice(a):
        rows = PB * 8
        lane = lax.broadcasted_iota(jnp.int32, (rows, LANES), 1)
        bits = [((lane >> (2 + b)) & 1) == 1 for b in range(3)]
        base_pat = NT * 4 * (lane & 3) + (lane >> 5) + 4 * ((lane >> 2) & 7)
        pats = [(base_pat + 4 * j) & (LANES - 1) for j in range(NT)]
        for g in range(HR // (16 * PB)):
            rs = pl.ds(g * 16 * PB, 16 * PB)
            z = []
            for i in range(NT):
                w = pltpu.bitcast(wq_raw[a, rs, pl.ds(i * LANES, LANES)],
                                  jnp.uint32)
                z.append(w if i == 0 else pltpu.roll(w, 4 * i, 1))
            for b in range(3):
                z = [jnp.where(bits[b], z[(k + (1 << b)) % NT], z[k])
                     for k in range(NT)]
            for j in range(NT):
                y = jnp.take_along_axis(z[(-j) % NT], pats[j], axis=1)
                wq_p[a, rs, pl.ds(j * LANES, LANES)] = pltpu.bitcast(y, _BF16)

    def permute_wo(n, never, pace1, pace2):
        nj = WOC // LANES
        i = 0
        for h in range(H):
            blk = wo_raw[n, pl.ds(h * DH, DH), :].astype(_F32)
            for a in range(DH // 8):
                for j in range(nj):
                    pc = blk[a * 8:(a + 1) * 8, j * LANES:(j + 1) * LANES]
                    pc = jnp.where(never, pace1[i], pc)
                    i += 1
                    wo_f[a * nj + j][pl.ds(h * WOP, 8), :] = pc
        i = 0
        for d in range(DH):
            for b in range(H // 8):
                rws = []
                for j in range(nj):
                    pc = wo_f[(d // 8) * nj + j][
                        pl.ds(b * 8 * WOP + d % 8, 8, stride=WOP), :]
                    pc = jnp.where(never, pace2[i], pc)
                    i += 1
                    rws.append(pc)
                wo_p[n, pl.ds(d * H + b * 8, 8), :] = jnp.concatenate(
                    rws, axis=1).astype(_BF16)

    def vregs(v):
        return [v[i * 8:(i + 1) * 8, n * LANES:(n + 1) * LANES]
                for n in range(v.shape[1] // LANES)
                for i in range(v.shape[0] // 8)]

    x_copy(0).wait()
    parts = ([], [])
    hh0 = None
    for i, (kind, lo, hi) in enumerate(pieces):
        w0_copy(i).wait()
        cols = pl.ds(lo, hi - lo)
        if kind < 2:
            parts[kind].append(
                _dot(x_v[pl.ds(0, TM0), :], (wg0, wu0)[kind][:, cols]))
        else:
            if hh0 is None:
                hh0 = (jnp.maximum(jnp.concatenate(parts[0], axis=1), 0.0)
                       * jnp.concatenate(parts[1], axis=1)).astype(_BF16)
            acc[pl.ds(0, TM0), cols] = _dot(hh0, wd0[:, cols])

    def phase0(t, carry):
        x_copy(t).wait()
        real = t <= NSL

        @pl.when(real)
        def _():
            wq_copy(t - 1).wait()

        real_o = t >= NR0 - NWO

        @pl.when(real_o)
        def _():
            wo_copy(t - (NR0 - NWO)).wait()

        rows = pl.ds(pl.multiple_of(t * TM0, TM0), TM0)
        xv = x_v[rows, :]
        gt = _dot(xv, wg0[...])
        up = _dot(xv, wu0[...])
        hh = (jnp.maximum(gt, 0.0) * up).astype(_BF16)
        dn = _dot(hh, wd0[...])
        acc[rows, :] = dn
        permute_slice(jnp.where(real, t - 1, NSL))
        never = lax.broadcasted_iota(jnp.int32, (8, LANES), 1) < -1 - t
        p2 = vregs(dn)
        p2 = [p2[i * WO_P2 // 4] for i in range(len(p2))]
        permute_wo(jnp.where(real_o, t - (NR0 - NWO), NWO), never,
                   vregs(gt) + vregs(up), p2)
        return carry

    lax.fori_loop(1, NR0, phase0, 0)
    gw_copy().wait()

    c_exp = (DH ** -0.5) * math.log2(math.e)
    neg = -1e9 / (DH ** -0.5)

    def attn_unit(r, row0, gw, never, link, masked):
        def tie(a, b):
            return a if b is None else jnp.where(never, b, a)

        base = r * TM + row0
        qs = [q_s[j, pl.ds(row0, UNIT), :] for j in range(NT)]
        logits = []
        for w in range(W):
            st = base + (HALO - DIL * w)
            q0 = tie(qs[0], link) if CHAIN_QK else qs[0]
            s = q0 * k_s[0, pl.ds(st, UNIT), :]
            for j in range(1, NT):
                s = s + qs[j] * k_s[j, pl.ds(st, UNIT), :]
            link = s
            s = s + pltpu.roll(s, 64, 1)
            s = s + pltpu.roll(s, 32, 1)
            if masked and w > 0:
                pos = base + lax.broadcasted_iota(jnp.int32, (UNIT, LANES), 0)
                s = jnp.where(pos >= DIL * w, s, neg)
            logits.append(s)
        m = logits[0]
        for w in range(1, W):
            m = jnp.maximum(m, logits[w])
        ps = [jnp.exp2((logits[w] - m) * c_exp) for w in range(W)]
        den = ps[0]
        for w in range(1, W):
            den = den + ps[w]
        xg = x_v[pl.ds(pl.multiple_of(base, UNIT), UNIT), :].astype(_F32) * gw
        gate = jax.nn.sigmoid(jnp.sum(xg, axis=-1, keepdims=True))
        gate = jnp.broadcast_to(gate, (UNIT, LANES))
        g_s[pl.ds(row0, UNIT), :] = 1.0 - gate
        rinv = gate / den
        olink = None
        for j in range(NT):
            p0 = tie(ps[0], olink) if CHAIN_PV else ps[0]
            o = p0 * v_s[j, pl.ds(base + HALO, UNIT), :]
            for w in range(1, W):
                o = o + ps[w] * v_s[j, pl.ds(base + (HALO - DIL * w), UNIT), :]
            olink = o
            o_s[pl.ds(row0, UNIT), pl.ds(j * LANES, LANES)] = (
                o * rinv).astype(_BF16)
        return olink if CHAIN_UNITS == 2 else (link if CHAIN_UNITS else None)

    def row_block(r, carry):
        rows = pl.ds(pl.multiple_of(r * TM, TM), TM)
        krows = pl.ds(pl.multiple_of(r * TM + HALO, HALO), TM)
        xv = x_v[rows, :]
        for sec, dst in enumerate((q_s, k_s, v_s)):
            wsec = wq_p[pl.ds(2 * sec, 2)].reshape(D, D)
            res = _dot(xv, wsec)
            for j in range(NT):
                piece = res[:, j * LANES:(j + 1) * LANES]
                if sec == 0:
                    dst[j] = piece
                else:
                    dst[j, krows, :] = piece
        AR = TM // NC

        def fa(c, carry2):
            @pl.when(r == 0)
            def _():
                for cp in ffn_copies(c):
                    cp.wait()

            gw = gw_ref[...].astype(_F32).reshape(1, D)
            nun = AR // UNIT

            never = lax.broadcasted_iota(jnp.int32, (UNIT, LANES), 1) < -1 - c
            link = None
            for un in range(nun):
                row0 = pl.multiple_of(c * AR + un * UNIT, UNIT)
                link = attn_unit(r, row0, gw, never, link,
                                 masked=(un * UNIT < HALO))
            xv2 = x_v[rows, :]
            gt = _dot(xv2, wg[c])
            up = _dot(xv2, wu[c])
            hh = (jnp.maximum(gt, 0.0) * up).astype(_BF16)
            acc[rows, :] += _dot(hh, wd[c])
            return carry2

        lax.fori_loop(0, NC, fa, 0)

        ov = o_s[...]
        g1 = g_s[...]
        g1 = jnp.concatenate([g1] * (WOC // LANES), axis=1)
        for n in range(NWO):
            cols = pl.ds(n * WOC, WOC)
            a = _dot(ov, wo_p[n])
            out_st[n][r] = (a + g1 * acc[rows, cols]).astype(_BF16)
            out_copy(r, n).start()
        return carry

    lax.fori_loop(0, NR, row_block, 0)
    for n in range(NWO):
        for r in range(NR):
            out_copy(r, n).wait()


@jax.jit
def pallas_gated_mix__sliding_local_dilated__glu_gated_reglu__prompt_kernel(
    A_x: jax.Array,
    A_wqkv: jax.Array,
    A_wo: jax.Array,
    B_x: jax.Array,
    B_W_gate: jax.Array,
    B_W_up: jax.Array,
    B_W_down: jax.Array,
    gate_w: jax.Array,
):
    del B_x
    B, S, D = A_x.shape
    F = B_W_gate.shape[1]
    assert B == 1 and D == H * DH == NT * LANES
    assert S % TM == 0 and (F - F0) % TF == 0
    NR = S // TM
    NC = (F - F0) // TF
    assert TM % (NC * UNIT) == 0 and S // TM0 >= 8

    n_sems = (S // TM0 + len(G_SPLIT) + len(U_SPLIT) + len(D_SPLIT) + 1 + 6
              + D // WOC + NC)
    any_spec = pl.BlockSpec(memory_space=pl.ANY)
    out = pl.pallas_call(
        functools.partial(_kernel, S=S, D=D, F=F),
        out_shape=jax.ShapeDtypeStruct((S, D), _BF16),
        in_specs=[any_spec] * 7,
        out_specs=any_spec,
        scratch_shapes=[
            pltpu.VMEM((S, D), _BF16),
            pltpu.VMEM((7, D // 2, D), _BF16),
            pltpu.VMEM((7, D // 2, D), _BF16),
            pltpu.VMEM((D // WOC + 1, D, WOC), _BF16),
            [pltpu.VMEM((H * WOP, LANES), _F32)] * (WOC // LANES * DH // 8),
            pltpu.VMEM((D // WOC + 1, D, WOC), _BF16),
            pltpu.VMEM((D, F0), _BF16),
            pltpu.VMEM((D, F0), _BF16),
            pltpu.VMEM((F0, D), _BF16),
            pltpu.VMEM((NC, D, TF), _BF16),
            pltpu.VMEM((NC, D, TF), _BF16),
            pltpu.VMEM((NC, TF, D), _BF16),
            pltpu.VMEM((S, D), _F32),
            pltpu.VMEM((NT, TM, LANES), _F32),
            pltpu.VMEM((NT, HALO + S, LANES), _F32),
            pltpu.VMEM((NT, HALO + S, LANES), _F32),
            pltpu.VMEM((TM, LANES), _F32),
            pltpu.VMEM((TM, D), _BF16),
            [pltpu.VMEM((NR, TM, WOC), _BF16)] * (D // WOC),
            pltpu.VMEM((D,), _BF16),
            pltpu.SemaphoreType.DMA((n_sems,)),
            pltpu.SemaphoreType.DMA((D // WOC,)),
        ],
        compiler_params=pltpu.CompilerParams(
            vmem_limit_bytes=120 * 1024 * 1024,
            disable_bounds_checks=True,
            disable_semaphore_checks=True),
        name="gated_mix",
    )(A_x.reshape(S, D), A_wqkv, A_wo, B_W_gate, B_W_up, B_W_down,
      gate_w)
    return out.reshape(B, S, D)
```

```python
import functools
import math

import jax
import jax.numpy as jnp
from jax import lax
import jax.experimental.pallas as pl
import jax.experimental.pallas.tpu as pltpu

H = 32
DH = 32
W = 8
DIL = 2
LANES = 128
NT = 8
HALO = 16

TM = 512
TM0 = 256
F0 = 512
TF = 768
UNIT = 8
WOC = 256
WOP = 9
CHAIN_QK = True
CHAIN_PV = True
CHAIN_UNITS = 2
WO_P2 = 3
G_SPLIT = (256, 256)
U_SPLIT = (256, 256)
D_SPLIT = (512, 512)
PB = 4

_F32 = jnp.float32
_BF16 = jnp.bfloat16


def _splits(sizes):
    out, lo = [], 0
    for n in sizes:
        out.append((lo, lo + n))
        lo += n
    return out


def _dot(a, b):
    return jnp.dot(a, b, preferred_element_type=_F32)


def _kernel(x_hbm, wqkv_hbm, wo_hbm, wg_hbm, wu_hbm, wd_hbm, gw_hbm, out_hbm,
            x_v, wq_raw, wq_p, wo_raw, wo_f, wo_p, wg0, wu0, wd0, wg, wu, wd,
            acc, q_s, k_s, v_s, g_s, o_s, out_st, gw_ref,
            sems, sem_out,
            *, S, D, F):
    NR = S // TM
    NR0 = S // TM0
    NC = (F - F0) // TF
    NSL = 6
    HR = D // 2

    NWO = D // WOC
    pieces = ([(0, lo, hi) for lo, hi in _splits(G_SPLIT)]
              + [(1, lo, hi) for lo, hi in _splits(U_SPLIT)]
              + [(2, lo, hi) for lo, hi in _splits(D_SPLIT)])
    SX = 0
    SW0 = SX + NR0
    SG = SW0 + len(pieces)
    SQ = SG + 1
    SO = SQ + NSL
    SR = SO + NWO

    def x_copy(t):
        return pltpu.make_async_copy(
            x_hbm.at[pl.ds(t * TM0, TM0), :], x_v.at[pl.ds(t * TM0, TM0), :],
            sems.at[SX + t])

    def w0_copy(i):
        kind, lo, hi = pieces[i]
        cols = pl.ds(lo, hi - lo)
        src = (wg_hbm.at[:, cols], wu_hbm.at[:, cols],
               wd_hbm.at[pl.ds(0, F0), cols])[kind]
        dst = (wg0, wu0, wd0)[kind].at[:, cols]
        return pltpu.make_async_copy(src, dst, sems.at[SW0 + i])

    def gw_copy():
        return pltpu.make_async_copy(gw_hbm, gw_ref, sems.at[SG])

    def wq_copy(a):
        sec = a // 2
        half = a % 2
        return pltpu.make_async_copy(
            wqkv_hbm.at[pl.ds(half * HR, HR), pl.ds(sec * D, D)],
            wq_raw.at[a], sems.at[SQ + a])

    def wo_copy(n):
        lo = n * WOC
        if not isinstance(n, int):
            lo = pl.multiple_of(lo, LANES)
        return pltpu.make_async_copy(
            wo_hbm.at[:, pl.ds(lo, WOC)], wo_raw.at[n], sems.at[SO + n])

    def ffn_copies(c):
        lo = F0 + c * TF
        if not isinstance(c, int):
            lo = pl.multiple_of(lo, LANES)
        sem = sems.at[SR + c]
        return (
            pltpu.make_async_copy(wg_hbm.at[:, pl.ds(lo, TF)], wg.at[c], sem),
            pltpu.make_async_copy(wu_hbm.at[:, pl.ds(lo, TF)], wu.at[c], sem),
            pltpu.make_async_copy(wd_hbm.at[pl.ds(lo, TF), :], wd.at[c], sem),
        )

    def out_copy(r, n):
        return pltpu.make_async_copy(
            out_st[n].at[r],
            out_hbm.at[pl.ds(r * TM, TM), pl.ds(n * WOC, WOC)],
            sem_out.at[n])

    x_copy(0).start()
    for i in range(len(pieces)):
        w0_copy(i).start()
    for t in range(1, NR0):
        x_copy(t).start()
        if t >= NR0 - NSL:
            wq_copy(t - (NR0 - NSL)).start()
        if t >= NR0 - NWO:
            wo_copy(t - (NR0 - NWO)).start()
    gw_copy().start()
    for c in range(NC):
        for cp in ffn_copies(c):
            cp.start()

    zeros_halo = jnp.zeros((HALO, LANES), _F32)
    for j in range(NT):
        k_s[j, pl.ds(0, HALO), :] = zeros_halo
        v_s[j, pl.ds(0, HALO), :] = zeros_halo

    def permute_slice(a):
        rows = PB * 8
        lane = lax.broadcasted_iota(jnp.int32, (rows, LANES), 1)
        bits = [((lane >> (2 + b)) & 1) == 1 for b in range(3)]
        base_pat = NT * 4 * (lane & 3) + (lane >> 5) + 4 * ((lane >> 2) & 7)
        pats = [(base_pat + 4 * j) & (LANES - 1) for j in range(NT)]
        for g in range(HR // (16 * PB)):
            rs = pl.ds(g * 16 * PB, 16 * PB)
            z = []
            for i in range(NT):
                w = pltpu.bitcast(wq_raw[a, rs, pl.ds(i * LANES, LANES)],
                                  jnp.uint32)
                z.append(w if i == 0 else pltpu.roll(w, 4 * i, 1))
            for b in range(3):
                z = [jnp.where(bits[b], z[(k + (1 << b)) % NT], z[k])
                     for k in range(NT)]
            for j in range(NT):
                y = jnp.take_along_axis(z[(-j) % NT], pats[j], axis=1)
                wq_p[a, rs, pl.ds(j * LANES, LANES)] = pltpu.bitcast(y, _BF16)

    def permute_wo(n, never, pace1, pace2):
        nj = WOC // LANES
        i = 0
        for h in range(H):
            blk = wo_raw[n, pl.ds(h * DH, DH), :].astype(_F32)
            for a in range(DH // 8):
                for j in range(nj):
                    pc = blk[a * 8:(a + 1) * 8, j * LANES:(j + 1) * LANES]
                    pc = jnp.where(never, pace1[i], pc)
                    i += 1
                    wo_f[a * nj + j][pl.ds(h * WOP, 8), :] = pc
        i = 0
        for d in range(DH):
            for b in range(H // 8):
                rws = []
                for j in range(nj):
                    pc = wo_f[(d // 8) * nj + j][
                        pl.ds(b * 8 * WOP + d % 8, 8, stride=WOP), :]
                    pc = jnp.where(never, pace2[i], pc)
                    i += 1
                    rws.append(pc)
                wo_p[n, pl.ds(d * H + b * 8, 8), :] = jnp.concatenate(
                    rws, axis=1).astype(_BF16)

    def vregs(v):
        return [v[i * 8:(i + 1) * 8, n * LANES:(n + 1) * LANES]
                for n in range(v.shape[1] // LANES)
                for i in range(v.shape[0] // 8)]

    x_copy(0).wait()
    parts = ([], [])
    hh0 = None
    for i, (kind, lo, hi) in enumerate(pieces):
        w0_copy(i).wait()
        cols = pl.ds(lo, hi - lo)
        if kind < 2:
            parts[kind].append(
                _dot(x_v[pl.ds(0, TM0), :], (wg0, wu0)[kind][:, cols]))
        else:
            if hh0 is None:
                hh0 = (jnp.maximum(jnp.concatenate(parts[0], axis=1), 0.0)
                       * jnp.concatenate(parts[1], axis=1)).astype(_BF16)
            acc[pl.ds(0, TM0), cols] = _dot(hh0, wd0[:, cols])

    def phase0(t, carry):
        x_copy(t).wait()
        real = t >= NR0 - NSL

        @pl.when(real)
        def _():
            wq_copy(t - (NR0 - NSL)).wait()

        real_o = t >= NR0 - NWO

        @pl.when(real_o)
        def _():
            wo_copy(t - (NR0 - NWO)).wait()

        rows = pl.ds(pl.multiple_of(t * TM0, TM0), TM0)
        xv = x_v[rows, :]
        gt = _dot(xv, wg0[...])
        up = _dot(xv, wu0[...])
        hh = (jnp.maximum(gt, 0.0) * up).astype(_BF16)
        dn = _dot(hh, wd0[...])
        acc[rows, :] = dn
        permute_slice(jnp.where(real, t - (NR0 - NSL), NSL))
        never = lax.broadcasted_iota(jnp.int32, (8, LANES), 1) < -1 - t
        p2 = vregs(dn)
        p2 = [p2[i * WO_P2 // 4] for i in range(len(p2))]
        permute_wo(jnp.where(real_o, t - (NR0 - NWO), NWO), never,
                   vregs(gt) + vregs(up), p2)
        return carry

    lax.fori_loop(1, NR0, phase0, 0)
    gw_copy().wait()

    c_exp = (DH ** -0.5) * math.log2(math.e)
    neg = -1e9 / (DH ** -0.5)

    def attn_unit(r, row0, gw, never, link, masked):
        def tie(a, b):
            return a if b is None else jnp.where(never, b, a)

        base = r * TM + row0
        qs = [q_s[j, pl.ds(row0, UNIT), :] for j in range(NT)]
        logits = []
        for w in range(W):
            st = base + (HALO - DIL * w)
            q0 = tie(qs[0], link) if CHAIN_QK else qs[0]
            s = q0 * k_s[0, pl.ds(st, UNIT), :]
            for j in range(1, NT):
                s = s + qs[j] * k_s[j, pl.ds(st, UNIT), :]
            link = s
            s = s + pltpu.roll(s, 64, 1)
            s = s + pltpu.roll(s, 32, 1)
            if masked and w > 0:
                pos = base + lax.broadcasted_iota(jnp.int32, (UNIT, LANES), 0)
                s = jnp.where(pos >= DIL * w, s, neg)
            logits.append(s)
        m = logits[0]
        for w in range(1, W):
            m = jnp.maximum(m, logits[w])
        ps = [jnp.exp2((logits[w] - m) * c_exp) for w in range(W)]
        den = ps[0]
        for w in range(1, W):
            den = den + ps[w]
        xg = x_v[pl.ds(pl.multiple_of(base, UNIT), UNIT), :].astype(_F32) * gw
        gate = jax.nn.sigmoid(jnp.sum(xg, axis=-1, keepdims=True))
        gate = jnp.broadcast_to(gate, (UNIT, LANES))
        g_s[pl.ds(row0, UNIT), :] = 1.0 - gate
        rinv = gate / den
        olink = None
        for j in range(NT):
            p0 = tie(ps[0], olink) if CHAIN_PV else ps[0]
            o = p0 * v_s[j, pl.ds(base + HALO, UNIT), :]
            for w in range(1, W):
                o = o + ps[w] * v_s[j, pl.ds(base + (HALO - DIL * w), UNIT), :]
            olink = o
            o_s[pl.ds(row0, UNIT), pl.ds(j * LANES, LANES)] = (
                o * rinv).astype(_BF16)
        return olink if CHAIN_UNITS == 2 else (link if CHAIN_UNITS else None)

    def row_block(r, carry):
        rows = pl.ds(pl.multiple_of(r * TM, TM), TM)
        krows = pl.ds(pl.multiple_of(r * TM + HALO, HALO), TM)
        xv = x_v[rows, :]
        for sec, dst in enumerate((q_s, k_s, v_s)):
            wsec = wq_p[pl.ds(2 * sec, 2)].reshape(D, D)
            res = _dot(xv, wsec)
            for j in range(NT):
                piece = res[:, j * LANES:(j + 1) * LANES]
                if sec == 0:
                    dst[j] = piece
                else:
                    dst[j, krows, :] = piece
        AR = TM // NC

        def fa(c, carry2):
            @pl.when(r == 0)
            def _():
                for cp in ffn_copies(c):
                    cp.wait()

            gw = gw_ref[...].astype(_F32).reshape(1, D)
            nun = AR // UNIT

            never = lax.broadcasted_iota(jnp.int32, (UNIT, LANES), 1) < -1 - c
            link = None
            for un in range(nun):
                row0 = pl.multiple_of(c * AR + un * UNIT, UNIT)
                link = attn_unit(r, row0, gw, never, link,
                                 masked=(un * UNIT < HALO))
            xv2 = x_v[rows, :]
            gt = _dot(xv2, wg[c])
            up = _dot(xv2, wu[c])
            hh = (jnp.maximum(gt, 0.0) * up).astype(_BF16)
            acc[rows, :] += _dot(hh, wd[c])
            return carry2

        lax.fori_loop(0, NC, fa, 0)

        ov = o_s[...]
        g1 = g_s[...]
        g1 = jnp.concatenate([g1] * (WOC // LANES), axis=1)
        for n in range(NWO):
            cols = pl.ds(n * WOC, WOC)
            a = _dot(ov, wo_p[n])
            out_st[n][r] = (a + g1 * acc[rows, cols]).astype(_BF16)
            out_copy(r, n).start()
        return carry

    lax.fori_loop(0, NR, row_block, 0)
    for n in range(NWO):
        for r in range(NR):
            out_copy(r, n).wait()


@jax.jit
def pallas_gated_mix__sliding_local_dilated__glu_gated_reglu__prompt_kernel(
    A_x: jax.Array,
    A_wqkv: jax.Array,
    A_wo: jax.Array,
    B_x: jax.Array,
    B_W_gate: jax.Array,
    B_W_up: jax.Array,
    B_W_down: jax.Array,
    gate_w: jax.Array,
):
    del B_x
    B, S, D = A_x.shape
    F = B_W_gate.shape[1]
    assert B == 1 and D == H * DH == NT * LANES
    assert S % TM == 0 and (F - F0) % TF == 0
    NR = S // TM
    NC = (F - F0) // TF
    assert TM % (NC * UNIT) == 0 and S // TM0 >= 8

    n_sems = (S // TM0 + len(G_SPLIT) + len(U_SPLIT) + len(D_SPLIT) + 1 + 6
              + D // WOC + NC)
    any_spec = pl.BlockSpec(memory_space=pl.ANY)
    out = pl.pallas_call(
        functools.partial(_kernel, S=S, D=D, F=F),
        out_shape=jax.ShapeDtypeStruct((S, D), _BF16),
        in_specs=[any_spec] * 7,
        out_specs=any_spec,
        scratch_shapes=[
            pltpu.VMEM((S, D), _BF16),
            pltpu.VMEM((7, D // 2, D), _BF16),
            pltpu.VMEM((7, D // 2, D), _BF16),
            pltpu.VMEM((D // WOC + 1, D, WOC), _BF16),
            [pltpu.VMEM((H * WOP, LANES), _F32)] * (WOC // LANES * DH // 8),
            pltpu.VMEM((D // WOC + 1, D, WOC), _BF16),
            pltpu.VMEM((D, F0), _BF16),
            pltpu.VMEM((D, F0), _BF16),
            pltpu.VMEM((F0, D), _BF16),
            pltpu.VMEM((NC, D, TF), _BF16),
            pltpu.VMEM((NC, D, TF), _BF16),
            pltpu.VMEM((NC, TF, D), _BF16),
            pltpu.VMEM((S, D), _F32),
            pltpu.VMEM((NT, TM, LANES), _F32),
            pltpu.VMEM((NT, HALO + S, LANES), _F32),
            pltpu.VMEM((NT, HALO + S, LANES), _F32),
            pltpu.VMEM((TM, LANES), _F32),
            pltpu.VMEM((TM, D), _BF16),
            [pltpu.VMEM((NR, TM, WOC), _BF16)] * (D // WOC),
            pltpu.VMEM((D,), _BF16),
            pltpu.SemaphoreType.DMA((n_sems,)),
            pltpu.SemaphoreType.DMA((D // WOC,)),
        ],
        compiler_params=pltpu.CompilerParams(
            vmem_limit_bytes=120 * 1024 * 1024,
            disable_bounds_checks=True,
            disable_semaphore_checks=True),
        name="gated_mix",
    )(A_x.reshape(S, D), A_wqkv, A_wo, B_W_gate, B_W_up, B_W_down,
      gate_w)
    return out.reshape(B, S, D)
```

```python
import functools
import math

import jax
import jax.numpy as jnp
from jax import lax
import jax.experimental.pallas as pl
import jax.experimental.pallas.tpu as pltpu

H = 32
DH = 32
W = 8
DIL = 2
LANES = 128
NT = 8
HALO = 16

TM = 512
TM0 = 256
F0 = 512
TF = 1024
UNIT = 8
WOC = 256
WOP = 9
CHAIN_QK = True
CHAIN_PV = True
CHAIN_UNITS = 2
WO_P2 = 3
PAD = 128
GATE_TIE = 1
NCHAIN = 1
G_SPLIT = (256, 256)
U_SPLIT = (256, 256)
D_SPLIT = (512, 512)
PB = 4

_F32 = jnp.float32
_BF16 = jnp.bfloat16


def _splits(sizes):
    out, lo = [], 0
    for n in sizes:
        out.append((lo, lo + n))
        lo += n
    return out


def _dot(a, b):
    return jnp.dot(a, b, preferred_element_type=_F32)


def _kernel(x_hbm, wqkv_hbm, wo_hbm, wg_hbm, wu_hbm, wd_hbm, gw_hbm, out_hbm,
            x_v, wq_raw, wq_p, wo_raw, wo_f, wo_p, wg0, wu0, wd0, wg, wu, wd,
            acc, q_s, k_s, v_s, g_s, o_s, out_st, gw_ref,
            sems, sem_out,
            *, S, D, F):
    NR = S // TM
    NR0 = S // TM0
    NC = (F - F0) // TF
    NSL = 6
    HR = D // 2

    NWO = D // WOC
    pieces = ([(0, lo, hi) for lo, hi in _splits(G_SPLIT)]
              + [(1, lo, hi) for lo, hi in _splits(U_SPLIT)]
              + [(2, lo, hi) for lo, hi in _splits(D_SPLIT)])
    SX = 0
    SW0 = SX + NR0
    SG = SW0 + len(pieces)
    SQ = SG + 1
    SO = SQ + NSL
    SR = SO + NWO

    def x_copy(t):
        return pltpu.make_async_copy(
            x_hbm.at[pl.ds(t * TM0, TM0), :], x_v.at[pl.ds(t * TM0, TM0), :],
            sems.at[SX + t])

    def w0_copy(i):
        kind, lo, hi = pieces[i]
        cols = pl.ds(lo, hi - lo)
        src = (wg_hbm.at[:, cols], wu_hbm.at[:, cols],
               wd_hbm.at[pl.ds(0, F0), cols])[kind]
        dst = (wg0, wu0, wd0)[kind].at[:, cols]
        return pltpu.make_async_copy(src, dst, sems.at[SW0 + i])

    def gw_copy():
        return pltpu.make_async_copy(gw_hbm, gw_ref, sems.at[SG])

    def wq_copy(a):
        sec = a // 2
        half = a % 2
        return pltpu.make_async_copy(
            wqkv_hbm.at[pl.ds(half * HR, HR), pl.ds(sec * D, D)],
            wq_raw.at[a], sems.at[SQ + a])

    def wo_copy(n):
        lo = n * WOC
        if not isinstance(n, int):
            lo = pl.multiple_of(lo, LANES)
        return pltpu.make_async_copy(
            wo_hbm.at[:, pl.ds(lo, WOC)], wo_raw.at[n], sems.at[SO + n])

    def ffn_copies(c):
        lo = F0 + c * TF
        if not isinstance(c, int):
            lo = pl.multiple_of(lo, LANES)
        sem = sems.at[SR + c]
        return (
            pltpu.make_async_copy(wg_hbm.at[:, pl.ds(lo, TF)],
                                  wg.at[c, :, pl.ds(0, TF)], sem),
            pltpu.make_async_copy(wu_hbm.at[:, pl.ds(lo, TF)], wu.at[c], sem),
            pltpu.make_async_copy(wd_hbm.at[pl.ds(lo, TF), :], wd.at[c], sem),
        )

    def out_copy(r, n):
        return pltpu.make_async_copy(
            out_st[n].at[r],
            out_hbm.at[pl.ds(r * TM, TM), pl.ds(n * WOC, WOC)],
            sem_out.at[n])

    x_copy(0).start()
    for i in range(len(pieces)):
        w0_copy(i).start()
    for t in range(1, NR0):
        x_copy(t).start()
        if t >= NR0 - NSL:
            wq_copy(t - (NR0 - NSL)).start()
        if t >= NR0 - NWO:
            wo_copy(t - (NR0 - NWO)).start()
    gw_copy().start()
    for c in range(NC):
        for cp in ffn_copies(c):
            cp.start()

    zeros_halo = jnp.zeros((HALO, LANES), _F32)
    for j in range(NT):
        k_s[j, pl.ds(0, HALO), :] = zeros_halo
        v_s[j, pl.ds(0, HALO), :] = zeros_halo

    def permute_slice(a):
        rows = PB * 8
        lane = lax.broadcasted_iota(jnp.int32, (rows, LANES), 1)
        bits = [((lane >> (2 + b)) & 1) == 1 for b in range(3)]
        base_pat = NT * 4 * (lane & 3) + (lane >> 5) + 4 * ((lane >> 2) & 7)
        pats = [(base_pat + 4 * j) & (LANES - 1) for j in range(NT)]
        for g in range(HR // (16 * PB)):
            rs = pl.ds(g * 16 * PB, 16 * PB)
            z = []
            for i in range(NT):
                w = pltpu.bitcast(wq_raw[a, rs, pl.ds(i * LANES, LANES)],
                                  jnp.uint32)
                z.append(w if i == 0 else pltpu.roll(w, 4 * i, 1))
            for b in range(3):
                z = [jnp.where(bits[b], z[(k + (1 << b)) % NT], z[k])
                     for k in range(NT)]
            for j in range(NT):
                y = jnp.take_along_axis(z[(-j) % NT], pats[j], axis=1)
                wq_p[a, rs, pl.ds(j * LANES, LANES)] = pltpu.bitcast(y, _BF16)

    def permute_wo(n, never, pace1, pace2):
        nj = WOC // LANES
        i = 0
        for h in range(H):
            blk = wo_raw[n, pl.ds(h * DH, DH), :].astype(_F32)
            for a in range(DH // 8):
                for j in range(nj):
                    pc = blk[a * 8:(a + 1) * 8, j * LANES:(j + 1) * LANES]
                    pc = jnp.where(never, pace1[i], pc)
                    i += 1
                    wo_f[a * nj + j][pl.ds(h * WOP, 8), :] = pc
        i = 0
        for d in range(DH):
            for b in range(H // 8):
                rws = []
                for j in range(nj):
                    pc = wo_f[(d // 8) * nj + j][
                        pl.ds(b * 8 * WOP + d % 8, 8, stride=WOP), :]
                    pc = jnp.where(never, pace2[i], pc)
                    i += 1
                    rws.append(pc)
                wo_p[n, pl.ds(d * H + b * 8, 8), :] = jnp.concatenate(
                    rws, axis=1).astype(_BF16)

    def vregs(v):
        return [v[i * 8:(i + 1) * 8, n * LANES:(n + 1) * LANES]
                for n in range(v.shape[1] // LANES)
                for i in range(v.shape[0] // 8)]

    x_copy(0).wait()
    parts = ([], [])
    hh0 = None
    for i, (kind, lo, hi) in enumerate(pieces):
        w0_copy(i).wait()
        cols = pl.ds(lo, hi - lo)
        if kind < 2:
            parts[kind].append(
                _dot(x_v[pl.ds(0, TM0), :], (wg0, wu0)[kind][:, cols]))
        else:
            if hh0 is None:
                hh0 = (jnp.maximum(jnp.concatenate(parts[0], axis=1), 0.0)
                       * jnp.concatenate(parts[1], axis=1)).astype(_BF16)
            acc[pl.ds(0, TM0), cols] = _dot(hh0, wd0[:, cols])

    def phase0(t, carry):
        x_copy(t).wait()
        real = t >= NR0 - NSL

        @pl.when(real)
        def _():
            wq_copy(t - (NR0 - NSL)).wait()

        real_o = t >= NR0 - NWO

        @pl.when(real_o)
        def _():
            wo_copy(t - (NR0 - NWO)).wait()

        rows = pl.ds(pl.multiple_of(t * TM0, TM0), TM0)
        xv = x_v[rows, :]
        gt = _dot(xv, wg0[:, pl.ds(0, F0)])
        up = _dot(xv, wu0[...])
        hh = (jnp.maximum(gt, 0.0) * up).astype(_BF16)
        dn = _dot(hh, wd0[...])
        acc[rows, :] = dn
        permute_slice(jnp.where(real, t - (NR0 - NSL), NSL))
        never = lax.broadcasted_iota(jnp.int32, (8, LANES), 1) < -1 - t
        p2 = vregs(dn)
        p2 = [p2[i * WO_P2 // 4] for i in range(len(p2))]
        permute_wo(jnp.where(real_o, t - (NR0 - NWO), NWO), never,
                   vregs(gt) + vregs(up), p2)
        return carry

    lax.fori_loop(1, NR0, phase0, 0)
    gw_copy().wait()

    c_exp = (DH ** -0.5) * math.log2(math.e)
    neg = -1e9 / (DH ** -0.5)

    def attn_unit(r, row0, gw, never, link, masked):
        def tie(a, b):
            return a if b is None else jnp.where(never, b, a)

        base = r * TM + row0
        qs = [q_s[j, pl.ds(row0, UNIT), :] for j in range(NT)]
        xr = x_v[pl.ds(pl.multiple_of(base, UNIT), UNIT), :].astype(_F32)
        xg = (tie(xr[:, 0:LANES], link) if GATE_TIE == 2 else xr[:, 0:LANES]) * gw[:, 0:LANES]
        for j in range(1, NT):
            cols = slice(j * LANES, (j + 1) * LANES)
            xg = xg + xr[:, cols] * gw[:, cols]
        logits = []
        for w in range(W):
            st = base + (HALO - DIL * w)
            q0 = tie(qs[0], link) if CHAIN_QK else qs[0]
            s = q0 * k_s[0, pl.ds(st, UNIT), :]
            for j in range(1, NT):
                s = s + qs[j] * k_s[j, pl.ds(st, UNIT), :]
            link = s
            s = s + pltpu.roll(s, 64, 1)
            s = s + pltpu.roll(s, 32, 1)
            if masked and w > 0:
                pos = base + lax.broadcasted_iota(jnp.int32, (UNIT, LANES), 0)
                s = jnp.where(pos >= DIL * w, s, neg)
            logits.append(s)
        m = logits[0]
        for w in range(1, W):
            m = jnp.maximum(m, logits[w])
        ps = [jnp.exp2((logits[w] - m) * c_exp) for w in range(W)]
        den = ps[0]
        for w in range(1, W):
            den = den + ps[w]
        gate = jax.nn.sigmoid(jnp.sum(xg, axis=-1, keepdims=True))
        gate = jnp.broadcast_to(gate, (UNIT, LANES))
        g_s[pl.ds(row0, UNIT), :] = 1.0 - gate
        rinv = gate / den
        olink = gate if GATE_TIE else None
        for j in range(NT):
            p0 = tie(ps[0], olink) if CHAIN_PV else ps[0]
            o = p0 * v_s[j, pl.ds(base + HALO, UNIT), :]
            for w in range(1, W):
                o = o + ps[w] * v_s[j, pl.ds(base + (HALO - DIL * w), UNIT), :]
            olink = o
            o_s[pl.ds(row0, UNIT), pl.ds(j * LANES, LANES)] = (
                (o * rinv).astype(_BF16))
        return olink if CHAIN_UNITS == 2 else (link if CHAIN_UNITS else None)

    def row_block(r, carry):
        rows = pl.ds(pl.multiple_of(r * TM, TM), TM)
        krows = pl.ds(pl.multiple_of(r * TM + HALO, HALO), TM)
        xv = x_v[rows, :]
        for sec, dst in enumerate((q_s, k_s, v_s)):
            wsec = wq_p[pl.ds(2 * sec, 2), :, pl.ds(0, D)].reshape(D, D)
            res = _dot(xv, wsec)
            for j in range(NT):
                piece = res[:, j * LANES:(j + 1) * LANES]
                if sec == 0:
                    dst[j] = piece
                else:
                    dst[j, krows, :] = piece
        AS = (TM // NC) // 32 * 32
        AR = TM - (NC - 1) * AS

        def fa(c, carry2):
            @pl.when(r == 0)
            def _():
                for cp in ffn_copies(c):
                    cp.wait()

            gw = gw_ref[...].astype(_F32).reshape(1, D)
            nun = AR // UNIT

            never = lax.broadcasted_iota(jnp.int32, (UNIT, LANES), 1) < -1 - c
            links = [None] * NCHAIN
            for un in range(nun):
                row0 = pl.multiple_of(c * AS + un * UNIT, UNIT)
                links[un % NCHAIN] = attn_unit(
                    r, row0, gw, never, links[un % NCHAIN],
                    masked=(un * UNIT < HALO))
            xv2 = x_v[rows, :]
            gt = _dot(xv2, wg[c, :, pl.ds(0, TF)])
            up = _dot(xv2, wu[c])
            hh = (jnp.maximum(gt, 0.0) * up).astype(_BF16)
            acc[rows, :] += _dot(hh, wd[c])
            return carry2

        lax.fori_loop(0, NC, fa, 0)

        ov = o_s[...]
        g1 = g_s[...]
        g1 = jnp.concatenate([g1] * (WOC // LANES), axis=1)
        for n in range(NWO):
            cols = pl.ds(n * WOC, WOC)
            a = _dot(ov, wo_p[n])
            out_st[n][r] = (a + g1 * acc[rows, cols]).astype(_BF16)
            out_copy(r, n).start()
        return carry

    lax.fori_loop(0, NR, row_block, 0)
    for n in range(NWO):
        for r in range(NR):
            out_copy(r, n).wait()


@jax.jit
def pallas_gated_mix__sliding_local_dilated__glu_gated_reglu__prompt_kernel(
    A_x: jax.Array,
    A_wqkv: jax.Array,
    A_wo: jax.Array,
    B_x: jax.Array,
    B_W_gate: jax.Array,
    B_W_up: jax.Array,
    B_W_down: jax.Array,
    gate_w: jax.Array,
):
    del B_x
    B, S, D = A_x.shape
    F = B_W_gate.shape[1]
    assert B == 1 and D == H * DH == NT * LANES
    assert S % TM == 0 and (F - F0) % TF == 0
    NR = S // TM
    NC = (F - F0) // TF
    assert S // TM0 >= 8

    n_sems = (S // TM0 + len(G_SPLIT) + len(U_SPLIT) + len(D_SPLIT) + 1 + 6
              + D // WOC + NC)
    any_spec = pl.BlockSpec(memory_space=pl.ANY)
    out = pl.pallas_call(
        functools.partial(_kernel, S=S, D=D, F=F),
        out_shape=jax.ShapeDtypeStruct((S, D), _BF16),
        in_specs=[any_spec] * 7,
        out_specs=any_spec,
        scratch_shapes=[
            pltpu.VMEM((S, D), _BF16),
            pltpu.VMEM((7, D // 2, D), _BF16),
            pltpu.VMEM((7, D // 2, D + PAD), _BF16),
            pltpu.VMEM((D // WOC + 1, D, WOC), _BF16),
            [pltpu.VMEM((H * WOP, LANES), _F32)] * (WOC // LANES * DH // 8),
            pltpu.VMEM((D // WOC + 1, D, WOC), _BF16),
            pltpu.VMEM((D, F0 + PAD), _BF16),
            pltpu.VMEM((D, F0), _BF16),
            pltpu.VMEM((F0, D), _BF16),
            pltpu.VMEM((NC, D, TF + PAD), _BF16),
            pltpu.VMEM((NC, D, TF), _BF16),
            pltpu.VMEM((NC, TF, D), _BF16),
            pltpu.VMEM((S, D), _F32),
            pltpu.VMEM((NT, TM, LANES), _F32),
            pltpu.VMEM((NT, HALO + S, LANES), _F32),
            pltpu.VMEM((NT, HALO + S, LANES), _F32),
            pltpu.VMEM((TM, LANES), _F32),
            pltpu.VMEM((TM, D), _BF16),
            [pltpu.VMEM((NR, TM, WOC), _BF16)] * (D // WOC),
            pltpu.VMEM((D,), _BF16),
            pltpu.SemaphoreType.DMA((n_sems,)),
            pltpu.SemaphoreType.DMA((D // WOC,)),
        ],
        compiler_params=pltpu.CompilerParams(
            vmem_limit_bytes=120 * 1024 * 1024,
            disable_bounds_checks=True,
            disable_semaphore_checks=True),
        name="gated_mix",
    )(A_x.reshape(S, D), A_wqkv, A_wo, B_W_gate, B_W_up, B_W_down,
      gate_w)
    return out.reshape(B, S, D)
```

```python
import functools
import math

import jax
import jax.numpy as jnp
from jax import lax
import jax.experimental.pallas as pl
import jax.experimental.pallas.tpu as pltpu

H = 32
DH = 32
W = 8
DIL = 2
LANES = 128
NT = 8
HALO = 16

TM = 512
TM0 = 256
F0 = 512
TF = 1024
UNIT = 8
WOC = 256
WOP = 9
CHAIN_QK = True
CHAIN_PV = True
CHAIN_UNITS = 2
WO_P2 = 3
PADX = 0
PADW = 0
PAD = 128
GATE_TIE = 1
NCHAIN = 1
G_SPLIT = (256, 256)
U_SPLIT = (256, 256)
D_SPLIT = (512, 512)
PB = 4

_F32 = jnp.float32
_BF16 = jnp.bfloat16


def _splits(sizes):
    out, lo = [], 0
    for n in sizes:
        out.append((lo, lo + n))
        lo += n
    return out


def _dot(a, b):
    return jnp.dot(a, b, preferred_element_type=_F32)


def _kernel(x_hbm, wqkv_hbm, wo_hbm, wg_hbm, wu_hbm, wd_hbm, gw_hbm, out_hbm,
            x_v, wq_raw, wq_p, wo_raw, wo_f, wo_p, wg0, wu0, wd0, wg, wu, wd,
            acc, q_s, k_s, v_s, g_s, o_s, out_st, gw_ref,
            sems, sem_out,
            *, S, D, F):
    NR = S // TM
    NR0 = S // TM0
    NC = (F - F0) // TF
    NSL = 6
    HR = D // 2

    dc = pl.ds(0, D)

    NWO = D // WOC
    pieces = ([(0, lo, hi) for lo, hi in _splits(G_SPLIT)]
              + [(1, lo, hi) for lo, hi in _splits(U_SPLIT)]
              + [(2, lo, hi) for lo, hi in _splits(D_SPLIT)])
    SX = 0
    SW0 = SX + NR0
    SG = SW0 + len(pieces)
    SQ = SG + 1
    SO = SQ + NSL
    SR = SO + NWO

    def x_copy(t):
        return pltpu.make_async_copy(
            x_hbm.at[pl.ds(t * TM0, TM0), :], x_v.at[pl.ds(t * TM0, TM0), dc],
            sems.at[SX + t])

    def w0_copy(i):
        kind, lo, hi = pieces[i]
        cols = pl.ds(lo, hi - lo)
        src = (wg_hbm.at[:, cols], wu_hbm.at[:, cols],
               wd_hbm.at[pl.ds(0, F0), cols])[kind]
        dst = (wg0, wu0, wd0)[kind].at[:, cols]
        return pltpu.make_async_copy(src, dst, sems.at[SW0 + i])

    def gw_copy():
        return pltpu.make_async_copy(gw_hbm, gw_ref, sems.at[SG])

    def wq_copy(a):
        sec = a // 2
        half = a % 2
        return pltpu.make_async_copy(
            wqkv_hbm.at[pl.ds(half * HR, HR), pl.ds(sec * D, D)],
            wq_raw.at[a, :, dc], sems.at[SQ + a])

    def wo_copy(n):
        lo = n * WOC
        if not isinstance(n, int):
            lo = pl.multiple_of(lo, LANES)
        return pltpu.make_async_copy(
            wo_hbm.at[:, pl.ds(lo, WOC)], wo_raw.at[n], sems.at[SO + n])

    def ffn_copies(c):
        lo = F0 + c * TF
        if not isinstance(c, int):
            lo = pl.multiple_of(lo, LANES)
        sem = sems.at[SR + c]
        return (
            pltpu.make_async_copy(wg_hbm.at[:, pl.ds(lo, TF)],
                                  wg.at[c, :, pl.ds(0, TF)], sem),
            pltpu.make_async_copy(wu_hbm.at[:, pl.ds(lo, TF)],
                                  wu.at[c, :, pl.ds(0, TF)], sem),
            pltpu.make_async_copy(wd_hbm.at[pl.ds(lo, TF), :],
                                  wd.at[c, :, dc], sem),
        )

    def out_copy(r, n):
        return pltpu.make_async_copy(
            out_st[n].at[r],
            out_hbm.at[pl.ds(r * TM, TM), pl.ds(n * WOC, WOC)],
            sem_out.at[n])

    x_copy(0).start()
    for i in range(len(pieces)):
        w0_copy(i).start()
    for t in range(1, NR0):
        x_copy(t).start()
        if t >= NR0 - NSL:
            wq_copy(t - (NR0 - NSL)).start()
        if t >= NR0 - NWO:
            wo_copy(t - (NR0 - NWO)).start()
    gw_copy().start()
    for c in range(NC):
        for cp in ffn_copies(c):
            cp.start()

    zeros_halo = jnp.zeros((HALO, LANES), _F32)
    for j in range(NT):
        k_s[j, pl.ds(0, HALO), :] = zeros_halo
        v_s[j, pl.ds(0, HALO), :] = zeros_halo

    def permute_slice(a):
        rows = PB * 8
        lane = lax.broadcasted_iota(jnp.int32, (rows, LANES), 1)
        bits = [((lane >> (2 + b)) & 1) == 1 for b in range(3)]
        base_pat = NT * 4 * (lane & 3) + (lane >> 5) + 4 * ((lane >> 2) & 7)
        pats = [(base_pat + 4 * j) & (LANES - 1) for j in range(NT)]
        for g in range(HR // (16 * PB)):
            rs = pl.ds(g * 16 * PB, 16 * PB)
            z = []
            for i in range(NT):
                w = pltpu.bitcast(wq_raw[a, rs, pl.ds(i * LANES, LANES)],
                                  jnp.uint32)
                z.append(w if i == 0 else pltpu.roll(w, 4 * i, 1))
            for b in range(3):
                z = [jnp.where(bits[b], z[(k + (1 << b)) % NT], z[k])
                     for k in range(NT)]
            for j in range(NT):
                y = jnp.take_along_axis(z[(-j) % NT], pats[j], axis=1)
                wq_p[a, rs, pl.ds(j * LANES, LANES)] = pltpu.bitcast(y, _BF16)

    def permute_wo(n, never, pace1, pace2):
        nj = WOC // LANES
        i = 0
        for h in range(H):
            blk = wo_raw[n, pl.ds(h * DH, DH), :].astype(_F32)
            for a in range(DH // 8):
                for j in range(nj):
                    pc = blk[a * 8:(a + 1) * 8, j * LANES:(j + 1) * LANES]
                    pc = jnp.where(never, pace1[i], pc)
                    i += 1
                    wo_f[a * nj + j][pl.ds(h * WOP, 8), :] = pc
        i = 0
        for d in range(DH):
            for b in range(H // 8):
                rws = []
                for j in range(nj):
                    pc = wo_f[(d // 8) * nj + j][
                        pl.ds(b * 8 * WOP + d % 8, 8, stride=WOP), :]
                    pc = jnp.where(never, pace2[i], pc)
                    i += 1
                    rws.append(pc)
                wo_p[n, pl.ds(d * H + b * 8, 8), :] = jnp.concatenate(
                    rws, axis=1).astype(_BF16)

    def vregs(v):
        return [v[i * 8:(i + 1) * 8, n * LANES:(n + 1) * LANES]
                for n in range(v.shape[1] // LANES)
                for i in range(v.shape[0] // 8)]

    x_copy(0).wait()
    parts = ([], [])
    hh0 = None
    for i, (kind, lo, hi) in enumerate(pieces):
        w0_copy(i).wait()
        cols = pl.ds(lo, hi - lo)
        if kind < 2:
            parts[kind].append(
                _dot(x_v[pl.ds(0, TM0), dc], (wg0, wu0)[kind][:, cols]))
        else:
            if hh0 is None:
                hh0 = (jnp.maximum(jnp.concatenate(parts[0], axis=1), 0.0)
                       * jnp.concatenate(parts[1], axis=1)).astype(_BF16)
            acc[pl.ds(0, TM0), cols] = _dot(hh0, wd0[:, cols])

    def phase0(t, carry):
        x_copy(t).wait()
        real = t >= NR0 - NSL

        @pl.when(real)
        def _():
            wq_copy(t - (NR0 - NSL)).wait()

        real_o = t >= NR0 - NWO

        @pl.when(real_o)
        def _():
            wo_copy(t - (NR0 - NWO)).wait()

        rows = pl.ds(pl.multiple_of(t * TM0, TM0), TM0)
        xv = x_v[rows, dc]
        gt = _dot(xv, wg0[:, pl.ds(0, F0)])
        up = _dot(xv, wu0[:, pl.ds(0, F0)])
        hh = (jnp.maximum(gt, 0.0) * up).astype(_BF16)
        dn = _dot(hh, wd0[:, dc])
        acc[rows, :] = dn
        permute_slice(jnp.where(real, t - (NR0 - NSL), NSL))
        never = lax.broadcasted_iota(jnp.int32, (8, LANES), 1) < -1 - t
        p2 = vregs(dn)
        p2 = [p2[i * WO_P2 // 4] for i in range(len(p2))]
        permute_wo(jnp.where(real_o, t - (NR0 - NWO), NWO), never,
                   vregs(gt) + vregs(up), p2)
        return carry

    lax.fori_loop(1, NR0, phase0, 0)
    gw_copy().wait()

    c_exp = (DH ** -0.5) * math.log2(math.e)
    neg = -1e9 / (DH ** -0.5)

    def attn_unit(r, row0, gw, never, link, masked):
        def tie(a, b):
            return a if b is None else jnp.where(never, b, a)

        base = r * TM + row0
        qs = [q_s[j, pl.ds(row0, UNIT), :] for j in range(NT)]
        xr = x_v[pl.ds(pl.multiple_of(base, UNIT), UNIT), dc].astype(_F32)
        xg = (tie(xr[:, 0:LANES], link) if GATE_TIE == 2 else xr[:, 0:LANES]) * gw[:, 0:LANES]
        for j in range(1, NT):
            cols = slice(j * LANES, (j + 1) * LANES)
            xg = xg + xr[:, cols] * gw[:, cols]
        logits = []
        for w in range(W):
            st = base + (HALO - DIL * w)
            q0 = tie(qs[0], link) if CHAIN_QK else qs[0]
            s = q0 * k_s[0, pl.ds(st, UNIT), :]
            for j in range(1, NT):
                s = s + qs[j] * k_s[j, pl.ds(st, UNIT), :]
            link = s
            s = s + pltpu.roll(s, 64, 1)
            s = s + pltpu.roll(s, 32, 1)
            if masked and w > 0:
                pos = base + lax.broadcasted_iota(jnp.int32, (UNIT, LANES), 0)
                s = jnp.where(pos >= DIL * w, s, neg)
            logits.append(s)
        m = logits[0]
        for w in range(1, W):
            m = jnp.maximum(m, logits[w])
        ps = [jnp.exp2((logits[w] - m) * c_exp) for w in range(W)]
        den = ps[0]
        for w in range(1, W):
            den = den + ps[w]
        gate = jax.nn.sigmoid(jnp.sum(xg, axis=-1, keepdims=True))
        gate = jnp.broadcast_to(gate, (UNIT, LANES))
        g_s[pl.ds(row0, UNIT), :] = 1.0 - gate
        rinv = gate / den
        olink = gate if GATE_TIE else None
        for j in range(NT):
            p0 = tie(ps[0], olink) if CHAIN_PV else ps[0]
            o = p0 * v_s[j, pl.ds(base + HALO, UNIT), :]
            for w in range(1, W):
                o = o + ps[w] * v_s[j, pl.ds(base + (HALO - DIL * w), UNIT), :]
            olink = o
            o_s[pl.ds(row0, UNIT), pl.ds(j * LANES, LANES)] = (
                (o * rinv).astype(_BF16))
        return olink if CHAIN_UNITS == 2 else (link if CHAIN_UNITS else None)

    def row_block(r, carry):
        rows = pl.ds(pl.multiple_of(r * TM, TM), TM)
        krows = pl.ds(pl.multiple_of(r * TM + HALO, HALO), TM)
        xv = x_v[rows, dc]
        for sec, dst in enumerate((q_s, k_s, v_s)):
            wsec = wq_p[pl.ds(2 * sec, 2), :, pl.ds(0, D)].reshape(D, D)
            res = _dot(xv, wsec)
            for j in range(NT):
                piece = res[:, j * LANES:(j + 1) * LANES]
                if sec == 0:
                    dst[j] = piece
                else:
                    dst[j, krows, :] = piece
        AS = (TM // NC) // 32 * 32
        AR = TM - (NC - 1) * AS

        def fa(c, carry2):
            @pl.when(r == 0)
            def _():
                for cp in ffn_copies(c):
                    cp.wait()

            gw = gw_ref[...].astype(_F32).reshape(1, D)
            nun = AR // UNIT

            never = lax.broadcasted_iota(jnp.int32, (UNIT, LANES), 1) < -1 - c
            links = [None] * NCHAIN
            for un in range(nun):
                row0 = pl.multiple_of(c * AS + un * UNIT, UNIT)
                links[un % NCHAIN] = attn_unit(
                    r, row0, gw, never, links[un % NCHAIN],
                    masked=(un * UNIT < HALO))
            xv2 = x_v[rows, dc]
            gt = _dot(xv2, wg[c, :, pl.ds(0, TF)])
            up = _dot(xv2, wu[c, :, pl.ds(0, TF)])
            hh = (jnp.maximum(gt, 0.0) * up).astype(_BF16)
            acc[rows, :] += _dot(hh, wd[c, :, dc])
            return carry2

        lax.fori_loop(0, NC, fa, 0)

        ov = o_s[:, dc]
        g1 = g_s[...]
        g1 = jnp.concatenate([g1] * (WOC // LANES), axis=1)
        for n in range(NWO):
            cols = pl.ds(n * WOC, WOC)
            a = _dot(ov, wo_p[n])
            out_st[n][r] = (a + g1 * acc[rows, cols]).astype(_BF16)
            out_copy(r, n).start()
        return carry

    lax.fori_loop(0, NR, row_block, 0)
    for n in range(NWO):
        for r in range(NR):
            out_copy(r, n).wait()


@jax.jit
def pallas_gated_mix__sliding_local_dilated__glu_gated_reglu__prompt_kernel(
    A_x: jax.Array,
    A_wqkv: jax.Array,
    A_wo: jax.Array,
    B_x: jax.Array,
    B_W_gate: jax.Array,
    B_W_up: jax.Array,
    B_W_down: jax.Array,
    gate_w: jax.Array,
):
    del B_x
    B, S, D = A_x.shape
    F = B_W_gate.shape[1]
    assert B == 1 and D == H * DH == NT * LANES
    assert S % TM == 0 and (F - F0) % TF == 0
    NR = S // TM
    NC = (F - F0) // TF
    assert S // TM0 >= 8

    n_sems = (S // TM0 + len(G_SPLIT) + len(U_SPLIT) + len(D_SPLIT) + 1 + 6
              + D // WOC + NC)
    any_spec = pl.BlockSpec(memory_space=pl.ANY)
    out = pl.pallas_call(
        functools.partial(_kernel, S=S, D=D, F=F),
        out_shape=jax.ShapeDtypeStruct((S, D), _BF16),
        in_specs=[any_spec] * 7,
        out_specs=any_spec,
        scratch_shapes=[
            pltpu.VMEM((S, D + PADX), _BF16),
            pltpu.VMEM((7, D // 2, D + PADW), _BF16),
            pltpu.VMEM((7, D // 2, D + PAD), _BF16),
            pltpu.VMEM((D // WOC + 1, D, WOC), _BF16),
            [pltpu.VMEM((H * WOP, LANES), _F32)] * (WOC // LANES * DH // 8),
            pltpu.VMEM((D // WOC + 1, D, WOC), _BF16),
            pltpu.VMEM((D, F0 + PAD), _BF16),
            pltpu.VMEM((D, F0 + PAD), _BF16),
            pltpu.VMEM((F0, D + PAD), _BF16),
            pltpu.VMEM((NC, D, TF + PAD), _BF16),
            pltpu.VMEM((NC, D, TF + PADW), _BF16),
            pltpu.VMEM((NC, TF, D + PADW), _BF16),
            pltpu.VMEM((S, D), _F32),
            pltpu.VMEM((NT, TM, LANES), _F32),
            pltpu.VMEM((NT, HALO + S, LANES), _F32),
            pltpu.VMEM((NT, HALO + S, LANES), _F32),
            pltpu.VMEM((TM, LANES), _F32),
            pltpu.VMEM((TM, D + PADX), _BF16),
            [pltpu.VMEM((NR, TM, WOC), _BF16)] * (D // WOC),
            pltpu.VMEM((D,), _BF16),
            pltpu.SemaphoreType.DMA((n_sems,)),
            pltpu.SemaphoreType.DMA((D // WOC,)),
        ],
        compiler_params=pltpu.CompilerParams(
            vmem_limit_bytes=120 * 1024 * 1024,
            disable_bounds_checks=True,
            disable_semaphore_checks=True),
        name="gated_mix",
    )(A_x.reshape(S, D), A_wqkv, A_wo, B_W_gate, B_W_up, B_W_down,
      gate_w)
    return out.reshape(B, S, D)
```

```python
import functools
import math

import jax
import jax.numpy as jnp
from jax import lax
import jax.experimental.pallas as pl
import jax.experimental.pallas.tpu as pltpu

H = 32
DH = 32
W = 8
DIL = 2
LANES = 128
NT = 8
HALO = 16

TM = 256
TM0 = 256
F0 = 768
FCH = (768, 768, 640, 640)
UNIT = 8
WOC = 256
WOP = 9
CHAIN_QK = True
CHAIN_PV = True
CHAIN_UNITS = 2
WO_P2 = 3
PADX = 0
PADW = 0
PAD = 128
GATE_TIE = 1
NCHAIN = 1
G_SPLIT = (256, 256, 256)
U_SPLIT = (384, 384)
D_SPLIT = (512, 512)
PB = 4

_F32 = jnp.float32
_BF16 = jnp.bfloat16


def _splits(sizes):
    out, lo = [], 0
    for n in sizes:
        out.append((lo, lo + n))
        lo += n
    return out


def _dot(a, b):
    return jnp.dot(a, b, preferred_element_type=_F32)


def _kernel(x_hbm, wqkv_hbm, wo_hbm, wg_hbm, wu_hbm, wd_hbm, gw_hbm, out_hbm,
            x_v, wq_raw, wq_p, wo_raw, wo_f, wo_p, wg0, wu0, wd0, wg, wu, wd,
            acc, q_s, k_s, v_s, g_s, o_s, out_st, gw_ref,
            sems, sem_out,
            *, S, D, F):
    NR = S // TM
    NR0 = S // TM0
    F1 = F - F0
    NSL = 6
    HR = D // 2

    dc = pl.ds(0, D)

    NWO = D // WOC
    pieces = ([(0, lo, hi) for lo, hi in _splits(G_SPLIT)]
              + [(1, lo, hi) for lo, hi in _splits(U_SPLIT)]
              + [(2, lo, hi) for lo, hi in _splits(D_SPLIT)])
    SX = 0
    SW0 = SX + NR0
    SG = SW0 + len(pieces)
    SQ = SG + 1
    SO = SQ + NSL
    SR = SO + NWO

    def x_copy(t):
        return pltpu.make_async_copy(
            x_hbm.at[pl.ds(t * TM0, TM0), :], x_v.at[pl.ds(t * TM0, TM0), dc],
            sems.at[SX + t])

    def w0_copy(i):
        kind, lo, hi = pieces[i]
        cols = pl.ds(lo, hi - lo)
        src = (wg_hbm.at[:, cols], wu_hbm.at[:, cols],
               wd_hbm.at[pl.ds(0, F0), cols])[kind]
        dst = (wg0, wu0, wd0)[kind].at[:, cols]
        return pltpu.make_async_copy(src, dst, sems.at[SW0 + i])

    def gw_copy():
        return pltpu.make_async_copy(gw_hbm, gw_ref, sems.at[SG])

    def wq_copy(a):
        sec = a // 2
        half = a % 2
        return pltpu.make_async_copy(
            wqkv_hbm.at[pl.ds(half * HR, HR), pl.ds(sec * D, D)],
            wq_raw.at[a, :, dc], sems.at[SQ + a])

    def wo_copy(n):
        lo = n * WOC
        if not isinstance(n, int):
            lo = pl.multiple_of(lo, LANES)
        return pltpu.make_async_copy(
            wo_hbm.at[:, pl.ds(lo, WOC)], wo_raw.at[n], sems.at[SO + n])

    def ffn_copies():
        sem = sems.at[SR]
        f1 = pl.ds(F0, F1)
        return (
            pltpu.make_async_copy(wg_hbm.at[:, f1], wg.at[:, pl.ds(0, F1)], sem),
            pltpu.make_async_copy(wu_hbm.at[:, f1], wu.at[:, pl.ds(0, F1)], sem),
            pltpu.make_async_copy(wd_hbm.at[f1, :], wd.at[:, dc], sem),
        )

    def out_copy(r, n):
        return pltpu.make_async_copy(
            out_st[n].at[r],
            out_hbm.at[pl.ds(r * TM, TM), pl.ds(n * WOC, WOC)],
            sem_out.at[n])

    x_copy(0).start()
    for i in range(len(pieces)):
        w0_copy(i).start()
    for t in range(1, NR0):
        x_copy(t).start()
        if t >= NR0 - NSL:
            wq_copy(t - (NR0 - NSL)).start()
        if t >= NR0 - NWO:
            wo_copy(t - (NR0 - NWO)).start()
    gw_copy().start()
    for cp in ffn_copies():
        cp.start()

    zeros_halo = jnp.zeros((HALO, LANES), _F32)
    for j in range(NT):
        k_s[j, pl.ds(0, HALO), :] = zeros_halo
        v_s[j, pl.ds(0, HALO), :] = zeros_halo

    def permute_slice(a):
        rows = PB * 8
        lane = lax.broadcasted_iota(jnp.int32, (rows, LANES), 1)
        bits = [((lane >> (2 + b)) & 1) == 1 for b in range(3)]
        base_pat = NT * 4 * (lane & 3) + (lane >> 5) + 4 * ((lane >> 2) & 7)
        pats = [(base_pat + 4 * j) & (LANES - 1) for j in range(NT)]
        for g in range(HR // (16 * PB)):
            rs = pl.ds(g * 16 * PB, 16 * PB)
            z = []
            for i in range(NT):
                w = pltpu.bitcast(wq_raw[a, rs, pl.ds(i * LANES, LANES)],
                                  jnp.uint32)
                z.append(w if i == 0 else pltpu.roll(w, 4 * i, 1))
            for b in range(3):
                z = [jnp.where(bits[b], z[(k + (1 << b)) % NT], z[k])
                     for k in range(NT)]
            for j in range(NT):
                y = jnp.take_along_axis(z[(-j) % NT], pats[j], axis=1)
                wq_p[a, rs, pl.ds(j * LANES, LANES)] = pltpu.bitcast(y, _BF16)

    def permute_wo(n, never, pace1, pace2):
        nj = WOC // LANES
        i = 0
        for h in range(H):
            blk = wo_raw[n, pl.ds(h * DH, DH), :].astype(_F32)
            for a in range(DH // 8):
                for j in range(nj):
                    pc = blk[a * 8:(a + 1) * 8, j * LANES:(j + 1) * LANES]
                    pc = jnp.where(never, pace1[i], pc)
                    i += 1
                    wo_f[a * nj + j][pl.ds(h * WOP, 8), :] = pc
        i = 0
        for d in range(DH):
            for b in range(H // 8):
                rws = []
                for j in range(nj):
                    pc = wo_f[(d // 8) * nj + j][
                        pl.ds(b * 8 * WOP + d % 8, 8, stride=WOP), :]
                    pc = jnp.where(never, pace2[i], pc)
                    i += 1
                    rws.append(pc)
                wo_p[n, pl.ds(d * H + b * 8, 8), :] = jnp.concatenate(
                    rws, axis=1).astype(_BF16)

    def vregs(v):
        return [v[i * 8:(i + 1) * 8, n * LANES:(n + 1) * LANES]
                for n in range(v.shape[1] // LANES)
                for i in range(v.shape[0] // 8)]

    x_copy(0).wait()
    parts = ([], [])
    hh0 = None
    for i, (kind, lo, hi) in enumerate(pieces):
        w0_copy(i).wait()
        cols = pl.ds(lo, hi - lo)
        if kind < 2:
            parts[kind].append(
                _dot(x_v[pl.ds(0, TM0), dc], (wg0, wu0)[kind][:, cols]))
        else:
            if hh0 is None:
                hh0 = (jnp.maximum(jnp.concatenate(parts[0], axis=1), 0.0)
                       * jnp.concatenate(parts[1], axis=1)).astype(_BF16)
            acc[pl.ds(0, TM0), cols] = _dot(hh0, wd0[:, cols])

    def phase0(t, carry):
        x_copy(t).wait()
        real = t >= NR0 - NSL

        @pl.when(real)
        def _():
            wq_copy(t - (NR0 - NSL)).wait()

        real_o = t >= NR0 - NWO

        @pl.when(real_o)
        def _():
            wo_copy(t - (NR0 - NWO)).wait()

        rows = pl.ds(pl.multiple_of(t * TM0, TM0), TM0)
        xv = x_v[rows, dc]
        gt = _dot(xv, wg0[:, pl.ds(0, F0)])
        up = _dot(xv, wu0[:, pl.ds(0, F0)])
        hh = (jnp.maximum(gt, 0.0) * up).astype(_BF16)
        dn = _dot(hh, wd0[:, dc])
        acc[rows, :] = dn
        permute_slice(jnp.where(real, t - (NR0 - NSL), NSL))
        never = lax.broadcasted_iota(jnp.int32, (8, LANES), 1) < -1 - t
        p2 = vregs(dn)
        p2 = [p2[i * WO_P2 // 4] for i in range(len(p2))]
        p1 = vregs(gt) + vregs(up)
        p1 = [p1[i * len(p1) // len(p2)] for i in range(len(p2))]
        permute_wo(jnp.where(real_o, t - (NR0 - NWO), NWO), never, p1, p2)
        return carry

    lax.fori_loop(1, NR0, phase0, 0)
    gw_copy().wait()
    for cp in ffn_copies():
        cp.wait()

    c_exp = (DH ** -0.5) * math.log2(math.e)
    neg = -1e9 / (DH ** -0.5)

    def attn_unit(r, row0, gw, never, link, masked):
        def tie(a, b):
            return a if b is None else jnp.where(never, b, a)

        base = r * TM + row0
        qs = [q_s[j, pl.ds(row0, UNIT), :] for j in range(NT)]
        xr = x_v[pl.ds(pl.multiple_of(base, UNIT), UNIT), dc].astype(_F32)
        xg = (tie(xr[:, 0:LANES], link) if GATE_TIE == 2 else xr[:, 0:LANES]) * gw[:, 0:LANES]
        for j in range(1, NT):
            cols = slice(j * LANES, (j + 1) * LANES)
            xg = xg + xr[:, cols] * gw[:, cols]
        logits = []
        for w in range(W):
            st = base + (HALO - DIL * w)
            q0 = tie(qs[0], link) if CHAIN_QK else qs[0]
            s = q0 * k_s[0, pl.ds(st, UNIT), :]
            for j in range(1, NT):
                s = s + qs[j] * k_s[j, pl.ds(st, UNIT), :]
            link = s
            s = s + pltpu.roll(s, 64, 1)
            s = s + pltpu.roll(s, 32, 1)
            if masked and w > 0:
                pos = base + lax.broadcasted_iota(jnp.int32, (UNIT, LANES), 0)
                s = jnp.where(pos >= DIL * w, s, neg)
            logits.append(s)
        m = logits[0]
        for w in range(1, W):
            m = jnp.maximum(m, logits[w])
        ps = [jnp.exp2((logits[w] - m) * c_exp) for w in range(W)]
        den = ps[0]
        for w in range(1, W):
            den = den + ps[w]
        gate = jax.nn.sigmoid(jnp.sum(xg, axis=-1, keepdims=True))
        gate = jnp.broadcast_to(gate, (UNIT, LANES))
        g_s[pl.ds(row0, UNIT), :] = 1.0 - gate
        rinv = gate / den
        olink = gate if GATE_TIE else None
        for j in range(NT):
            p0 = tie(ps[0], olink) if CHAIN_PV else ps[0]
            o = p0 * v_s[j, pl.ds(base + HALO, UNIT), :]
            for w in range(1, W):
                o = o + ps[w] * v_s[j, pl.ds(base + (HALO - DIL * w), UNIT), :]
            olink = o
            o_s[pl.ds(row0, UNIT), pl.ds(j * LANES, LANES)] = (
                (o * rinv).astype(_BF16))
        return olink if CHAIN_UNITS == 2 else (link if CHAIN_UNITS else None)

    def row_block(r, carry):
        rows = pl.ds(pl.multiple_of(r * TM, TM), TM)
        krows = pl.ds(pl.multiple_of(r * TM + HALO, HALO), TM)
        xv = x_v[rows, dc]
        for sec, dst in enumerate((q_s, k_s, v_s)):
            wsec = wq_p[pl.ds(2 * sec, 2), :, pl.ds(0, D)].reshape(D, D)
            res = _dot(xv, wsec)
            for j in range(NT):
                piece = res[:, j * LANES:(j + 1) * LANES]
                if sec == 0:
                    dst[j] = piece
                else:
                    dst[j, krows, :] = piece
        gw = gw_ref[...].astype(_F32).reshape(1, D)
        never = lax.broadcasted_iota(jnp.int32, (UNIT, LANES), 1) < -1 - r
        links = [None] * NCHAIN
        for un in range(TM // UNIT):
            links[un % NCHAIN] = attn_unit(
                r, un * UNIT, gw, never, links[un % NCHAIN],
                masked=(un * UNIT < HALO))
        for lo, hi in _splits(FCH):
            cols = pl.ds(lo, hi - lo)
            gt = _dot(xv, wg[:, cols])
            up = _dot(xv, wu[:, cols])
            hh = (jnp.maximum(gt, 0.0) * up).astype(_BF16)
            acc[rows, :] += _dot(hh, wd[cols, dc])

        ov = o_s[:, dc]
        g1 = g_s[...]
        g1 = jnp.concatenate([g1] * (WOC // LANES), axis=1)
        for n in range(NWO):
            cols = pl.ds(n * WOC, WOC)
            a = _dot(ov, wo_p[n])
            out_st[n][r] = (a + g1 * acc[rows, cols]).astype(_BF16)
            out_copy(r, n).start()
        return carry

    lax.fori_loop(0, NR, row_block, 0)
    for n in range(NWO):
        for r in range(NR):
            out_copy(r, n).wait()


@jax.jit
def pallas_gated_mix__sliding_local_dilated__glu_gated_reglu__prompt_kernel(
    A_x: jax.Array,
    A_wqkv: jax.Array,
    A_wo: jax.Array,
    B_x: jax.Array,
    B_W_gate: jax.Array,
    B_W_up: jax.Array,
    B_W_down: jax.Array,
    gate_w: jax.Array,
):
    del B_x
    B, S, D = A_x.shape
    F = B_W_gate.shape[1]
    assert B == 1 and D == H * DH == NT * LANES
    assert S % TM == 0 and F - F0 == sum(FCH)
    NR = S // TM
    F1 = F - F0
    assert S // TM0 >= 8

    n_sems = (S // TM0 + len(G_SPLIT) + len(U_SPLIT) + len(D_SPLIT) + 1 + 6
              + D // WOC + 1)
    any_spec = pl.BlockSpec(memory_space=pl.ANY)
    out = pl.pallas_call(
        functools.partial(_kernel, S=S, D=D, F=F),
        out_shape=jax.ShapeDtypeStruct((S, D), _BF16),
        in_specs=[any_spec] * 7,
        out_specs=any_spec,
        scratch_shapes=[
            pltpu.VMEM((S, D + PADX), _BF16),
            pltpu.VMEM((7, D // 2, D + PADW), _BF16),
            pltpu.VMEM((7, D // 2, D + PAD), _BF16),
            pltpu.VMEM((D // WOC + 1, D, WOC), _BF16),
            [pltpu.VMEM((H * WOP, LANES), _F32)] * (WOC // LANES * DH // 8),
            pltpu.VMEM((D // WOC + 1, D, WOC), _BF16),
            pltpu.VMEM((D, F0 + PAD), _BF16),
            pltpu.VMEM((D, F0 + PAD), _BF16),
            pltpu.VMEM((F0, D + PAD), _BF16),
            pltpu.VMEM((D, F1), _BF16),
            pltpu.VMEM((D, F1), _BF16),
            pltpu.VMEM((F1, D + PADW), _BF16),
            pltpu.VMEM((S, D), _F32),
            pltpu.VMEM((NT, TM, LANES), _F32),
            pltpu.VMEM((NT, HALO + S, LANES), _F32),
            pltpu.VMEM((NT, HALO + S, LANES), _F32),
            pltpu.VMEM((TM, LANES), _F32),
            pltpu.VMEM((TM, D + PADX), _BF16),
            [pltpu.VMEM((NR, TM, WOC), _BF16)] * (D // WOC),
            pltpu.VMEM((D,), _BF16),
            pltpu.SemaphoreType.DMA((n_sems,)),
            pltpu.SemaphoreType.DMA((D // WOC,)),
        ],
        compiler_params=pltpu.CompilerParams(
            vmem_limit_bytes=120 * 1024 * 1024,
            disable_bounds_checks=True,
            disable_semaphore_checks=True),
        name="gated_mix",
    )(A_x.reshape(S, D), A_wqkv, A_wo, B_W_gate, B_W_up, B_W_down,
      gate_w)
    return out.reshape(B, S, D)
```

```python
import functools
import math

import jax
import jax.numpy as jnp
from jax import lax
import jax.experimental.pallas as pl
import jax.experimental.pallas.tpu as pltpu

H = 32
DH = 32
W = 8
DIL = 2
LANES = 128
NT = 8
HALO = 16

TM = 256
TM0 = 256
F0 = 768
FCH = (768, 768, 640, 640)
UNIT = 8
WOC = 256
WOP = 9
CHAIN_QK = True
CHAIN_PV = True
CHAIN_UNITS = 2
WO_P2 = 3
PADX = 0
PADW = 0
PAD = 128
GATE_TIE = 1
NCHAIN = 1
G_SPLIT = (128, 128, 256, 256)
U_SPLIT = (384, 384)
D_SPLIT = (512, 512)
PB = 4

_F32 = jnp.float32
_BF16 = jnp.bfloat16


def _splits(sizes):
    out, lo = [], 0
    for n in sizes:
        out.append((lo, lo + n))
        lo += n
    return out


def _dot(a, b):
    return jnp.dot(a, b, preferred_element_type=_F32)


def _kernel(x_hbm, wqkv_hbm, wo_hbm, wg_hbm, wu_hbm, wd_hbm, gw_hbm, out_hbm,
            x_v, wq_raw, wq_p, wo_raw, wo_f, wo_p, wg0, wu0, wd0, wg, wu, wd,
            acc, q_s, k_s, v_s, g_s, o_s, out_st, gw_ref,
            sems, sem_out,
            *, S, D, F):
    NR = S // TM
    NR0 = S // TM0
    F1 = F - F0
    NSL = 6
    HR = D // 2

    dc = pl.ds(0, D)

    NWO = D // WOC
    pieces = ([(0, lo, hi) for lo, hi in _splits(G_SPLIT)]
              + [(1, lo, hi) for lo, hi in _splits(U_SPLIT)]
              + [(2, lo, hi) for lo, hi in _splits(D_SPLIT)])
    SX = 0
    SW0 = SX + NR0
    SG = SW0 + len(pieces)
    SQ = SG + 1
    SO = SQ + NSL
    SR = SO + NWO

    def x_copy(t):
        return pltpu.make_async_copy(
            x_hbm.at[pl.ds(t * TM0, TM0), :], x_v.at[pl.ds(t * TM0, TM0), dc],
            sems.at[SX + t])

    def w0_copy(i):
        kind, lo, hi = pieces[i]
        cols = pl.ds(lo, hi - lo)
        src = (wg_hbm.at[:, cols], wu_hbm.at[:, cols],
               wd_hbm.at[pl.ds(0, F0), cols])[kind]
        dst = (wg0, wu0, wd0)[kind].at[:, cols]
        return pltpu.make_async_copy(src, dst, sems.at[SW0 + i])

    def gw_copy():
        return pltpu.make_async_copy(gw_hbm, gw_ref, sems.at[SG])

    def wq_copy(a):
        sec = a // 2
        half = a % 2
        return pltpu.make_async_copy(
            wqkv_hbm.at[pl.ds(half * HR, HR), pl.ds(sec * D, D)],
            wq_raw.at[a, :, dc], sems.at[SQ + a])

    def wo_copy(n):
        lo = n * WOC
        if not isinstance(n, int):
            lo = pl.multiple_of(lo, LANES)
        return pltpu.make_async_copy(
            wo_hbm.at[:, pl.ds(lo, WOC)], wo_raw.at[n], sems.at[SO + n])

    def ffn_copies():
        sem = sems.at[SR]
        f1 = pl.ds(F0, F1)
        return (
            pltpu.make_async_copy(wg_hbm.at[:, f1], wg.at[:, pl.ds(0, F1)], sem),
            pltpu.make_async_copy(wu_hbm.at[:, f1], wu.at[:, pl.ds(0, F1)], sem),
            pltpu.make_async_copy(wd_hbm.at[f1, :], wd.at[:, dc], sem),
        )

    def out_copy(r, n):
        return pltpu.make_async_copy(
            out_st[n].at[r],
            out_hbm.at[pl.ds(r * TM, TM), pl.ds(n * WOC, WOC)],
            sem_out.at[n])

    x_copy(0).start()
    for i in range(len(pieces)):
        w0_copy(i).start()
    for t in range(1, NR0):
        x_copy(t).start()
        if t >= NR0 - NSL:
            wq_copy(t - (NR0 - NSL)).start()
        if t >= NR0 - NWO:
            wo_copy(t - (NR0 - NWO)).start()
    gw_copy().start()
    for cp in ffn_copies():
        cp.start()

    zeros_halo = jnp.zeros((HALO, LANES), _F32)
    for j in range(NT):
        k_s[j, pl.ds(0, HALO), :] = zeros_halo
        v_s[j, pl.ds(0, HALO), :] = zeros_halo

    def clear(i, carry):
        rs = pl.ds(pl.multiple_of(i * 32, 32), 32)
        wq_raw[NSL, rs, :] = jnp.zeros((32, D), _BF16)
        rs = pl.ds(pl.multiple_of(i * 64, 64), 64)
        wo_raw[NWO, rs, :] = jnp.zeros((64, WOC), _BF16)
        return carry

    lax.fori_loop(0, HR // 32, clear, 0)

    def permute_slice(a):
        rows = PB * 8
        lane = lax.broadcasted_iota(jnp.int32, (rows, LANES), 1)
        bits = [((lane >> (2 + b)) & 1) == 1 for b in range(3)]
        base_pat = NT * 4 * (lane & 3) + (lane >> 5) + 4 * ((lane >> 2) & 7)
        pats = [(base_pat + 4 * j) & (LANES - 1) for j in range(NT)]
        for g in range(HR // (16 * PB)):
            rs = pl.ds(g * 16 * PB, 16 * PB)
            z = []
            for i in range(NT):
                w = pltpu.bitcast(wq_raw[a, rs, pl.ds(i * LANES, LANES)],
                                  jnp.uint32)
                z.append(w if i == 0 else pltpu.roll(w, 4 * i, 1))
            for b in range(3):
                z = [jnp.where(bits[b], z[(k + (1 << b)) % NT], z[k])
                     for k in range(NT)]
            for j in range(NT):
                y = jnp.take_along_axis(z[(-j) % NT], pats[j], axis=1)
                wq_p[a, rs, pl.ds(j * LANES, LANES)] = pltpu.bitcast(y, _BF16)

    def permute_wo(n, never, pace1, pace2):
        nj = WOC // LANES
        i = 0
        for h in range(H):
            blk = wo_raw[n, pl.ds(h * DH, DH), :].astype(_F32)
            for a in range(DH // 8):
                for j in range(nj):
                    pc = blk[a * 8:(a + 1) * 8, j * LANES:(j + 1) * LANES]
                    pc = jnp.where(never, pace1[i], pc)
                    i += 1
                    wo_f[a * nj + j][pl.ds(h * WOP, 8), :] = pc
        i = 0
        for d in range(DH):
            for b in range(H // 8):
                rws = []
                for j in range(nj):
                    pc = wo_f[(d // 8) * nj + j][
                        pl.ds(b * 8 * WOP + d % 8, 8, stride=WOP), :]
                    pc = jnp.where(never, pace2[i], pc)
                    i += 1
                    rws.append(pc)
                wo_p[n, pl.ds(d * H + b * 8, 8), :] = jnp.concatenate(
                    rws, axis=1).astype(_BF16)

    def vregs(v):
        return [v[i * 8:(i + 1) * 8, n * LANES:(n + 1) * LANES]
                for n in range(v.shape[1] // LANES)
                for i in range(v.shape[0] // 8)]

    x_copy(0).wait()
    parts = ([], [])
    hh0 = None
    for i, (kind, lo, hi) in enumerate(pieces):
        w0_copy(i).wait()
        cols = pl.ds(lo, hi - lo)
        if kind < 2:
            parts[kind].append(
                _dot(x_v[pl.ds(0, TM0), dc], (wg0, wu0)[kind][:, cols]))
        else:
            if hh0 is None:
                hh0 = (jnp.maximum(jnp.concatenate(parts[0], axis=1), 0.0)
                       * jnp.concatenate(parts[1], axis=1)).astype(_BF16)
            acc[pl.ds(0, TM0), cols] = _dot(hh0, wd0[:, cols])

    def phase0(t, carry):
        x_copy(t).wait()
        real = t >= NR0 - NSL

        @pl.when(real)
        def _():
            wq_copy(t - (NR0 - NSL)).wait()

        real_o = t >= NR0 - NWO

        @pl.when(real_o)
        def _():
            wo_copy(t - (NR0 - NWO)).wait()

        rows = pl.ds(pl.multiple_of(t * TM0, TM0), TM0)
        xv = x_v[rows, dc]
        gt = _dot(xv, wg0[:, pl.ds(0, F0)])
        up = _dot(xv, wu0[:, pl.ds(0, F0)])
        hh = (jnp.maximum(gt, 0.0) * up).astype(_BF16)
        dn = _dot(hh, wd0[:, dc])
        acc[rows, :] = dn
        permute_slice(jnp.where(real, t - (NR0 - NSL), NSL))
        never = lax.broadcasted_iota(jnp.int32, (8, LANES), 1) < -1 - t
        p2 = vregs(dn)
        p2 = [p2[i * WO_P2 // 4] for i in range(len(p2))]
        p1 = vregs(gt) + vregs(up)
        p1 = [p1[i * len(p1) // len(p2)] for i in range(len(p2))]
        permute_wo(jnp.where(real_o, t - (NR0 - NWO), NWO), never, p1, p2)
        return carry

    lax.fori_loop(1, NR0, phase0, 0)
    gw_copy().wait()
    for cp in ffn_copies():
        cp.wait()

    c_exp = (DH ** -0.5) * math.log2(math.e)
    neg = -1e9 / (DH ** -0.5)

    def attn_unit(r, row0, gw, never, link, masked):
        def tie(a, b):
            return a if b is None else jnp.where(never, b, a)

        base = r * TM + row0
        qs = [q_s[j, pl.ds(row0, UNIT), :] for j in range(NT)]
        xr = x_v[pl.ds(pl.multiple_of(base, UNIT), UNIT), dc].astype(_F32)
        xg = (tie(xr[:, 0:LANES], link) if GATE_TIE == 2 else xr[:, 0:LANES]) * gw[:, 0:LANES]
        for j in range(1, NT):
            cols = slice(j * LANES, (j + 1) * LANES)
            xg = xg + xr[:, cols] * gw[:, cols]
        logits = []
        for w in range(W):
            st = base + (HALO - DIL * w)
            q0 = tie(qs[0], link) if CHAIN_QK else qs[0]
            s = q0 * k_s[0, pl.ds(st, UNIT), :]
            for j in range(1, NT):
                s = s + qs[j] * k_s[j, pl.ds(st, UNIT), :]
            link = s
            s = s + pltpu.roll(s, 64, 1)
            s = s + pltpu.roll(s, 32, 1)
            if masked and w > 0:
                pos = base + lax.broadcasted_iota(jnp.int32, (UNIT, LANES), 0)
                s = jnp.where(pos >= DIL * w, s, neg)
            logits.append(s)
        m = logits[0]
        for w in range(1, W):
            m = jnp.maximum(m, logits[w])
        ps = [jnp.exp2((logits[w] - m) * c_exp) for w in range(W)]
        den = ps[0]
        for w in range(1, W):
            den = den + ps[w]
        gate = jax.nn.sigmoid(jnp.sum(xg, axis=-1, keepdims=True))
        gate = jnp.broadcast_to(gate, (UNIT, LANES))
        g_s[pl.ds(row0, UNIT), :] = 1.0 - gate
        rinv = gate / den
        olink = gate if GATE_TIE else None
        for j in range(NT):
            p0 = tie(ps[0], olink) if CHAIN_PV else ps[0]
            o = p0 * v_s[j, pl.ds(base + HALO, UNIT), :]
            for w in range(1, W):
                o = o + ps[w] * v_s[j, pl.ds(base + (HALO - DIL * w), UNIT), :]
            olink = o
            o_s[pl.ds(row0, UNIT), pl.ds(j * LANES, LANES)] = (
                (o * rinv).astype(_BF16))
        return olink if CHAIN_UNITS == 2 else (link if CHAIN_UNITS else None)

    def row_block(r, carry):
        rows = pl.ds(pl.multiple_of(r * TM, TM), TM)
        krows = pl.ds(pl.multiple_of(r * TM + HALO, HALO), TM)
        xv = x_v[rows, dc]
        for sec, dst in enumerate((q_s, k_s, v_s)):
            wsec = wq_p[pl.ds(2 * sec, 2), :, pl.ds(0, D)].reshape(D, D)
            res = _dot(xv, wsec)
            for j in range(NT):
                piece = res[:, j * LANES:(j + 1) * LANES]
                if sec == 0:
                    dst[j] = piece
                else:
                    dst[j, krows, :] = piece
        gw = gw_ref[...].astype(_F32).reshape(1, D)
        never = lax.broadcasted_iota(jnp.int32, (UNIT, LANES), 1) < -1 - r
        links = [None] * NCHAIN
        for un in range(TM // UNIT):
            links[un % NCHAIN] = attn_unit(
                r, un * UNIT, gw, never, links[un % NCHAIN],
                masked=(un * UNIT < HALO))
        for lo, hi in _splits(FCH):
            cols = pl.ds(lo, hi - lo)
            gt = _dot(xv, wg[:, cols])
            up = _dot(xv, wu[:, cols])
            hh = (jnp.maximum(gt, 0.0) * up).astype(_BF16)
            acc[rows, :] += _dot(hh, wd[cols, dc])

        ov = o_s[:, dc]
        g1 = g_s[...]
        g1 = jnp.concatenate([g1] * (WOC // LANES), axis=1)
        for n in range(NWO):
            cols = pl.ds(n * WOC, WOC)
            a = _dot(ov, wo_p[n])
            out_st[n][r] = (a + g1 * acc[rows, cols]).astype(_BF16)
            out_copy(r, n).start()
        return carry

    lax.fori_loop(0, NR, row_block, 0)
    for n in range(NWO):
        for r in range(NR):
            out_copy(r, n).wait()


@jax.jit
def pallas_gated_mix__sliding_local_dilated__glu_gated_reglu__prompt_kernel(
    A_x: jax.Array,
    A_wqkv: jax.Array,
    A_wo: jax.Array,
    B_x: jax.Array,
    B_W_gate: jax.Array,
    B_W_up: jax.Array,
    B_W_down: jax.Array,
    gate_w: jax.Array,
):
    del B_x
    B, S, D = A_x.shape
    F = B_W_gate.shape[1]
    assert B == 1 and D == H * DH == NT * LANES
    assert S % TM == 0 and F - F0 == sum(FCH)
    NR = S // TM
    F1 = F - F0
    assert S // TM0 >= 8

    n_sems = (S // TM0 + len(G_SPLIT) + len(U_SPLIT) + len(D_SPLIT) + 1 + 6
              + D // WOC + 1)
    any_spec = pl.BlockSpec(memory_space=pl.ANY)
    out = pl.pallas_call(
        functools.partial(_kernel, S=S, D=D, F=F),
        out_shape=jax.ShapeDtypeStruct((S, D), _BF16),
        in_specs=[any_spec] * 7,
        out_specs=any_spec,
        scratch_shapes=[
            pltpu.VMEM((S, D + PADX), _BF16),
            pltpu.VMEM((7, D // 2, D + PADW), _BF16),
            pltpu.VMEM((7, D // 2, D + PAD), _BF16),
            pltpu.VMEM((D // WOC + 1, D, WOC), _BF16),
            [pltpu.VMEM((H * (WOP + 1), LANES), _F32)] * (WOC // LANES * DH // 8),
            pltpu.VMEM((D // WOC + 1, D, WOC), _BF16),
            pltpu.VMEM((D, F0 + PAD), _BF16),
            pltpu.VMEM((D, F0 + PAD), _BF16),
            pltpu.VMEM((F0, D + PAD), _BF16),
            pltpu.VMEM((D, F1), _BF16),
            pltpu.VMEM((D, F1), _BF16),
            pltpu.VMEM((F1, D + PADW), _BF16),
            pltpu.VMEM((S, D), _F32),
            pltpu.VMEM((NT, TM, LANES), _F32),
            pltpu.VMEM((NT, HALO + S, LANES), _F32),
            pltpu.VMEM((NT, HALO + S, LANES), _F32),
            pltpu.VMEM((TM, LANES), _F32),
            pltpu.VMEM((TM, D + PADX), _BF16),
            [pltpu.VMEM((NR, TM, WOC), _BF16)] * (D // WOC),
            pltpu.VMEM((D,), _BF16),
            pltpu.SemaphoreType.DMA((n_sems,)),
            pltpu.SemaphoreType.DMA((D // WOC,)),
        ],
        compiler_params=pltpu.CompilerParams(
            vmem_limit_bytes=120 * 1024 * 1024,
            disable_bounds_checks=True,
            disable_semaphore_checks=True),
        name="gated_mix",
    )(A_x.reshape(S, D), A_wqkv, A_wo, B_W_gate, B_W_up, B_W_down,
      gate_w)
    return out.reshape(B, S, D)
```

```python
import functools
import math

import jax
import jax.numpy as jnp
from jax import lax
import jax.experimental.pallas as pl
import jax.experimental.pallas.tpu as pltpu

H = 32
DH = 32
W = 8
DIL = 2
LANES = 128
NT = 8
HALO = 16

TM = 256
TM0 = 512
FH = 384
F0 = 2 * FH
FCH = (768, 768, 640, 640)
UNIT = 8
WOC = 256
WOP = 9
CHAIN_QK = True
CHAIN_PV = True
CHAIN_UNITS = 2
PAD = 128
GATE_TIE = 1
NCHAIN = 1
START_LOADS = (("x", 0, 256), ("g", 0, 128), ("g", 128, 384), ("x", 256, 512),
               ("u", 0, 384), ("d", 0, 1024))
START_STAGES = ((2, (("g", 0, 256, 0, 128),)),
                (1, (("g", 0, 256, 128, 384),)),
                (1, (("g", 256, 512, 0, 384),)),
                (1, (("u", 0, 512, 0, 384),)),
                (1, (("d", 0, 512, 0, 1024),)))
PB = 4

_F32 = jnp.float32
_BF16 = jnp.bfloat16


def _splits(sizes):
    out, lo = [], 0
    for n in sizes:
        out.append((lo, lo + n))
        lo += n
    return out


def _dot(a, b):
    return jnp.dot(a, b, preferred_element_type=_F32)


def _kernel(x_hbm, wqkv_hbm, wo_hbm, wg_hbm, wu_hbm, wd_hbm, gw_hbm, out_hbm,
            x_v, wq_raw, wq_p, wo_raw, wo_f, wo_p, wg0, wu0, wd0, wg, wu, wd,
            acc, q_s, k_s, v_s, g_s, o_s, out_st, gw_ref,
            sems, sem_out,
            *, S, D, F):
    NR = S // TM
    NR0 = S // TM0
    NP0 = 2 * NR0
    F1 = F - F0
    NSL = 6
    HR = D // 2

    dc = pl.ds(0, D)

    NWO = D // WOC
    SW0 = 0
    SX = SW0 + len(START_LOADS)
    SW1 = SX + NR0 - 1
    SG = SW1 + 1
    SQ = SG + 1
    SO = SQ + NSL
    SR = SO + NWO

    def start_copy(i):
        kind, lo, hi = START_LOADS[i]
        sl = pl.ds(lo, hi - lo)
        hs = pl.ds(0, FH)
        if kind == "x":
            src, dst = x_hbm.at[sl, :], x_v.at[sl, :]
        elif kind == "g":
            src, dst = wg_hbm.at[:, sl], wg0.at[0, :, sl]
        elif kind == "u":
            src, dst = wu_hbm.at[:, sl], wu0.at[0, :, sl]
        else:
            src, dst = wd_hbm.at[hs, sl], wd0.at[0, :, sl]
        return pltpu.make_async_copy(src, dst, sems.at[SW0 + i])

    def x_copy(r):
        rows = pl.ds(r * TM0, TM0)
        return pltpu.make_async_copy(
            x_hbm.at[rows, :], x_v.at[rows, :], sems.at[SX + r - 1])

    def w1_copies():
        sem = sems.at[SW1]
        h1 = pl.ds(FH, FH)
        hs = pl.ds(0, FH)
        return (
            pltpu.make_async_copy(wg_hbm.at[:, h1], wg0.at[1, :, hs], sem),
            pltpu.make_async_copy(wu_hbm.at[:, h1], wu0.at[1, :, hs], sem),
            pltpu.make_async_copy(wd_hbm.at[h1, :], wd0.at[1, :, dc], sem),
        )

    def gw_copy():
        return pltpu.make_async_copy(gw_hbm, gw_ref, sems.at[SG])

    def wq_copy(a):
        sec = a // 2
        half = a % 2
        return pltpu.make_async_copy(
            wqkv_hbm.at[pl.ds(half * HR, HR), pl.ds(sec * D, D)],
            wq_raw.at[a], sems.at[SQ + a])

    def wo_copy(n):
        lo = n * WOC
        if not isinstance(n, int):
            lo = pl.multiple_of(lo, LANES)
        return pltpu.make_async_copy(
            wo_hbm.at[:, pl.ds(lo, WOC)], wo_raw.at[n], sems.at[SO + n])

    def ffn_copies():
        sem = sems.at[SR]
        f1 = pl.ds(F0, F1)
        return (
            pltpu.make_async_copy(wg_hbm.at[:, f1], wg, sem),
            pltpu.make_async_copy(wu_hbm.at[:, f1], wu, sem),
            pltpu.make_async_copy(wd_hbm.at[f1, :], wd, sem),
        )

    def out_copy(r, n):
        return pltpu.make_async_copy(
            out_st[n].at[r],
            out_hbm.at[pl.ds(r * TM, TM), pl.ds(n * WOC, WOC)],
            sem_out.at[n])

    for i in range(len(START_LOADS)):
        start_copy(i).start()
    for cp in w1_copies():
        cp.start()
    for t in range(2, NP0):
        if t % 2 == 0:
            x_copy(t // 2).start()
        if t >= NP0 - NSL:
            wq_copy(t - (NP0 - NSL)).start()
        if t >= NP0 - NWO:
            wo_copy(t - (NP0 - NWO)).start()
    gw_copy().start()
    for cp in ffn_copies():
        cp.start()

    zeros_halo = jnp.zeros((HALO, LANES), _F32)
    for j in range(NT):
        k_s[j, pl.ds(0, HALO), :] = zeros_halo
        v_s[j, pl.ds(0, HALO), :] = zeros_halo

    def clear(i, carry):
        rs = pl.ds(pl.multiple_of(i * 32, 32), 32)
        wq_raw[NSL, rs, :] = jnp.zeros((32, D), _BF16)
        rs = pl.ds(pl.multiple_of(i * 64, 64), 64)
        wo_raw[NWO, rs, :] = jnp.zeros((64, WOC), _BF16)
        return carry

    lax.fori_loop(0, HR // 32, clear, 0)

    def permute_slice(a):
        rows = PB * 8
        lane = lax.broadcasted_iota(jnp.int32, (rows, LANES), 1)
        bits = [((lane >> (2 + b)) & 1) == 1 for b in range(3)]
        base_pat = NT * 4 * (lane & 3) + (lane >> 5) + 4 * ((lane >> 2) & 7)
        pats = [(base_pat + 4 * j) & (LANES - 1) for j in range(NT)]
        for g in range(HR // (16 * PB)):
            rs = pl.ds(g * 16 * PB, 16 * PB)
            z = []
            for i in range(NT):
                w = pltpu.bitcast(wq_raw[a, rs, pl.ds(i * LANES, LANES)],
                                  jnp.uint32)
                z.append(w if i == 0 else pltpu.roll(w, 4 * i, 1))
            for b in range(3):
                z = [jnp.where(bits[b], z[(k + (1 << b)) % NT], z[k])
                     for k in range(NT)]
            for j in range(NT):
                y = jnp.take_along_axis(z[(-j) % NT], pats[j], axis=1)
                wq_p[a, rs, pl.ds(j * LANES, LANES)] = pltpu.bitcast(y, _BF16)

    def permute_wo(n, never, pace1, pace2):
        nj = WOC // LANES
        i = 0
        for h in range(H):
            blk = wo_raw[n, pl.ds(h * DH, DH), :].astype(_F32)
            for a in range(DH // 8):
                for j in range(nj):
                    pc = blk[a * 8:(a + 1) * 8, j * LANES:(j + 1) * LANES]
                    pc = jnp.where(never, pace1[i], pc)
                    i += 1
                    wo_f[a * nj + j][pl.ds(h * WOP, 8), :] = pc
        i = 0
        for d in range(DH):
            for b in range(H // 8):
                rws = []
                for j in range(nj):
                    pc = wo_f[(d // 8) * nj + j][
                        pl.ds(b * 8 * WOP + d % 8, 8, stride=WOP), :]
                    pc = jnp.where(never, pace2[i], pc)
                    i += 1
                    rws.append(pc)
                wo_p[n, pl.ds(d * H + b * 8, 8), :] = jnp.concatenate(
                    rws, axis=1).astype(_BF16)

    def vregs(v):
        return [v[i * 8:(i + 1) * 8, n * LANES:(n + 1) * LANES]
                for n in range(v.shape[1] // LANES)
                for i in range(v.shape[0] // 8)]

    done = 0
    parts = {"g": {}, "u": {}}
    hh0 = None

    def assemble(pcs):
        row_los = sorted({k[0] for k in pcs})
        return jnp.concatenate(
            [jnp.concatenate([pcs[k] for k in sorted(pcs) if k[0] == r0], axis=1)
             for r0 in row_los], axis=0)

    for nwait, work in START_STAGES:
        for i in range(done, done + nwait):
            start_copy(i).wait()
        done += nwait
        for kind, r0, r1, c0, c1 in work:
            cols = pl.ds(c0, c1 - c0)
            if kind != "d":
                wref = wg0 if kind == "g" else wu0
                res = _dot(x_v[pl.ds(r0, r1 - r0), :], wref[0, :, cols])
                for rr in range(r0, r1, 256):
                    for cc in range(c0, c1, LANES):
                        parts[kind][(rr, cc)] = res[
                            rr - r0:rr - r0 + 256, cc - c0:cc - c0 + LANES]
            else:
                if hh0 is None:
                    hh0 = (jnp.maximum(assemble(parts["g"]), 0.0)
                           * assemble(parts["u"])).astype(_BF16)
                acc[pl.ds(r0, r1 - r0), cols] = _dot(
                    hh0[r0:r1], wd0[0, :, cols])

    def phase0(t, carry):
        r = t // 2
        half = t % 2

        @pl.when(t == 1)
        def _():
            for cp in w1_copies():
                cp.wait()

        @pl.when(half == 0)
        def _():
            x_copy(r).wait()

        real = t >= NP0 - NSL

        @pl.when(real)
        def _():
            wq_copy(t - (NP0 - NSL)).wait()

        real_o = t >= NP0 - NWO

        @pl.when(real_o)
        def _():
            wo_copy(t - (NP0 - NWO)).wait()

        rows = pl.ds(pl.multiple_of(r * TM0, TM0), TM0)
        xv = x_v[rows, :]
        gt = _dot(xv, wg0[half, :, pl.ds(0, FH)])
        up = _dot(xv, wu0[half, :, pl.ds(0, FH)])
        hh = (jnp.maximum(gt, 0.0) * up).astype(_BF16)
        dn = _dot(hh, wd0[half, :, dc])
        acc[rows, :] = dn + jnp.where(half == 1, acc[rows, :], 0.0)
        permute_slice(jnp.where(real, t - (NP0 - NSL), NSL))
        never = lax.broadcasted_iota(jnp.int32, (8, LANES), 1) < -1 - t
        npc = D * WOC // (8 * LANES)
        p1 = vregs(gt) + vregs(up)
        p1 = [p1[i * len(p1) // npc] for i in range(npc)]
        p2 = vregs(dn)
        p2 = [p2[i * 3 * len(p2) // (4 * npc)] for i in range(npc)]
        permute_wo(jnp.where(real_o, t - (NP0 - NWO), NWO), never, p1, p2)
        return carry

    lax.fori_loop(1, NP0, phase0, 0)
    gw_copy().wait()
    for cp in ffn_copies():
        cp.wait()

    c_exp = (DH ** -0.5) * math.log2(math.e)
    neg = -1e9 / (DH ** -0.5)

    def attn_unit(r, row0, gw, never, link, masked):
        def tie(a, b):
            return a if b is None else jnp.where(never, b, a)

        base = r * TM + row0
        qs = [q_s[j, pl.ds(row0, UNIT), :] for j in range(NT)]
        xr = x_v[pl.ds(pl.multiple_of(base, UNIT), UNIT), :].astype(_F32)
        xg = (tie(xr[:, 0:LANES], link) if GATE_TIE == 2 else xr[:, 0:LANES]) * gw[:, 0:LANES]
        for j in range(1, NT):
            cols = slice(j * LANES, (j + 1) * LANES)
            xg = xg + xr[:, cols] * gw[:, cols]
        logits = []
        for w in range(W):
            st = base + (HALO - DIL * w)
            q0 = tie(qs[0], link) if CHAIN_QK else qs[0]
            s = q0 * k_s[0, pl.ds(st, UNIT), :]
            for j in range(1, NT):
                s = s + qs[j] * k_s[j, pl.ds(st, UNIT), :]
            link = s
            s = s + pltpu.roll(s, 64, 1)
            s = s + pltpu.roll(s, 32, 1)
            if masked and w > 0:
                pos = base + lax.broadcasted_iota(jnp.int32, (UNIT, LANES), 0)
                s = jnp.where(pos >= DIL * w, s, neg)
            logits.append(s)
        m = logits[0]
        for w in range(1, W):
            m = jnp.maximum(m, logits[w])
        ps = [jnp.exp2((logits[w] - m) * c_exp) for w in range(W)]
        den = ps[0]
        for w in range(1, W):
            den = den + ps[w]
        gate = jax.nn.sigmoid(jnp.sum(xg, axis=-1, keepdims=True))
        gate = jnp.broadcast_to(gate, (UNIT, LANES))
        g_s[pl.ds(row0, UNIT), :] = 1.0 - gate
        rinv = gate / den
        olink = gate if GATE_TIE else None
        for j in range(NT):
            p0 = tie(ps[0], olink) if CHAIN_PV else ps[0]
            o = p0 * v_s[j, pl.ds(base + HALO, UNIT), :]
            for w in range(1, W):
                o = o + ps[w] * v_s[j, pl.ds(base + (HALO - DIL * w), UNIT), :]
            olink = o
            o_s[pl.ds(row0, UNIT), pl.ds(j * LANES, LANES)] = (
                (o * rinv).astype(_BF16))
        return olink if CHAIN_UNITS == 2 else (link if CHAIN_UNITS else None)

    def row_block(r, carry):
        rows = pl.ds(pl.multiple_of(r * TM, TM), TM)
        krows = pl.ds(pl.multiple_of(r * TM + HALO, HALO), TM)
        xv = x_v[rows, :]
        for sec, dst in enumerate((q_s, k_s, v_s)):
            wsec = wq_p[pl.ds(2 * sec, 2), :, pl.ds(0, D)].reshape(D, D)
            res = _dot(xv, wsec)
            for j in range(NT):
                piece = res[:, j * LANES:(j + 1) * LANES]
                if sec == 0:
                    dst[j] = piece
                else:
                    dst[j, krows, :] = piece
        gw = gw_ref[...].astype(_F32).reshape(1, D)
        never = lax.broadcasted_iota(jnp.int32, (UNIT, LANES), 1) < -1 - r
        links = [None] * NCHAIN
        for un in range(TM // UNIT):
            links[un % NCHAIN] = attn_unit(
                r, un * UNIT, gw, never, links[un % NCHAIN],
                masked=(un * UNIT < HALO))
        for lo, hi in _splits(FCH):
            cols = pl.ds(lo, hi - lo)
            gt = _dot(xv, wg[:, cols])
            up = _dot(xv, wu[:, cols])
            hh = (jnp.maximum(gt, 0.0) * up).astype(_BF16)
            acc[rows, :] += _dot(hh, wd[cols, :])

        ov = o_s[...]
        g1 = g_s[...]
        g1 = jnp.concatenate([g1] * (WOC // LANES), axis=1)
        for n in range(NWO):
            cols = pl.ds(n * WOC, WOC)
            a = _dot(ov, wo_p[n])
            out_st[n][r] = (a + g1 * acc[rows, cols]).astype(_BF16)
            out_copy(r, n).start()
        return carry

    lax.fori_loop(0, NR, row_block, 0)
    for n in range(NWO):
        for r in range(NR):
            out_copy(r, n).wait()


@jax.jit
def pallas_gated_mix__sliding_local_dilated__glu_gated_reglu__prompt_kernel(
    A_x: jax.Array,
    A_wqkv: jax.Array,
    A_wo: jax.Array,
    B_x: jax.Array,
    B_W_gate: jax.Array,
    B_W_up: jax.Array,
    B_W_down: jax.Array,
    gate_w: jax.Array,
):
    del B_x
    B, S, D = A_x.shape
    F = B_W_gate.shape[1]
    assert B == 1 and D == H * DH == NT * LANES
    assert S % TM == 0 and F - F0 == sum(FCH)
    NR = S // TM
    F1 = F - F0
    assert 2 * (S // TM0) >= 8

    n_sems = len(START_LOADS) + S // TM0 + 1 + 6 + D // WOC + 1
    any_spec = pl.BlockSpec(memory_space=pl.ANY)
    out = pl.pallas_call(
        functools.partial(_kernel, S=S, D=D, F=F),
        out_shape=jax.ShapeDtypeStruct((S, D), _BF16),
        in_specs=[any_spec] * 7,
        out_specs=any_spec,
        scratch_shapes=[
            pltpu.VMEM((S, D), _BF16),
            pltpu.VMEM((7, D // 2, D), _BF16),
            pltpu.VMEM((7, D // 2, D + PAD), _BF16),
            pltpu.VMEM((D // WOC + 1, D, WOC), _BF16),
            [pltpu.VMEM((H * (WOP + 1), LANES), _F32)] * (WOC // LANES * DH // 8),
            pltpu.VMEM((D // WOC + 1, D, WOC), _BF16),
            pltpu.VMEM((2, D, FH), _BF16),
            pltpu.VMEM((2, D, FH), _BF16),
            pltpu.VMEM((2, FH, D + PAD), _BF16),
            pltpu.VMEM((D, F1), _BF16),
            pltpu.VMEM((D, F1), _BF16),
            pltpu.VMEM((F1, D), _BF16),
            pltpu.VMEM((S, D), _F32),
            pltpu.VMEM((NT, TM, LANES), _F32),
            pltpu.VMEM((NT, HALO + S, LANES), _F32),
            pltpu.VMEM((NT, HALO + S, LANES), _F32),
            pltpu.VMEM((TM, LANES), _F32),
            pltpu.VMEM((TM, D), _BF16),
            [pltpu.VMEM((NR, TM, WOC), _BF16)] * (D // WOC),
            pltpu.VMEM((D,), _BF16),
            pltpu.SemaphoreType.DMA((n_sems,)),
            pltpu.SemaphoreType.DMA((D // WOC,)),
        ],
        compiler_params=pltpu.CompilerParams(
            vmem_limit_bytes=120 * 1024 * 1024,
            disable_bounds_checks=True,
            disable_semaphore_checks=True),
        name="gated_mix",
    )(A_x.reshape(S, D), A_wqkv, A_wo, B_W_gate, B_W_up, B_W_down,
      gate_w)
    return out.reshape(B, S, D)
```

```python
import functools
import math

import jax
import jax.numpy as jnp
from jax import lax
import jax.experimental.pallas as pl
import jax.experimental.pallas.tpu as pltpu

H = 32
DH = 32
W = 8
DIL = 2
LANES = 128
NT = 8
HALO = 16

TM = 256
TM0 = 512
FH = 384
F0 = 2 * FH
FCH = (768, 768, 640, 640)
UNIT = 8
WOC = 256
WOP = 9
CHAIN_QK = True
CHAIN_PV = True
CHAIN_UNITS = 2
PAD = 128
GATE_TIE = 1
NCHAIN = 1
START_LOADS = (("x", 0, 256), ("g", 0, 128), ("g", 128, 384), ("x", 256, 512),
               ("u", 0, 384), ("d", 0, 1024))
START_STAGES = ((2, (("g", 0, 256, 0, 128),)),
                (1, (("g", 0, 256, 128, 384),)),
                (1, (("g", 256, 512, 0, 384),)),
                (1, (("u", 0, 512, 0, 384),)),
                (1, (("d", 0, 512, 0, 1024),)))
PB = 4

_F32 = jnp.float32
_BF16 = jnp.bfloat16


def _splits(sizes):
    out, lo = [], 0
    for n in sizes:
        out.append((lo, lo + n))
        lo += n
    return out


def _dot(a, b):
    return jnp.dot(a, b, preferred_element_type=_F32)


def _kernel(x_hbm, wqkv_hbm, wo_hbm, wg_hbm, wu_hbm, wd_hbm, gw_hbm, out_hbm,
            x_v, wq_raw, wq_p, wo_raw, wo_f, wo_p, wg0, wu0, wd0, wg, wu, wd,
            acc, q_s, k_s, v_s, g_s, o_s, out_st, gw_ref,
            sems, sem_out,
            *, S, D, F):
    NR = S // TM
    NR0 = S // TM0
    NP0 = 2 * NR0
    F1 = F - F0
    NSL = 6
    HR = D // 2

    dc = pl.ds(0, D)

    NWO = D // WOC
    SW0 = 0
    SX = SW0 + len(START_LOADS)
    SW1 = SX + NR0 - 1
    SG = SW1 + 1
    SQ = SG + 1
    SO = SQ + NSL
    SR = SO + NWO

    def start_copy(i):
        kind, lo, hi = START_LOADS[i]
        sl = pl.ds(lo, hi - lo)
        hs = pl.ds(0, FH)
        if kind == "x":
            src, dst = x_hbm.at[sl, :], x_v.at[sl, :]
        elif kind == "g":
            src, dst = wg_hbm.at[:, sl], wg0.at[0, :, sl]
        elif kind == "u":
            src, dst = wu_hbm.at[:, sl], wu0.at[0, :, sl]
        else:
            src, dst = wd_hbm.at[hs, sl], wd0.at[0, :, sl]
        return pltpu.make_async_copy(src, dst, sems.at[SW0 + i])

    def x_copy(r):
        rows = pl.ds(r * TM0, TM0)
        return pltpu.make_async_copy(
            x_hbm.at[rows, :], x_v.at[rows, :], sems.at[SX + r - 1])

    def w1_copies():
        sem = sems.at[SW1]
        h1 = pl.ds(FH, FH)
        hs = pl.ds(0, FH)
        return (
            pltpu.make_async_copy(wg_hbm.at[:, h1], wg0.at[1, :, hs], sem),
            pltpu.make_async_copy(wu_hbm.at[:, h1], wu0.at[1, :, hs], sem),
            pltpu.make_async_copy(wd_hbm.at[h1, :], wd0.at[1, :, dc], sem),
        )

    def gw_copy():
        return pltpu.make_async_copy(gw_hbm, gw_ref, sems.at[SG])

    def wq_copy(a):
        sec = a // 2
        half = a % 2
        return pltpu.make_async_copy(
            wqkv_hbm.at[pl.ds(half * HR, HR), pl.ds(sec * D, D)],
            wq_raw.at[a], sems.at[SQ + a])

    def wo_copy(n):
        lo = n * WOC
        if not isinstance(n, int):
            lo = pl.multiple_of(lo, LANES)
        return pltpu.make_async_copy(
            wo_hbm.at[:, pl.ds(lo, WOC)], wo_raw.at[n], sems.at[SO + n])

    def ffn_copies():
        sem = sems.at[SR]
        f1 = pl.ds(F0, F1)
        return (
            pltpu.make_async_copy(wg_hbm.at[:, f1], wg, sem),
            pltpu.make_async_copy(wu_hbm.at[:, f1], wu, sem),
            pltpu.make_async_copy(wd_hbm.at[f1, :], wd, sem),
        )

    def out_copy(r, n):
        return pltpu.make_async_copy(
            out_st[n].at[r],
            out_hbm.at[pl.ds(r * TM, TM), pl.ds(n * WOC, WOC)],
            sem_out.at[n])

    for i in range(len(START_LOADS)):
        start_copy(i).start()
    for t in range(1, NP0):
        if t < NR0:
            x_copy(t).start()
        if t == NR0:
            for cp in w1_copies():
                cp.start()
        if t >= NP0 - NSL:
            wq_copy(t - (NP0 - NSL)).start()
        if t >= NP0 - NWO:
            wo_copy(t - (NP0 - NWO)).start()
    gw_copy().start()
    for cp in ffn_copies():
        cp.start()

    zeros_halo = jnp.zeros((HALO, LANES), _F32)
    for j in range(NT):
        k_s[j, pl.ds(0, HALO), :] = zeros_halo
        v_s[j, pl.ds(0, HALO), :] = zeros_halo

    def clear(i, carry):
        rs = pl.ds(pl.multiple_of(i * 32, 32), 32)
        wq_raw[NSL, rs, :] = jnp.zeros((32, D), _BF16)
        rs = pl.ds(pl.multiple_of(i * 64, 64), 64)
        wo_raw[NWO, rs, :] = jnp.zeros((64, WOC), _BF16)
        return carry

    lax.fori_loop(0, HR // 32, clear, 0)

    def permute_slice(a):
        rows = PB * 8
        lane = lax.broadcasted_iota(jnp.int32, (rows, LANES), 1)
        bits = [((lane >> (2 + b)) & 1) == 1 for b in range(3)]
        base_pat = NT * 4 * (lane & 3) + (lane >> 5) + 4 * ((lane >> 2) & 7)
        pats = [(base_pat + 4 * j) & (LANES - 1) for j in range(NT)]
        for g in range(HR // (16 * PB)):
            rs = pl.ds(g * 16 * PB, 16 * PB)
            z = []
            for i in range(NT):
                w = pltpu.bitcast(wq_raw[a, rs, pl.ds(i * LANES, LANES)],
                                  jnp.uint32)
                z.append(w if i == 0 else pltpu.roll(w, 4 * i, 1))
            for b in range(3):
                z = [jnp.where(bits[b], z[(k + (1 << b)) % NT], z[k])
                     for k in range(NT)]
            for j in range(NT):
                y = jnp.take_along_axis(z[(-j) % NT], pats[j], axis=1)
                wq_p[a, rs, pl.ds(j * LANES, LANES)] = pltpu.bitcast(y, _BF16)

    def permute_wo(n, never, pace1, pace2):
        nj = WOC // LANES
        i = 0
        for h in range(H):
            blk = wo_raw[n, pl.ds(h * DH, DH), :].astype(_F32)
            for a in range(DH // 8):
                for j in range(nj):
                    pc = blk[a * 8:(a + 1) * 8, j * LANES:(j + 1) * LANES]
                    pc = jnp.where(never, pace1[i], pc)
                    i += 1
                    wo_f[a * nj + j][pl.ds(h * WOP, 8), :] = pc
        i = 0
        for d in range(DH):
            for b in range(H // 8):
                rws = []
                for j in range(nj):
                    pc = wo_f[(d // 8) * nj + j][
                        pl.ds(b * 8 * WOP + d % 8, 8, stride=WOP), :]
                    pc = jnp.where(never, pace2[i], pc)
                    i += 1
                    rws.append(pc)
                wo_p[n, pl.ds(d * H + b * 8, 8), :] = jnp.concatenate(
                    rws, axis=1).astype(_BF16)

    def vregs(v):
        return [v[i * 8:(i + 1) * 8, n * LANES:(n + 1) * LANES]
                for n in range(v.shape[1] // LANES)
                for i in range(v.shape[0] // 8)]

    done = 0
    parts = {"g": {}, "u": {}}
    hh0 = None

    def assemble(pcs):
        row_los = sorted({k[0] for k in pcs})
        return jnp.concatenate(
            [jnp.concatenate([pcs[k] for k in sorted(pcs) if k[0] == r0], axis=1)
             for r0 in row_los], axis=0)

    for nwait, work in START_STAGES:
        for i in range(done, done + nwait):
            start_copy(i).wait()
        done += nwait
        for kind, r0, r1, c0, c1 in work:
            cols = pl.ds(c0, c1 - c0)
            if kind != "d":
                wref = wg0 if kind == "g" else wu0
                res = _dot(x_v[pl.ds(r0, r1 - r0), :], wref[0, :, cols])
                for rr in range(r0, r1, 256):
                    for cc in range(c0, c1, LANES):
                        parts[kind][(rr, cc)] = res[
                            rr - r0:rr - r0 + 256, cc - c0:cc - c0 + LANES]
            else:
                if hh0 is None:
                    hh0 = (jnp.maximum(assemble(parts["g"]), 0.0)
                           * assemble(parts["u"])).astype(_BF16)
                acc[pl.ds(r0, r1 - r0), cols] = _dot(
                    hh0[r0:r1], wd0[0, :, cols])

    def phase0(t, carry):
        half = (t >= NR0).astype(jnp.int32)
        r = t - half * NR0

        @pl.when(t == NR0)
        def _():
            for cp in w1_copies():
                cp.wait()

        @pl.when(t < NR0)
        def _():
            x_copy(r).wait()

        real = t >= NP0 - NSL

        @pl.when(real)
        def _():
            wq_copy(t - (NP0 - NSL)).wait()

        real_o = t >= NP0 - NWO

        @pl.when(real_o)
        def _():
            wo_copy(t - (NP0 - NWO)).wait()

        rows = pl.ds(pl.multiple_of(r * TM0, TM0), TM0)
        xv = x_v[rows, :]
        gt = _dot(xv, wg0[half, :, pl.ds(0, FH)])
        up = _dot(xv, wu0[half, :, pl.ds(0, FH)])
        hh = (jnp.maximum(gt, 0.0) * up).astype(_BF16)
        dn = _dot(hh, wd0[half, :, dc])
        acc[rows, :] = dn + jnp.where(t >= NR0, acc[rows, :], 0.0)
        permute_slice(jnp.where(real, t - (NP0 - NSL), NSL))
        never = lax.broadcasted_iota(jnp.int32, (8, LANES), 1) < -1 - t
        npc = D * WOC // (8 * LANES)
        p1 = vregs(gt) + vregs(up)
        p1 = [p1[i * len(p1) // npc] for i in range(npc)]
        p2 = vregs(dn)
        p2 = [p2[i * 3 * len(p2) // (4 * npc)] for i in range(npc)]
        permute_wo(jnp.where(real_o, t - (NP0 - NWO), NWO), never, p1, p2)
        return carry

    lax.fori_loop(1, NP0, phase0, 0)
    gw_copy().wait()
    for cp in ffn_copies():
        cp.wait()

    c_exp = (DH ** -0.5) * math.log2(math.e)
    neg = -1e9 / (DH ** -0.5)

    def attn_unit(r, row0, gw, never, link, masked):
        def tie(a, b):
            return a if b is None else jnp.where(never, b, a)

        base = r * TM + row0
        qs = [q_s[j, pl.ds(row0, UNIT), :] for j in range(NT)]
        xr = x_v[pl.ds(pl.multiple_of(base, UNIT), UNIT), :].astype(_F32)
        xg = (tie(xr[:, 0:LANES], link) if GATE_TIE == 2 else xr[:, 0:LANES]) * gw[:, 0:LANES]
        for j in range(1, NT):
            cols = slice(j * LANES, (j + 1) * LANES)
            xg = xg + xr[:, cols] * gw[:, cols]
        logits = []
        for w in range(W):
            st = base + (HALO - DIL * w)
            q0 = tie(qs[0], link) if CHAIN_QK else qs[0]
            s = q0 * k_s[0, pl.ds(st, UNIT), :]
            for j in range(1, NT):
                s = s + qs[j] * k_s[j, pl.ds(st, UNIT), :]
            link = s
            s = s + pltpu.roll(s, 64, 1)
            s = s + pltpu.roll(s, 32, 1)
            if masked and w > 0:
                pos = base + lax.broadcasted_iota(jnp.int32, (UNIT, LANES), 0)
                s = jnp.where(pos >= DIL * w, s, neg)
            logits.append(s)
        m = logits[0]
        for w in range(1, W):
            m = jnp.maximum(m, logits[w])
        ps = [jnp.exp2((logits[w] - m) * c_exp) for w in range(W)]
        den = ps[0]
        for w in range(1, W):
            den = den + ps[w]
        gate = jax.nn.sigmoid(jnp.sum(xg, axis=-1, keepdims=True))
        gate = jnp.broadcast_to(gate, (UNIT, LANES))
        g_s[pl.ds(row0, UNIT), :] = 1.0 - gate
        rinv = gate / den
        olink = gate if GATE_TIE else None
        for j in range(NT):
            p0 = tie(ps[0], olink) if CHAIN_PV else ps[0]
            o = p0 * v_s[j, pl.ds(base + HALO, UNIT), :]
            for w in range(1, W):
                o = o + ps[w] * v_s[j, pl.ds(base + (HALO - DIL * w), UNIT), :]
            olink = o
            o_s[pl.ds(row0, UNIT), pl.ds(j * LANES, LANES)] = (
                (o * rinv).astype(_BF16))
        return olink if CHAIN_UNITS == 2 else (link if CHAIN_UNITS else None)

    def row_block(r, carry):
        rows = pl.ds(pl.multiple_of(r * TM, TM), TM)
        krows = pl.ds(pl.multiple_of(r * TM + HALO, HALO), TM)
        xv = x_v[rows, :]
        for sec, dst in enumerate((q_s, k_s, v_s)):
            wsec = wq_p[pl.ds(2 * sec, 2), :, pl.ds(0, D)].reshape(D, D)
            res = _dot(xv, wsec)
            for j in range(NT):
                piece = res[:, j * LANES:(j + 1) * LANES]
                if sec == 0:
                    dst[j] = piece
                else:
                    dst[j, krows, :] = piece
        gw = gw_ref[...].astype(_F32).reshape(1, D)
        never = lax.broadcasted_iota(jnp.int32, (UNIT, LANES), 1) < -1 - r
        links = [None] * NCHAIN
        for un in range(TM // UNIT):
            links[un % NCHAIN] = attn_unit(
                r, un * UNIT, gw, never, links[un % NCHAIN],
                masked=(un * UNIT < HALO))
        for lo, hi in _splits(FCH):
            cols = pl.ds(lo, hi - lo)
            gt = _dot(xv, wg[:, cols])
            up = _dot(xv, wu[:, cols])
            hh = (jnp.maximum(gt, 0.0) * up).astype(_BF16)
            acc[rows, :] += _dot(hh, wd[cols, :])

        ov = o_s[...]
        g1 = g_s[...]
        g1 = jnp.concatenate([g1] * (WOC // LANES), axis=1)
        for n in range(NWO):
            cols = pl.ds(n * WOC, WOC)
            a = _dot(ov, wo_p[n])
            out_st[n][r] = (a + g1 * acc[rows, cols]).astype(_BF16)
            out_copy(r, n).start()
        return carry

    lax.fori_loop(0, NR, row_block, 0)
    for n in range(NWO):
        for r in range(NR):
            out_copy(r, n).wait()


@jax.jit
def pallas_gated_mix__sliding_local_dilated__glu_gated_reglu__prompt_kernel(
    A_x: jax.Array,
    A_wqkv: jax.Array,
    A_wo: jax.Array,
    B_x: jax.Array,
    B_W_gate: jax.Array,
    B_W_up: jax.Array,
    B_W_down: jax.Array,
    gate_w: jax.Array,
):
    del B_x
    B, S, D = A_x.shape
    F = B_W_gate.shape[1]
    assert B == 1 and D == H * DH == NT * LANES
    assert S % TM == 0 and F - F0 == sum(FCH)
    NR = S // TM
    F1 = F - F0
    assert 2 * (S // TM0) >= 8

    n_sems = len(START_LOADS) + S // TM0 + 1 + 6 + D // WOC + 1
    any_spec = pl.BlockSpec(memory_space=pl.ANY)
    out = pl.pallas_call(
        functools.partial(_kernel, S=S, D=D, F=F),
        out_shape=jax.ShapeDtypeStruct((S, D), _BF16),
        in_specs=[any_spec] * 7,
        out_specs=any_spec,
        scratch_shapes=[
            pltpu.VMEM((S, D), _BF16),
            pltpu.VMEM((7, D // 2, D), _BF16),
            pltpu.VMEM((7, D // 2, D + PAD), _BF16),
            pltpu.VMEM((D // WOC + 1, D, WOC), _BF16),
            [pltpu.VMEM((H * (WOP + 1), LANES), _F32)] * (WOC // LANES * DH // 8),
            pltpu.VMEM((D // WOC + 1, D, WOC), _BF16),
            pltpu.VMEM((2, D, FH), _BF16),
            pltpu.VMEM((2, D, FH), _BF16),
            pltpu.VMEM((2, FH, D + PAD), _BF16),
            pltpu.VMEM((D, F1), _BF16),
            pltpu.VMEM((D, F1), _BF16),
            pltpu.VMEM((F1, D), _BF16),
            pltpu.VMEM((S, D), _F32),
            pltpu.VMEM((NT, TM, LANES), _F32),
            pltpu.VMEM((NT, HALO + S, LANES), _F32),
            pltpu.VMEM((NT, HALO + S, LANES), _F32),
            pltpu.VMEM((TM, LANES), _F32),
            pltpu.VMEM((TM, D), _BF16),
            [pltpu.VMEM((NR, TM, WOC), _BF16)] * (D // WOC),
            pltpu.VMEM((D,), _BF16),
            pltpu.SemaphoreType.DMA((n_sems,)),
            pltpu.SemaphoreType.DMA((D // WOC,)),
        ],
        compiler_params=pltpu.CompilerParams(
            vmem_limit_bytes=120 * 1024 * 1024,
            disable_bounds_checks=True,
            disable_semaphore_checks=True),
        name="gated_mix",
    )(A_x.reshape(S, D), A_wqkv, A_wo, B_W_gate, B_W_up, B_W_down,
      gate_w)
    return out.reshape(B, S, D)
```

```python
import functools
import math

import jax
import jax.numpy as jnp
from jax import lax
import jax.experimental.pallas as pl
import jax.experimental.pallas.tpu as pltpu

H = 32
DH = 32
W = 8
DIL = 2
LANES = 128
NT = 8
HALO = 16

TM = 256
TM0 = 512
FH = 384
F0 = 2 * FH
FCH = (2816,)
UNIT = 8
WOC = 256
WOP = 9
CHAIN_QK = True
CHAIN_PV = True
CHAIN_UNITS = 2
PAD = 128
GATE_TIE = 1
NCHAIN = 1
START_LOADS = (("x", 0, 256), ("g", 0, 128), ("g", 128, 384), ("x", 256, 512),
               ("u", 0, 384), ("d", 0, 1024))
START_STAGES = ((2, (("g", 0, 256, 0, 128),)),
                (1, (("g", 0, 256, 128, 384),)),
                (1, (("g", 256, 512, 0, 384),)),
                (1, (("u", 0, 512, 0, 384),)),
                (1, (("d", 0, 512, 0, 1024),)))
OUT_PIECES = ((0, 256, 0, 256), (0, 256, 256, 512), (0, 256, 512, 768),
              (0, 256, 768, 896), (0, 128, 896, 1024), (128, 256, 896, 1024))
PB = 4

_F32 = jnp.float32
_BF16 = jnp.bfloat16


def _splits(sizes):
    out, lo = [], 0
    for n in sizes:
        out.append((lo, lo + n))
        lo += n
    return out


def _dot(a, b):
    return jnp.dot(a, b, preferred_element_type=_F32)


def _kernel(x_hbm, wqkv_hbm, wo_hbm, wg_hbm, wu_hbm, wd_hbm, gw_hbm, out_hbm,
            x_v, wq_raw, wq_p, wo_raw, wo_f, wo_p, wg0, wu0, wd0, wg, wu, wd,
            acc, q_s, k_s, v_s, g_s, o_s, out_st, gw_ref,
            sems, sem_out,
            *, S, D, F):
    NR = S // TM
    NR0 = S // TM0
    NP0 = 2 * NR0
    F1 = F - F0
    NSL = 6
    HR = D // 2

    dc = pl.ds(0, D)

    NWO = D // WOC
    SW0 = 0
    SX = SW0 + len(START_LOADS)
    SW1 = SX + NR0 - 1
    SG = SW1 + 1
    SQ = SG + 1
    SO = SQ + NSL
    SR = SO + NWO

    def start_copy(i):
        kind, lo, hi = START_LOADS[i]
        sl = pl.ds(lo, hi - lo)
        hs = pl.ds(0, FH)
        if kind == "x":
            src, dst = x_hbm.at[sl, :], x_v.at[sl, :]
        elif kind == "g":
            src, dst = wg_hbm.at[:, sl], wg0.at[0, :, sl]
        elif kind == "u":
            src, dst = wu_hbm.at[:, sl], wu0.at[0, :, sl]
        else:
            src, dst = wd_hbm.at[hs, sl], wd0.at[0, :, sl]
        return pltpu.make_async_copy(src, dst, sems.at[SW0 + i])

    def x_copy(r):
        rows = pl.ds(r * TM0, TM0)
        return pltpu.make_async_copy(
            x_hbm.at[rows, :], x_v.at[rows, :], sems.at[SX + r - 1])

    def w1_copies():
        sem = sems.at[SW1]
        h1 = pl.ds(FH, FH)
        hs = pl.ds(0, FH)
        return (
            pltpu.make_async_copy(wg_hbm.at[:, h1], wg0.at[1, :, hs], sem),
            pltpu.make_async_copy(wu_hbm.at[:, h1], wu0.at[1, :, hs], sem),
            pltpu.make_async_copy(wd_hbm.at[h1, :], wd0.at[1, :, dc], sem),
        )

    def gw_copy():
        return pltpu.make_async_copy(gw_hbm, gw_ref, sems.at[SG])

    def wq_copy(a):
        sec = a // 2
        half = a % 2
        return pltpu.make_async_copy(
            wqkv_hbm.at[pl.ds(half * HR, HR), pl.ds(sec * D, D)],
            wq_raw.at[a], sems.at[SQ + a])

    def wo_copy(n):
        lo = n * WOC
        if not isinstance(n, int):
            lo = pl.multiple_of(lo, LANES)
        return pltpu.make_async_copy(
            wo_hbm.at[:, pl.ds(lo, WOC)], wo_raw.at[n], sems.at[SO + n])

    def ffn_copies():
        sem = sems.at[SR]
        f1 = pl.ds(F0, F1)
        return (
            pltpu.make_async_copy(wg_hbm.at[:, f1], wg, sem),
            pltpu.make_async_copy(wu_hbm.at[:, f1], wu, sem),
            pltpu.make_async_copy(wd_hbm.at[f1, :], wd, sem),
        )

    def out_copy(r, i):
        r0, r1, c0, c1 = OUT_PIECES[i]
        return pltpu.make_async_copy(
            out_st[i].at[r],
            out_hbm.at[pl.ds(r * TM + r0, r1 - r0), pl.ds(c0, c1 - c0)],
            sem_out.at[i])

    for i in range(len(START_LOADS)):
        start_copy(i).start()
    for t in range(1, NP0):
        if t < NR0:
            x_copy(t).start()
        if t == NR0:
            for cp in w1_copies():
                cp.start()
        if t >= NP0 - NSL:
            wq_copy(t - (NP0 - NSL)).start()
        if t >= NP0 - NWO:
            wo_copy(t - (NP0 - NWO)).start()
    gw_copy().start()
    for cp in ffn_copies():
        cp.start()

    zeros_halo = jnp.zeros((HALO, LANES), _F32)
    for j in range(NT):
        k_s[j, pl.ds(0, HALO), :] = zeros_halo
        v_s[j, pl.ds(0, HALO), :] = zeros_halo

    def clear(i, carry):
        rs = pl.ds(pl.multiple_of(i * 32, 32), 32)
        wq_raw[NSL, rs, :] = jnp.zeros((32, D), _BF16)
        rs = pl.ds(pl.multiple_of(i * 64, 64), 64)
        wo_raw[NWO, rs, :] = jnp.zeros((64, WOC), _BF16)
        return carry

    lax.fori_loop(0, HR // 32, clear, 0)

    def permute_slice(a):
        rows = PB * 8
        lane = lax.broadcasted_iota(jnp.int32, (rows, LANES), 1)
        bits = [((lane >> (2 + b)) & 1) == 1 for b in range(3)]
        base_pat = NT * 4 * (lane & 3) + (lane >> 5) + 4 * ((lane >> 2) & 7)
        pats = [(base_pat + 4 * j) & (LANES - 1) for j in range(NT)]
        for g in range(HR // (16 * PB)):
            rs = pl.ds(g * 16 * PB, 16 * PB)
            z = []
            for i in range(NT):
                w = pltpu.bitcast(wq_raw[a, rs, pl.ds(i * LANES, LANES)],
                                  jnp.uint32)
                z.append(w if i == 0 else pltpu.roll(w, 4 * i, 1))
            for b in range(3):
                z = [jnp.where(bits[b], z[(k + (1 << b)) % NT], z[k])
                     for k in range(NT)]
            for j in range(NT):
                y = jnp.take_along_axis(z[(-j) % NT], pats[j], axis=1)
                wq_p[a, rs, pl.ds(j * LANES, LANES)] = pltpu.bitcast(y, _BF16)

    def permute_wo(n, never, pace1, pace2):
        nj = WOC // LANES
        i = 0
        for h in range(H):
            blk = wo_raw[n, pl.ds(h * DH, DH), :].astype(_F32)
            for a in range(DH // 8):
                for j in range(nj):
                    pc = blk[a * 8:(a + 1) * 8, j * LANES:(j + 1) * LANES]
                    pc = jnp.where(never, pace1[i], pc)
                    i += 1
                    wo_f[a * nj + j][pl.ds(h * WOP, 8), :] = pc
        i = 0
        for d in range(DH):
            for b in range(H // 8):
                rws = []
                for j in range(nj):
                    pc = wo_f[(d // 8) * nj + j][
                        pl.ds(b * 8 * WOP + d % 8, 8, stride=WOP), :]
                    pc = jnp.where(never, pace2[i], pc)
                    i += 1
                    rws.append(pc)
                wo_p[n, pl.ds(d * H + b * 8, 8), :] = jnp.concatenate(
                    rws, axis=1).astype(_BF16)

    def vregs(v):
        return [v[i * 8:(i + 1) * 8, n * LANES:(n + 1) * LANES]
                for n in range(v.shape[1] // LANES)
                for i in range(v.shape[0] // 8)]

    done = 0
    parts = {"g": {}, "u": {}}
    hh0 = None

    def assemble(pcs):
        row_los = sorted({k[0] for k in pcs})
        return jnp.concatenate(
            [jnp.concatenate([pcs[k] for k in sorted(pcs) if k[0] == r0], axis=1)
             for r0 in row_los], axis=0)

    for nwait, work in START_STAGES:
        for i in range(done, done + nwait):
            start_copy(i).wait()
        done += nwait
        for kind, r0, r1, c0, c1 in work:
            cols = pl.ds(c0, c1 - c0)
            if kind != "d":
                wref = wg0 if kind == "g" else wu0
                res = _dot(x_v[pl.ds(r0, r1 - r0), :], wref[0, :, cols])
                for rr in range(r0, r1, 256):
                    for cc in range(c0, c1, LANES):
                        parts[kind][(rr, cc)] = res[
                            rr - r0:rr - r0 + 256, cc - c0:cc - c0 + LANES]
            else:
                if hh0 is None:
                    hh0 = (jnp.maximum(assemble(parts["g"]), 0.0)
                           * assemble(parts["u"])).astype(_BF16)
                acc[pl.ds(r0, r1 - r0), cols] = _dot(
                    hh0[r0:r1], wd0[0, :, cols])

    def phase0(t, carry):
        half = (t >= NR0).astype(jnp.int32)
        r = t - half * NR0

        @pl.when(t == NR0)
        def _():
            for cp in w1_copies():
                cp.wait()

        @pl.when(t < NR0)
        def _():
            x_copy(r).wait()

        real = t >= NP0 - NSL

        @pl.when(real)
        def _():
            wq_copy(t - (NP0 - NSL)).wait()

        real_o = t >= NP0 - NWO

        @pl.when(real_o)
        def _():
            wo_copy(t - (NP0 - NWO)).wait()

        rows = pl.ds(pl.multiple_of(r * TM0, TM0), TM0)
        xv = x_v[rows, :]
        gt = _dot(xv, wg0[half, :, pl.ds(0, FH)])
        up = _dot(xv, wu0[half, :, pl.ds(0, FH)])
        hh = (jnp.maximum(gt, 0.0) * up).astype(_BF16)
        dn = _dot(hh, wd0[half, :, dc])
        acc[rows, :] = dn + jnp.where(t >= NR0, acc[rows, :], 0.0)
        permute_slice(jnp.where(real, t - (NP0 - NSL), NSL))
        never = lax.broadcasted_iota(jnp.int32, (8, LANES), 1) < -1 - t
        npc = D * WOC // (8 * LANES)
        p1 = vregs(gt) + vregs(up)
        p1 = [p1[i * len(p1) // npc] for i in range(npc)]
        p2 = vregs(dn)
        p2 = [p2[i * 3 * len(p2) // (4 * npc)] for i in range(npc)]
        permute_wo(jnp.where(real_o, t - (NP0 - NWO), NWO), never, p1, p2)
        return carry

    lax.fori_loop(1, NP0, phase0, 0)
    gw_copy().wait()
    for cp in ffn_copies():
        cp.wait()

    c_exp = (DH ** -0.5) * math.log2(math.e)
    neg = -1e9 / (DH ** -0.5)

    def attn_unit(r, row0, gw, never, link, masked):
        def tie(a, b):
            return a if b is None else jnp.where(never, b, a)

        base = r * TM + row0
        qs = [q_s[j, pl.ds(row0, UNIT), :] for j in range(NT)]
        xr = x_v[pl.ds(pl.multiple_of(base, UNIT), UNIT), :].astype(_F32)
        xg = (tie(xr[:, 0:LANES], link) if GATE_TIE == 2 else xr[:, 0:LANES]) * gw[:, 0:LANES]
        for j in range(1, NT):
            cols = slice(j * LANES, (j + 1) * LANES)
            xg = xg + xr[:, cols] * gw[:, cols]
        logits = []
        for w in range(W):
            st = base + (HALO - DIL * w)
            q0 = tie(qs[0], link) if CHAIN_QK else qs[0]
            s = q0 * k_s[0, pl.ds(st, UNIT), :]
            for j in range(1, NT):
                s = s + qs[j] * k_s[j, pl.ds(st, UNIT), :]
            link = s
            s = s + pltpu.roll(s, 64, 1)
            s = s + pltpu.roll(s, 32, 1)
            if masked and w > 0:
                pos = base + lax.broadcasted_iota(jnp.int32, (UNIT, LANES), 0)
                s = jnp.where(pos >= DIL * w, s, neg)
            logits.append(s)
        m = logits[0]
        for w in range(1, W):
            m = jnp.maximum(m, logits[w])
        ps = [jnp.exp2((logits[w] - m) * c_exp) for w in range(W)]
        den = ps[0]
        for w in range(1, W):
            den = den + ps[w]
        gate = jax.nn.sigmoid(jnp.sum(xg, axis=-1, keepdims=True))
        gate = jnp.broadcast_to(gate, (UNIT, LANES))
        g_s[pl.ds(row0, UNIT), :] = 1.0 - gate
        rinv = gate / den
        olink = gate if GATE_TIE else None
        for j in range(NT):
            p0 = tie(ps[0], olink) if CHAIN_PV else ps[0]
            o = p0 * v_s[j, pl.ds(base + HALO, UNIT), :]
            for w in range(1, W):
                o = o + ps[w] * v_s[j, pl.ds(base + (HALO - DIL * w), UNIT), :]
            olink = o
            o_s[pl.ds(row0, UNIT), pl.ds(j * LANES, LANES)] = (
                (o * rinv).astype(_BF16))
        return olink if CHAIN_UNITS == 2 else (link if CHAIN_UNITS else None)

    def row_block(r, carry):
        rows = pl.ds(pl.multiple_of(r * TM, TM), TM)
        krows = pl.ds(pl.multiple_of(r * TM + HALO, HALO), TM)
        xv = x_v[rows, :]
        for sec, dst in enumerate((q_s, k_s, v_s)):
            wsec = wq_p[pl.ds(2 * sec, 2), :, pl.ds(0, D)].reshape(D, D)
            res = _dot(xv, wsec)
            for j in range(NT):
                piece = res[:, j * LANES:(j + 1) * LANES]
                if sec == 0:
                    dst[j] = piece
                else:
                    dst[j, krows, :] = piece
        gw = gw_ref[...].astype(_F32).reshape(1, D)
        never = lax.broadcasted_iota(jnp.int32, (UNIT, LANES), 1) < -1 - r
        links = [None] * NCHAIN
        for un in range(TM // UNIT):
            links[un % NCHAIN] = attn_unit(
                r, un * UNIT, gw, never, links[un % NCHAIN],
                masked=(un * UNIT < HALO))
        for lo, hi in _splits(FCH):
            cols = pl.ds(lo, hi - lo)
            gt = _dot(xv, wg[:, cols])
            up = _dot(xv, wu[:, cols])
            hh = (jnp.maximum(gt, 0.0) * up).astype(_BF16)
            acc[rows, :] += _dot(hh, wd[cols, :])

        ov = o_s[...]
        g1 = g_s[...]
        g1 = jnp.concatenate([g1] * (WOC // LANES), axis=1)
        for n in range(NWO):
            cols = pl.ds(n * WOC, WOC)
            a = _dot(ov, wo_p[n])
            res = (a + g1 * acc[rows, cols]).astype(_BF16)
            for i, (r0, r1, c0, c1) in enumerate(OUT_PIECES):
                if c0 // WOC == n:
                    out_st[i][r] = res[r0:r1, c0 - n * WOC:c1 - n * WOC]
                    out_copy(r, i).start()
        return carry

    lax.fori_loop(0, NR, row_block, 0)
    for i in range(len(OUT_PIECES)):
        for r in range(NR):
            out_copy(r, i).wait()


@jax.jit
def pallas_gated_mix__sliding_local_dilated__glu_gated_reglu__prompt_kernel(
    A_x: jax.Array,
    A_wqkv: jax.Array,
    A_wo: jax.Array,
    B_x: jax.Array,
    B_W_gate: jax.Array,
    B_W_up: jax.Array,
    B_W_down: jax.Array,
    gate_w: jax.Array,
):
    del B_x
    B, S, D = A_x.shape
    F = B_W_gate.shape[1]
    assert B == 1 and D == H * DH == NT * LANES
    assert S % TM == 0 and F - F0 == sum(FCH)
    NR = S // TM
    F1 = F - F0
    assert 2 * (S // TM0) >= 8

    n_sems = len(START_LOADS) + S // TM0 + 1 + 6 + D // WOC + 1
    any_spec = pl.BlockSpec(memory_space=pl.ANY)
    out = pl.pallas_call(
        functools.partial(_kernel, S=S, D=D, F=F),
        out_shape=jax.ShapeDtypeStruct((S, D), _BF16),
        in_specs=[any_spec] * 7,
        out_specs=any_spec,
        scratch_shapes=[
            pltpu.VMEM((S, D), _BF16),
            pltpu.VMEM((7, D // 2, D), _BF16),
            pltpu.VMEM((7, D // 2, D + PAD), _BF16),
            pltpu.VMEM((D // WOC + 1, D, WOC), _BF16),
            [pltpu.VMEM((H * (WOP + 1), LANES), _F32)] * (WOC // LANES * DH // 8),
            pltpu.VMEM((D // WOC + 1, D, WOC), _BF16),
            pltpu.VMEM((2, D, FH), _BF16),
            pltpu.VMEM((2, D, FH), _BF16),
            pltpu.VMEM((2, FH, D + PAD), _BF16),
            pltpu.VMEM((D, F1), _BF16),
            pltpu.VMEM((D, F1), _BF16),
            pltpu.VMEM((F1, D), _BF16),
            pltpu.VMEM((S, D), _F32),
            pltpu.VMEM((NT, TM, LANES), _F32),
            pltpu.VMEM((NT, HALO + S, LANES), _F32),
            pltpu.VMEM((NT, HALO + S, LANES), _F32),
            pltpu.VMEM((TM, LANES), _F32),
            pltpu.VMEM((TM, D), _BF16),
            [pltpu.VMEM((NR, r1 - r0, c1 - c0), _BF16)
             for r0, r1, c0, c1 in OUT_PIECES],
            pltpu.VMEM((D,), _BF16),
            pltpu.SemaphoreType.DMA((n_sems,)),
            pltpu.SemaphoreType.DMA((len(OUT_PIECES),)),
        ],
        compiler_params=pltpu.CompilerParams(
            vmem_limit_bytes=120 * 1024 * 1024,
            disable_bounds_checks=True,
            disable_semaphore_checks=True),
        name="gated_mix",
    )(A_x.reshape(S, D), A_wqkv, A_wo, B_W_gate, B_W_up, B_W_down,
      gate_w)
    return out.reshape(B, S, D)
```

```python
import functools
import math

import jax
import jax.numpy as jnp
from jax import lax
import jax.experimental.pallas as pl
import jax.experimental.pallas.tpu as pltpu

H = 32
DH = 32
W = 8
DIL = 2
LANES = 128
NT = 8
HALO = 16

TM = 256
TM0 = 1024
FH = 256
NG = 3
F0 = NG * FH
NSL = 4
FCH = (2816,)
UNIT = 8
WOC = 256
WOP = 9
CHAIN_QK = True
CHAIN_PV = True
CHAIN_UNITS = 2
PAD = 128
GATE_TIE = 1
NCHAIN = 1
START_LOADS = (("x", 0, 256), ("g", 0, 128), ("g", 128, 256), ("x", 256, 512),
               ("u", 0, 256), ("x", 512, 1024), ("d", 0, 1024))
START_STAGES = ((2, (("g", 0, 256, 0, 128),)),
                (1, (("g", 0, 256, 128, 256),)),
                (1, (("g", 256, 512, 0, 256),)),
                (1, (("u", 0, 512, 0, 256),)),
                (1, (("g", 512, 1024, 0, 256), ("u", 512, 1024, 0, 256))),
                (1, (("d", 0, 1024, 0, 1024),)))
OUT_PIECES = ((0, 256, 0, 256), (0, 256, 256, 512), (0, 256, 512, 768),
              (0, 256, 768, 896), (0, 128, 896, 1024), (128, 256, 896, 1024))
PB = 4

_F32 = jnp.float32
_BF16 = jnp.bfloat16


def _splits(sizes):
    out, lo = [], 0
    for n in sizes:
        out.append((lo, lo + n))
        lo += n
    return out


def _dot(a, b):
    return jnp.dot(a, b, preferred_element_type=_F32)


def _kernel(x_hbm, wqkv_hbm, wo_hbm, wg_hbm, wu_hbm, wd_hbm, gw_hbm, out_hbm,
            x_v, wq_raw, wq_p, wo_raw, wo_f, wo_p, wg0, wu0, wd0, wg, wu, wd,
            acc, q_s, k_s, v_s, g_s, o_s, out_st, gw_ref,
            sems, sem_out,
            *, S, D, F):
    NR = S // TM
    NR0 = S // TM0
    NP0 = NG * NR0
    F1 = F - F0
    HR = 3 * D // NSL

    dc = pl.ds(0, D)

    NWO = D // WOC
    SW0 = 0
    SX = SW0 + len(START_LOADS)
    SW1 = SX + NR0 - 1
    SG = SW1 + NG - 1
    SQ = SG + 1
    SO = SQ + NSL
    SR = SO + NWO

    def start_copy(i):
        kind, lo, hi = START_LOADS[i]
        sl = pl.ds(lo, hi - lo)
        hs = pl.ds(0, FH)
        if kind == "x":
            src, dst = x_hbm.at[sl, :], x_v.at[sl, :]
        elif kind == "g":
            src, dst = wg_hbm.at[:, sl], wg0.at[0, :, sl]
        elif kind == "u":
            src, dst = wu_hbm.at[:, sl], wu0.at[0, :, sl]
        else:
            src, dst = wd_hbm.at[hs, sl], wd0.at[0, :, sl]
        return pltpu.make_async_copy(src, dst, sems.at[SW0 + i])

    def x_copy(r):
        rows = pl.ds(r * TM0, TM0)
        return pltpu.make_async_copy(
            x_hbm.at[rows, :], x_v.at[rows, :], sems.at[SX + r - 1])

    def w1_copies(gi):
        sem = sems.at[SW1 + gi - 1]
        lo = gi * FH
        if not isinstance(gi, int):
            lo = pl.multiple_of(lo, LANES)
        h1 = pl.ds(lo, FH)
        hs = pl.ds(0, FH)
        return (
            pltpu.make_async_copy(wg_hbm.at[:, h1], wg0.at[gi, :, hs], sem),
            pltpu.make_async_copy(wu_hbm.at[:, h1], wu0.at[gi, :, hs], sem),
            pltpu.make_async_copy(wd_hbm.at[h1, :], wd0.at[gi, :, dc], sem),
        )

    def gw_copy():
        return pltpu.make_async_copy(gw_hbm, gw_ref, sems.at[SG])

    def wq_copies(a):
        cps = []
        lo, hi = a * HR, (a + 1) * HR
        while lo < hi:
            sec = lo // D
            nxt = min(hi, (sec + 1) * D)
            cps.append(pltpu.make_async_copy(
                wqkv_hbm.at[pl.ds(lo - sec * D, nxt - lo), pl.ds(sec * D, D)],
                wq_raw.at[a, pl.ds(lo - a * HR, nxt - lo), :], sems.at[SQ + a]))
            lo = nxt
        return cps

    def wq_wait(a):
        pltpu.make_async_copy(
            wq_raw.at[a], wq_raw.at[a], sems.at[SQ + a]).wait()

    def wo_copy(n):
        lo = n * WOC
        if not isinstance(n, int):
            lo = pl.multiple_of(lo, LANES)
        return pltpu.make_async_copy(
            wo_hbm.at[:, pl.ds(lo, WOC)], wo_raw.at[n], sems.at[SO + n])

    def ffn_copies():
        sem = sems.at[SR]
        f1 = pl.ds(F0, F1)
        return (
            pltpu.make_async_copy(wg_hbm.at[:, f1], wg, sem),
            pltpu.make_async_copy(wu_hbm.at[:, f1], wu, sem),
            pltpu.make_async_copy(wd_hbm.at[f1, :], wd, sem),
        )

    def out_copy(r, i):
        r0, r1, c0, c1 = OUT_PIECES[i]
        return pltpu.make_async_copy(
            out_st[i].at[r],
            out_hbm.at[pl.ds(r * TM + r0, r1 - r0), pl.ds(c0, c1 - c0)],
            sem_out.at[i])

    for i in range(len(START_LOADS)):
        start_copy(i).start()
    for t in range(1, NP0):
        if t < NR0:
            x_copy(t).start()
        if t % NR0 == 0:
            for cp in w1_copies(t // NR0):
                cp.start()
        if t >= NP0 - NSL:
            for cp in wq_copies(t - (NP0 - NSL)):
                cp.start()
        if t >= NP0 - NWO:
            wo_copy(t - (NP0 - NWO)).start()
    gw_copy().start()
    for cp in ffn_copies():
        cp.start()

    zeros_halo = jnp.zeros((HALO, LANES), _F32)
    for j in range(NT):
        k_s[j, pl.ds(0, HALO), :] = zeros_halo
        v_s[j, pl.ds(0, HALO), :] = zeros_halo

    def clear(i, carry):
        rs = pl.ds(pl.multiple_of(i * 48, 16), 48)
        wq_raw[NSL, rs, :] = jnp.zeros((48, D), _BF16)
        rs = pl.ds(pl.multiple_of(i * 64, 64), 64)
        wo_raw[NWO, rs, :] = jnp.zeros((64, WOC), _BF16)
        return carry

    lax.fori_loop(0, 16, clear, 0)

    def permute_slice(a):
        rows = PB * 8
        lane = lax.broadcasted_iota(jnp.int32, (rows, LANES), 1)
        bits = [((lane >> (2 + b)) & 1) == 1 for b in range(3)]
        base_pat = NT * 4 * (lane & 3) + (lane >> 5) + 4 * ((lane >> 2) & 7)
        pats = [(base_pat + 4 * j) & (LANES - 1) for j in range(NT)]
        for g in range(HR // (16 * PB)):
            rs = pl.ds(g * 16 * PB, 16 * PB)
            rp = pl.ds(g * 8 * PB, 8 * PB)
            z = []
            for i in range(NT):
                w = pltpu.bitcast(wq_raw[a, rs, pl.ds(i * LANES, LANES)],
                                  jnp.uint32)
                z.append(w if i == 0 else pltpu.roll(w, 4 * i, 1))
            for b in range(3):
                z = [jnp.where(bits[b], z[(k + (1 << b)) % NT], z[k])
                     for k in range(NT)]
            for j in range(NT):
                y = jnp.take_along_axis(z[(-j) % NT], pats[j], axis=1)
                wq_p[a, rp, pl.ds(j * LANES, LANES)] = y

    def permute_wo(n, never, pace1, pace2):
        nj = WOC // LANES
        i = 0
        for h in range(H):
            blk = wo_raw[n, pl.ds(h * DH, DH), :].astype(_F32)
            for a in range(DH // 8):
                for j in range(nj):
                    pc = blk[a * 8:(a + 1) * 8, j * LANES:(j + 1) * LANES]
                    pc = jnp.where(never, pace1[i], pc)
                    i += 1
                    wo_f[a * nj + j][pl.ds(h * WOP, 8), :] = pc
        i = 0
        for d in range(DH):
            for b in range(H // 8):
                rws = []
                for j in range(nj):
                    pc = wo_f[(d // 8) * nj + j][
                        pl.ds(b * 8 * WOP + d % 8, 8, stride=WOP), :]
                    pc = jnp.where(never, pace2[i], pc)
                    i += 1
                    rws.append(pc)
                wo_p[n, pl.ds(d * H + b * 8, 8), :] = jnp.concatenate(
                    rws, axis=1).astype(_BF16)

    def vregs(v):
        return [v[i * 8:(i + 1) * 8, n * LANES:(n + 1) * LANES]
                for n in range(v.shape[1] // LANES)
                for i in range(v.shape[0] // 8)]

    done = 0
    parts = {"g": {}, "u": {}}
    hh0 = None

    def assemble(pcs):
        row_los = sorted({k[0] for k in pcs})
        return jnp.concatenate(
            [jnp.concatenate([pcs[k] for k in sorted(pcs) if k[0] == r0], axis=1)
             for r0 in row_los], axis=0)

    for nwait, work in START_STAGES:
        for i in range(done, done + nwait):
            start_copy(i).wait()
        done += nwait
        for kind, r0, r1, c0, c1 in work:
            cols = pl.ds(c0, c1 - c0)
            if kind != "d":
                wref = wg0 if kind == "g" else wu0
                res = _dot(x_v[pl.ds(r0, r1 - r0), :], wref[0, :, cols])
                for rr in range(r0, r1, 256):
                    for cc in range(c0, c1, LANES):
                        parts[kind][(rr, cc)] = res[
                            rr - r0:rr - r0 + 256, cc - c0:cc - c0 + LANES]
            else:
                if hh0 is None:
                    hh0 = (jnp.maximum(assemble(parts["g"]), 0.0)
                           * assemble(parts["u"])).astype(_BF16)
                acc[pl.ds(r0, r1 - r0), cols] = _dot(
                    hh0[r0:r1], wd0[0, :, cols])

    def phase0(t, carry):
        half = lax.shift_right_logical(t, 1)
        r = t & 1

        @pl.when(r == 0)
        def _():
            for cp in w1_copies(half):
                cp.wait()

        @pl.when(t < NR0)
        def _():
            x_copy(r).wait()

        real = t >= NP0 - NSL

        @pl.when(real)
        def _():
            wq_wait(t - (NP0 - NSL))

        real_o = t >= NP0 - NWO

        @pl.when(real_o)
        def _():
            wo_copy(t - (NP0 - NWO)).wait()

        rows = pl.ds(pl.multiple_of(r * TM0, TM0), TM0)
        xv = x_v[rows, :]
        gt = _dot(xv, wg0[half, :, pl.ds(0, FH)])
        up = _dot(xv, wu0[half, :, pl.ds(0, FH)])
        hh = (jnp.maximum(gt, 0.0) * up).astype(_BF16)
        dn = _dot(hh, wd0[half, :, dc])
        acc[rows, :] = dn + jnp.where(t >= NR0, acc[rows, :], 0.0)
        permute_slice(jnp.where(real, t - (NP0 - NSL), NSL))
        never = lax.broadcasted_iota(jnp.int32, (8, LANES), 1) < -1 - t
        npc = D * WOC // (8 * LANES)
        p1 = vregs(gt) + vregs(up)
        p1 = [p1[i * len(p1) // npc] for i in range(npc)]
        p2 = vregs(dn)
        p2 = [p2[i * 3 * len(p2) // (4 * npc)] for i in range(npc)]
        permute_wo(jnp.where(real_o, t - (NP0 - NWO), NWO), never, p1, p2)
        return carry

    lax.fori_loop(1, NP0, phase0, 0)
    gw_copy().wait()
    for cp in ffn_copies():
        cp.wait()

    c_exp = (DH ** -0.5) * math.log2(math.e)
    neg = -1e9 / (DH ** -0.5)

    def attn_unit(r, row0, gw, never, link, masked):
        def tie(a, b):
            return a if b is None else jnp.where(never, b, a)

        base = r * TM + row0
        qs = [q_s[j, pl.ds(row0, UNIT), :] for j in range(NT)]
        xr = x_v[pl.ds(pl.multiple_of(base, UNIT), UNIT), :].astype(_F32)
        xg = (tie(xr[:, 0:LANES], link) if GATE_TIE == 2 else xr[:, 0:LANES]) * gw[:, 0:LANES]
        for j in range(1, NT):
            cols = slice(j * LANES, (j + 1) * LANES)
            xg = xg + xr[:, cols] * gw[:, cols]
        logits = []
        for w in range(W):
            st = base + (HALO - DIL * w)
            q0 = tie(qs[0], link) if CHAIN_QK else qs[0]
            s = q0 * k_s[0, pl.ds(st, UNIT), :]
            for j in range(1, NT):
                s = s + qs[j] * k_s[j, pl.ds(st, UNIT), :]
            link = s
            s = s + pltpu.roll(s, 64, 1)
            s = s + pltpu.roll(s, 32, 1)
            if masked and w > 0:
                pos = base + lax.broadcasted_iota(jnp.int32, (UNIT, LANES), 0)
                s = jnp.where(pos >= DIL * w, s, neg)
            logits.append(s)
        m = logits[0]
        for w in range(1, W):
            m = jnp.maximum(m, logits[w])
        ps = [jnp.exp2((logits[w] - m) * c_exp) for w in range(W)]
        den = ps[0]
        for w in range(1, W):
            den = den + ps[w]
        gate = jax.nn.sigmoid(jnp.sum(xg, axis=-1, keepdims=True))
        gate = jnp.broadcast_to(gate, (UNIT, LANES))
        g_s[pl.ds(row0, UNIT), :] = 1.0 - gate
        rinv = gate / den
        olink = gate if GATE_TIE else None
        for j in range(NT):
            p0 = tie(ps[0], olink) if CHAIN_PV else ps[0]
            o = p0 * v_s[j, pl.ds(base + HALO, UNIT), :]
            for w in range(1, W):
                o = o + ps[w] * v_s[j, pl.ds(base + (HALO - DIL * w), UNIT), :]
            olink = o
            o_s[pl.ds(row0, UNIT), pl.ds(j * LANES, LANES)] = (
                (o * rinv).astype(_BF16))
        return olink if CHAIN_UNITS == 2 else (link if CHAIN_UNITS else None)

    def row_block(r, carry):
        rows = pl.ds(pl.multiple_of(r * TM, TM), TM)
        krows = pl.ds(pl.multiple_of(r * TM + HALO, HALO), TM)
        xv = x_v[rows, :]
        for sec, dst in enumerate((q_s, k_s, v_s)):
            pcs = []
            lo, hi = sec * D, (sec + 1) * D
            while lo < hi:
                a = lo // HR
                nxt = min(hi, (a + 1) * HR)
                pcs.append(wq_p[a, pl.ds((lo - a * HR) // 2, (nxt - lo) // 2), dc])
                lo = nxt
            wsec = pltpu.bitcast(jnp.concatenate(pcs, axis=0), _BF16)
            res = _dot(xv, wsec)
            for j in range(NT):
                piece = res[:, j * LANES:(j + 1) * LANES]
                if sec == 0:
                    dst[j] = piece
                else:
                    dst[j, krows, :] = piece
        gw = gw_ref[...].astype(_F32).reshape(1, D)
        never = lax.broadcasted_iota(jnp.int32, (UNIT, LANES), 1) < -1 - r
        links = [None] * NCHAIN
        for un in range(TM // UNIT):
            links[un % NCHAIN] = attn_unit(
                r, un * UNIT, gw, never, links[un % NCHAIN],
                masked=(un * UNIT < HALO))
        for lo, hi in _splits(FCH):
            cols = pl.ds(lo, hi - lo)
            gt = _dot(xv, wg[:, cols])
            up = _dot(xv, wu[:, cols])
            hh = (jnp.maximum(gt, 0.0) * up).astype(_BF16)
            acc[rows, :] += _dot(hh, wd[cols, :])

        ov = o_s[...]
        g1 = g_s[...]
        g1 = jnp.concatenate([g1] * (WOC // LANES), axis=1)
        for n in range(NWO):
            cols = pl.ds(n * WOC, WOC)
            a = _dot(ov, wo_p[n])
            res = (a + g1 * acc[rows, cols]).astype(_BF16)
            for i, (r0, r1, c0, c1) in enumerate(OUT_PIECES):
                if c0 // WOC == n:
                    out_st[i][r] = res[r0:r1, c0 - n * WOC:c1 - n * WOC]
                    out_copy(r, i).start()
        return carry

    lax.fori_loop(0, NR, row_block, 0)
    for i in range(len(OUT_PIECES)):
        for r in range(NR):
            out_copy(r, i).wait()


@jax.jit
def pallas_gated_mix__sliding_local_dilated__glu_gated_reglu__prompt_kernel(
    A_x: jax.Array,
    A_wqkv: jax.Array,
    A_wo: jax.Array,
    B_x: jax.Array,
    B_W_gate: jax.Array,
    B_W_up: jax.Array,
    B_W_down: jax.Array,
    gate_w: jax.Array,
):
    del B_x
    B, S, D = A_x.shape
    F = B_W_gate.shape[1]
    assert B == 1 and D == H * DH == NT * LANES
    assert S % TM == 0 and F - F0 == sum(FCH)
    NR = S // TM
    F1 = F - F0
    assert S // TM0 == 2

    n_sems = len(START_LOADS) + S // TM0 + NG - 1 + NSL + D // WOC + 1
    any_spec = pl.BlockSpec(memory_space=pl.ANY)
    out = pl.pallas_call(
        functools.partial(_kernel, S=S, D=D, F=F),
        out_shape=jax.ShapeDtypeStruct((S, D), _BF16),
        in_specs=[any_spec] * 7,
        out_specs=any_spec,
        scratch_shapes=[
            pltpu.VMEM((S, D), _BF16),
            pltpu.VMEM((NSL + 1, 3 * D // NSL, D), _BF16),
            pltpu.VMEM((NSL + 1, 3 * D // NSL // 2, D + PAD), jnp.uint32),
            pltpu.VMEM((D // WOC + 1, D, WOC), _BF16),
            [pltpu.VMEM((H * (WOP + 1), LANES), _F32)] * (WOC // LANES * DH // 8),
            pltpu.VMEM((D // WOC + 1, D, WOC), _BF16),
            pltpu.VMEM((NG, D, FH), _BF16),
            pltpu.VMEM((NG, D, FH), _BF16),
            pltpu.VMEM((NG, FH, D + PAD), _BF16),
            pltpu.VMEM((D, F1), _BF16),
            pltpu.VMEM((D, F1), _BF16),
            pltpu.VMEM((F1, D), _BF16),
            pltpu.VMEM((S, D), _F32),
            pltpu.VMEM((NT, TM, LANES), _F32),
            pltpu.VMEM((NT, HALO + S, LANES), _F32),
            pltpu.VMEM((NT, HALO + S, LANES), _F32),
            pltpu.VMEM((TM, LANES), _F32),
            pltpu.VMEM((TM, D), _BF16),
            [pltpu.VMEM((NR, r1 - r0, c1 - c0), _BF16)
             for r0, r1, c0, c1 in OUT_PIECES],
            pltpu.VMEM((D,), _BF16),
            pltpu.SemaphoreType.DMA((n_sems,)),
            pltpu.SemaphoreType.DMA((len(OUT_PIECES),)),
        ],
        compiler_params=pltpu.CompilerParams(
            vmem_limit_bytes=120 * 1024 * 1024,
            disable_bounds_checks=True,
            disable_semaphore_checks=True),
        name="gated_mix",
    )(A_x.reshape(S, D), A_wqkv, A_wo, B_W_gate, B_W_up, B_W_down,
      gate_w)
    return out.reshape(B, S, D)
```

```python
import functools
import math

import jax
import jax.numpy as jnp
from jax import lax
import jax.experimental.pallas as pl
import jax.experimental.pallas.tpu as pltpu

H = 32
DH = 32
W = 8
DIL = 2

LANES = 128
NT = 8
HALO = 16

TM = 256
TM0 = 1024
FH = 256
NG = 3
F0 = NG * FH
UNIT = 8
NSL = 4
PB = 4
WOC = 256
WOP = 9
PAD = 128

START_LOADS = (("x", 0, 256), ("g", 0, 128), ("g", 128, 256), ("x", 256, 512),
               ("u", 0, 256), ("x", 512, 1024), ("d", 0, 1024))
START_STAGES = ((2, (("g", 0, 256, 0, 128),)),
                (1, (("g", 0, 256, 128, 256),)),
                (1, (("g", 256, 512, 0, 256),)),
                (1, (("u", 0, 512, 0, 256),)),
                (1, (("g", 512, 1024, 0, 256), ("u", 512, 1024, 0, 256))),
                (1, (("d", 0, 1024, 0, 1024),)))
START_ROWS = 256

_F32 = jnp.float32
_BF16 = jnp.bfloat16


def _out_pieces():
    return ((0, TM, 0, 256), (0, TM, 256, 512), (0, TM, 512, 768),
            (0, TM, 768, 896), (0, TM // 2, 896, 1024),
            (TM // 2, TM, 896, 1024))


def _dot(a, b):
    return jnp.dot(a, b, preferred_element_type=_F32)


def _vregs(v):
    return [v[i * 8:(i + 1) * 8, n * LANES:(n + 1) * LANES]
            for n in range(v.shape[1] // LANES)
            for i in range(v.shape[0] // 8)]


def _kernel(x_hbm, wqkv_hbm, wo_hbm, wg_hbm, wu_hbm, wd_hbm, gw_hbm, out_hbm,
            x_v, wq_raw, wq_p, wo_raw, wo_f, wo_p, wg0, wu0, wd0, wg, wu, wd,
            acc, q_s, k_s, v_s, g_s, o_s, out_st, gw_ref,
            sems, sem_out,
            *, S, D, F):
    NR = S // TM
    NR0 = S // TM0
    NP0 = NG * NR0
    F1 = F - F0
    HR = 3 * D // NSL
    NWO = D // WOC
    out_pieces = _out_pieces()
    dc = pl.ds(0, D)

    SW0 = 0
    SX = SW0 + len(START_LOADS)
    SW1 = SX + NR0 - 1
    SG = SW1 + NG - 1
    SQ = SG + 1
    SO = SQ + NSL
    SR = SO + NWO

    def start_copy(i):
        kind, lo, hi = START_LOADS[i]
        sl = pl.ds(lo, hi - lo)
        if kind == "x":
            src, dst = x_hbm.at[sl, :], x_v.at[sl, :]
        elif kind == "g":
            src, dst = wg_hbm.at[:, sl], wg0.at[0, :, sl]
        elif kind == "u":
            src, dst = wu_hbm.at[:, sl], wu0.at[0, :, sl]
        else:
            src, dst = wd_hbm.at[pl.ds(0, FH), sl], wd0.at[0, :, sl]
        return pltpu.make_async_copy(src, dst, sems.at[SW0 + i])

    def x_copy(r):
        rows = pl.ds(r * TM0, TM0)
        return pltpu.make_async_copy(
            x_hbm.at[rows, :], x_v.at[rows, :], sems.at[SX + r - 1])

    def group_copies(gi):
        sem = sems.at[SW1 + gi - 1]
        lo = gi * FH
        if not isinstance(gi, int):
            lo = pl.multiple_of(lo, LANES)
        fs = pl.ds(lo, FH)
        return (
            pltpu.make_async_copy(wg_hbm.at[:, fs], wg0.at[gi], sem),
            pltpu.make_async_copy(wu_hbm.at[:, fs], wu0.at[gi], sem),
            pltpu.make_async_copy(wd_hbm.at[fs, :], wd0.at[gi, :, dc], sem),
        )

    def gw_copy():
        return pltpu.make_async_copy(gw_hbm, gw_ref, sems.at[SG])

    def wq_copies(a):
        cps = []
        lo, hi = a * HR, (a + 1) * HR
        while lo < hi:
            sec = lo // D
            nxt = min(hi, (sec + 1) * D)
            cps.append(pltpu.make_async_copy(
                wqkv_hbm.at[pl.ds(lo - sec * D, nxt - lo), pl.ds(sec * D, D)],
                wq_raw.at[a, pl.ds(lo - a * HR, nxt - lo), :],
                sems.at[SQ + a]))
            lo = nxt
        return cps

    def wq_wait(a):
        pltpu.make_async_copy(
            wq_raw.at[a], wq_raw.at[a], sems.at[SQ + a]).wait()

    def wo_copy(n):
        lo = n * WOC
        if not isinstance(n, int):
            lo = pl.multiple_of(lo, LANES)
        return pltpu.make_async_copy(
            wo_hbm.at[:, pl.ds(lo, WOC)], wo_raw.at[n], sems.at[SO + n])

    def ffn_copies():
        sem = sems.at[SR]
        f1 = pl.ds(F0, F1)
        return (
            pltpu.make_async_copy(wg_hbm.at[:, f1], wg, sem),
            pltpu.make_async_copy(wu_hbm.at[:, f1], wu, sem),
            pltpu.make_async_copy(wd_hbm.at[f1, :], wd, sem),
        )

    def out_copy(r, i):
        r0, r1, c0, c1 = out_pieces[i]
        return pltpu.make_async_copy(
            out_st[i].at[r],
            out_hbm.at[pl.ds(r * TM + r0, r1 - r0), pl.ds(c0, c1 - c0)],
            sem_out.at[i])

    for i in range(len(START_LOADS)):
        start_copy(i).start()
    for t in range(1, NP0):
        if t < NR0:
            x_copy(t).start()
        if t % NR0 == 0:
            for cp in group_copies(t // NR0):
                cp.start()
        if t >= NP0 - NSL:
            for cp in wq_copies(t - (NP0 - NSL)):
                cp.start()
        if t >= NP0 - NWO:
            wo_copy(t - (NP0 - NWO)).start()
    gw_copy().start()
    for cp in ffn_copies():
        cp.start()

    zeros_halo = jnp.zeros((HALO, LANES), _F32)
    for j in range(NT):
        k_s[j, pl.ds(0, HALO), :] = zeros_halo
        v_s[j, pl.ds(0, HALO), :] = zeros_halo

    n_clear = 16

    def clear(i, carry):
        n = HR // n_clear
        wq_raw[NSL, pl.ds(pl.multiple_of(i * n, 16), n), :] = (
            jnp.zeros((n, D), _BF16))
        n = D // n_clear
        wo_raw[NWO, pl.ds(pl.multiple_of(i * n, 16), n), :] = (
            jnp.zeros((n, WOC), _BF16))
        n = (S - TM0) // n_clear
        acc[pl.ds(pl.multiple_of(TM0 + i * n, 8), n), :] = (
            jnp.zeros((n, D), _F32))
        return carry

    lax.fori_loop(0, n_clear, clear, 0)

    def permute_wqkv(a):
        lane = lax.broadcasted_iota(jnp.int32, (PB * 8, LANES), 1)
        bits = [((lane >> (2 + b)) & 1) == 1 for b in range(3)]
        base_pat = DH * (lane & 3) + (lane >> 5) + 4 * ((lane >> 2) & 7)
        pats = [(base_pat + 4 * j) & (LANES - 1) for j in range(NT)]
        for g in range(HR // (16 * PB)):
            z = []
            for i in range(NT):
                w = pltpu.bitcast(
                    wq_raw[a, pl.ds(g * 16 * PB, 16 * PB),
                           pl.ds(i * LANES, LANES)], jnp.uint32)
                z.append(w if i == 0 else pltpu.roll(w, 4 * i, 1))
            for b in range(3):
                z = [jnp.where(bits[b], z[(k + (1 << b)) % NT], z[k])
                     for k in range(NT)]
            for j in range(NT):
                wq_p[a, pl.ds(g * 8 * PB, 8 * PB), pl.ds(j * LANES, LANES)] = (
                    jnp.take_along_axis(z[(-j) % NT], pats[j], axis=1))

    def permute_wo(n, never, pace1, pace2):
        nj = WOC // LANES
        i = 0
        for h in range(H):
            blk = wo_raw[n, pl.ds(h * DH, DH), :].astype(_F32)
            for a in range(DH // 8):
                for j in range(nj):
                    pc = blk[a * 8:(a + 1) * 8, j * LANES:(j + 1) * LANES]
                    wo_f[a * nj + j][pl.ds(h * WOP, 8), :] = jnp.where(
                        never, pace1[i], pc)
                    i += 1
        i = 0
        for d in range(DH):
            for b in range(H // 8):
                rws = []
                for j in range(nj):
                    pc = wo_f[(d // 8) * nj + j][
                        pl.ds(b * 8 * WOP + d % 8, 8, stride=WOP), :]
                    rws.append(jnp.where(never, pace2[i], pc))
                    i += 1
                wo_p[n, pl.ds(d * H + b * 8, 8), :] = jnp.concatenate(
                    rws, axis=1).astype(_BF16)

    def assemble(pcs):
        return jnp.concatenate(
            [jnp.concatenate([pcs[k] for k in sorted(pcs) if k[0] == r0],
                             axis=1)
             for r0 in sorted({k[0] for k in pcs})], axis=0)

    waited = 0
    parts = {"g": {}, "u": {}}
    for nwait, work in START_STAGES:
        for i in range(waited, waited + nwait):
            start_copy(i).wait()
        waited += nwait
        for kind, r0, r1, c0, c1 in work:
            cols = pl.ds(c0, c1 - c0)
            if kind != "d":
                wref = wg0 if kind == "g" else wu0
                res = _dot(x_v[pl.ds(r0, r1 - r0), :], wref[0, :, cols])
                for rr in range(r0, r1, START_ROWS):
                    for cc in range(c0, c1, LANES):
                        parts[kind][(rr, cc)] = res[
                            rr - r0:rr - r0 + START_ROWS,
                            cc - c0:cc - c0 + LANES]
            else:
                sel = {kd: {k: v for k, v in parts[kd].items()
                            if r0 <= k[0] < r1} for kd in parts}
                hh0 = (jnp.maximum(assemble(sel["g"]), 0.0)
                       * assemble(sel["u"])).astype(_BF16)
                acc[pl.ds(r0, r1 - r0), cols] = _dot(hh0, wd0[0, :, cols])

    def phase0(t, carry):
        gi = lax.shift_right_logical(t, 1)
        r = t & 1

        @pl.when(r == 0)
        def _():
            for cp in group_copies(gi):
                cp.wait()

        @pl.when(t < NR0)
        def _():
            x_copy(r).wait()

        real_q = t >= NP0 - NSL

        @pl.when(real_q)
        def _():
            wq_wait(t - (NP0 - NSL))

        real_o = t >= NP0 - NWO

        @pl.when(real_o)
        def _():
            wo_copy(t - (NP0 - NWO)).wait()

        rows = pl.ds(pl.multiple_of(r * TM0, TM0), TM0)
        xv = x_v[rows, :]
        gt = _dot(xv, wg0[gi])
        up = _dot(xv, wu0[gi])
        hh = (jnp.maximum(gt, 0.0) * up).astype(_BF16)
        dn = _dot(hh, wd0[gi, :, dc])
        acc[rows, :] += dn
        permute_wqkv(jnp.where(real_q, t - (NP0 - NSL), NSL))
        never = lax.broadcasted_iota(jnp.int32, (8, LANES), 1) < -1 - t
        npc = D * WOC // (8 * LANES)
        p1 = _vregs(gt) + _vregs(up)
        p1 = [p1[i * len(p1) // npc] for i in range(npc)]
        p2 = _vregs(dn)
        p2 = [p2[i * 3 * len(p2) // (4 * npc)] for i in range(npc)]
        permute_wo(jnp.where(real_o, t - (NP0 - NWO), NWO), never, p1, p2)
        return carry

    lax.fori_loop(1, NP0, phase0, 0)
    gw_copy().wait()
    for cp in ffn_copies():
        cp.wait()

    scale = DH ** -0.5
    c_exp = scale * math.log2(math.e)
    neg = -1e9 / scale

    def attn_unit(r, row0, gw, never, link, masked):
        def tie(a, b):
            return a if b is None else jnp.where(never, b, a)

        base = r * TM + row0
        qs = [q_s[j, pl.ds(row0, UNIT), :] for j in range(NT)]
        xr = x_v[pl.ds(pl.multiple_of(base, UNIT), UNIT), :].astype(_F32)
        xg = xr[:, 0:LANES] * gw[:, 0:LANES]
        for j in range(1, NT):
            cols = slice(j * LANES, (j + 1) * LANES)
            xg = xg + xr[:, cols] * gw[:, cols]
        logits = []
        for w in range(W):
            st = base + (HALO - DIL * w)
            s = tie(qs[0], link) * k_s[0, pl.ds(st, UNIT), :]
            for j in range(1, NT):
                s = s + qs[j] * k_s[j, pl.ds(st, UNIT), :]
            link = s
            s = s + pltpu.roll(s, 64, 1)
            s = s + pltpu.roll(s, 32, 1)
            if masked and w > 0:
                pos = base + lax.broadcasted_iota(jnp.int32, (UNIT, LANES), 0)
                s = jnp.where(pos >= DIL * w, s, neg)
            logits.append(s)
        m = logits[0]
        for w in range(1, W):
            m = jnp.maximum(m, logits[w])
        ps = [jnp.exp2((logits[w] - m) * c_exp) for w in range(W)]
        den = ps[0]
        for w in range(1, W):
            den = den + ps[w]
        gate = jax.nn.sigmoid(jnp.sum(xg, axis=-1, keepdims=True))
        gate = jnp.broadcast_to(gate, (UNIT, LANES))
        g_s[pl.ds(row0, UNIT), :] = 1.0 - gate
        rinv = gate / den
        link = gate
        for j in range(NT):
            o = tie(ps[0], link) * v_s[j, pl.ds(base + HALO, UNIT), :]
            for w in range(1, W):
                o = o + ps[w] * v_s[j, pl.ds(base + (HALO - DIL * w), UNIT), :]
            link = o
            o_s[pl.ds(row0, UNIT), pl.ds(j * LANES, LANES)] = (
                (o * rinv).astype(_BF16))
        return link

    def row_block(r, carry):
        rows = pl.ds(pl.multiple_of(r * TM, TM), TM)
        krows = pl.ds(pl.multiple_of(r * TM + HALO, HALO), TM)
        xv = x_v[rows, :]
        for sec, dst in enumerate((q_s, k_s, v_s)):
            pcs = []
            lo, hi = sec * D, (sec + 1) * D
            while lo < hi:
                a = lo // HR
                nxt = min(hi, (a + 1) * HR)
                pcs.append(
                    wq_p[a, pl.ds((lo - a * HR) // 2, (nxt - lo) // 2), dc])
                lo = nxt
            res = _dot(xv, pltpu.bitcast(jnp.concatenate(pcs, axis=0), _BF16))
            for j in range(NT):
                piece = res[:, j * LANES:(j + 1) * LANES]
                if sec == 0:
                    dst[j] = piece
                else:
                    dst[j, krows, :] = piece

        gw = gw_ref[...].astype(_F32).reshape(1, D)
        never = lax.broadcasted_iota(jnp.int32, (UNIT, LANES), 1) < -1 - r
        link = None
        for un in range(TM // UNIT):
            link = attn_unit(r, un * UNIT, gw, never, link,
                             masked=(un * UNIT < HALO))

        gt = _dot(xv, wg[...])
        up = _dot(xv, wu[...])
        hh = (jnp.maximum(gt, 0.0) * up).astype(_BF16)
        acc[rows, :] += _dot(hh, wd[...])

        ov = o_s[...]
        g1 = jnp.concatenate([g_s[...]] * (WOC // LANES), axis=1)
        for n in range(NWO):
            res = (_dot(ov, wo_p[n])
                   + g1 * acc[rows, pl.ds(n * WOC, WOC)]).astype(_BF16)
            for i, (r0, r1, c0, c1) in enumerate(out_pieces):
                if c0 // WOC == n:
                    out_st[i][r] = res[r0:r1, c0 - n * WOC:c1 - n * WOC]
                    out_copy(r, i).start()
        return carry

    lax.fori_loop(0, NR, row_block, 0)
    for i in range(len(out_pieces)):
        for r in range(NR):
            out_copy(r, i).wait()


@jax.jit
def pallas_gated_mix__sliding_local_dilated__glu_gated_reglu__prompt_kernel(
    A_x: jax.Array,
    A_wqkv: jax.Array,
    A_wo: jax.Array,
    B_x: jax.Array,
    B_W_gate: jax.Array,
    B_W_up: jax.Array,
    B_W_down: jax.Array,
    gate_w: jax.Array,
):
    del B_x
    B, S, D = A_x.shape
    F = B_W_gate.shape[1]
    assert B == 1 and D == H * DH == NT * LANES
    assert S % TM == 0 and S == 2 * TM0 and F > F0 and F % LANES == 0
    NR = S // TM
    F1 = F - F0
    HR = 3 * D // NSL
    NWO = D // WOC
    out_pieces = _out_pieces()
    n_sems = len(START_LOADS) + S // TM0 + NG - 1 + NSL + NWO + 1

    any_spec = pl.BlockSpec(memory_space=pl.ANY)
    out = pl.pallas_call(
        functools.partial(_kernel, S=S, D=D, F=F),
        out_shape=jax.ShapeDtypeStruct((S, D), _BF16),
        in_specs=[any_spec] * 7,
        out_specs=any_spec,
        scratch_shapes=[
            pltpu.VMEM((S, D), _BF16),
            pltpu.VMEM((NSL + 1, HR, D), _BF16),
            pltpu.VMEM((NSL + 1, HR // 2, D + PAD), jnp.uint32),
            pltpu.VMEM((NWO + 1, D, WOC), _BF16),
            [pltpu.VMEM((H * (WOP + 1), LANES), _F32)
             for _ in range(WOC // LANES * DH // 8)],
            pltpu.VMEM((NWO + 1, D, WOC), _BF16),
            pltpu.VMEM((NG, D, FH), _BF16),
            pltpu.VMEM((NG, D, FH), _BF16),
            pltpu.VMEM((NG, FH, D + PAD), _BF16),
            pltpu.VMEM((D, F1), _BF16),
            pltpu.VMEM((D, F1), _BF16),
            pltpu.VMEM((F1, D), _BF16),
            pltpu.VMEM((S, D), _F32),
            pltpu.VMEM((NT, TM, LANES), _F32),
            pltpu.VMEM((NT, HALO + S, LANES), _F32),
            pltpu.VMEM((NT, HALO + S, LANES), _F32),
            pltpu.VMEM((TM, LANES), _F32),
            pltpu.VMEM((TM, D), _BF16),
            [pltpu.VMEM((NR, r1 - r0, c1 - c0), _BF16)
             for r0, r1, c0, c1 in out_pieces],
            pltpu.VMEM((D,), _BF16),
            pltpu.SemaphoreType.DMA((n_sems,)),
            pltpu.SemaphoreType.DMA((len(out_pieces),)),
        ],
        compiler_params=pltpu.CompilerParams(
            vmem_limit_bytes=120 * 1024 * 1024,
            disable_bounds_checks=True,
            disable_semaphore_checks=True),
        name="gated_mix",
    )(A_x.reshape(S, D), A_wqkv, A_wo, B_W_gate, B_W_up, B_W_down, gate_w)
    return out.reshape(B, S, D)
```

```python
import functools
import math

import jax
import jax.numpy as jnp
from jax import lax
import jax.experimental.pallas as pl
import jax.experimental.pallas.tpu as pltpu

H = 32
DH = 32
W = 8
DIL = 2

LANES = 128
NT = 8
HALO = 16

TM = 256
TM0 = 1024
FH = 256
NG = 3
F0 = NG * FH
UNIT = 8
NSL = 4
PB = 4
WOC = 256
WOP = 9
PAD = 128

START_LOADS = (("x", 0, 256), ("g", 0, 128), ("g", 128, 256), ("x", 256, 512),
               ("u", 0, 256), ("x", 512, 1024), ("d", 0, 1024))
START_STAGES = ((2, (("g", 0, 256, 0, 128),)),
                (1, (("g", 0, 256, 128, 256),)),
                (1, (("g", 256, 512, 0, 256),)),
                (1, (("u", 0, 512, 0, 256),)),
                (1, (("g", 512, 1024, 0, 256), ("u", 512, 1024, 0, 256))),
                (1, (("d", 0, 1024, 0, 1024),)))
START_ROWS = 256

_F32 = jnp.float32
_BF16 = jnp.bfloat16


def _out_pieces():
    return ((0, TM, 0, 256), (0, TM, 256, 512), (0, TM, 512, 768),
            (0, TM, 768, 896), (0, TM // 2, 896, 1024),
            (TM // 2, TM, 896, 1024))


def _dot(a, b):
    return jnp.dot(a, b, preferred_element_type=_F32)


def _vregs(v):
    return [v[i * 8:(i + 1) * 8, n * LANES:(n + 1) * LANES]
            for n in range(v.shape[1] // LANES)
            for i in range(v.shape[0] // 8)]


def _kernel(x_hbm, wqkv_hbm, wo_hbm, wg_hbm, wu_hbm, wd_hbm, gw_hbm, out_hbm,
            x_v, wq_raw, wq_p, wo_raw, wo_f, wo_p, wg0, wu0, wd0, wg, wu, wd,
            acc, q_s, k_s, v_s, g_s, o_s, out_st, gw_ref,
            sems, sem_out,
            *, S, D, F):
    NR = S // TM
    NR0 = S // TM0
    NP0 = NG * NR0
    F1 = F - F0
    HR = 3 * D // NSL
    NWO = D // WOC
    out_pieces = _out_pieces()
    dc = pl.ds(0, D)

    SW0 = 0
    SX = SW0 + len(START_LOADS)
    SW1 = SX + NR0 - 1
    SG = SW1 + NG - 1
    SQ = SG + 1
    SO = SQ + NSL
    SR = SO + NWO

    def start_copy(i):
        kind, lo, hi = START_LOADS[i]
        sl = pl.ds(lo, hi - lo)
        if kind == "x":
            src, dst = x_hbm.at[sl, :], x_v.at[sl, :]
        elif kind == "g":
            src, dst = wg_hbm.at[:, sl], wg0.at[0, :, sl]
        elif kind == "u":
            src, dst = wu_hbm.at[:, sl], wu0.at[0, :, sl]
        else:
            src, dst = wd_hbm.at[pl.ds(0, FH), sl], wd0.at[0, :, sl]
        return pltpu.make_async_copy(src, dst, sems.at[SW0 + i])

    def x_copy(r):
        rows = pl.ds(r * TM0, TM0)
        return pltpu.make_async_copy(
            x_hbm.at[rows, :], x_v.at[rows, :], sems.at[SX + r - 1])

    def group_copies(gi):
        sem = sems.at[SW1 + gi - 1]
        lo = gi * FH
        if not isinstance(gi, int):
            lo = pl.multiple_of(lo, LANES)
        fs = pl.ds(lo, FH)
        return (
            pltpu.make_async_copy(wg_hbm.at[:, fs], wg0.at[gi], sem),
            pltpu.make_async_copy(wu_hbm.at[:, fs], wu0.at[gi], sem),
            pltpu.make_async_copy(wd_hbm.at[fs, :], wd0.at[gi, :, dc], sem),
        )

    def gw_copy():
        return pltpu.make_async_copy(gw_hbm, gw_ref, sems.at[SG])

    def wq_copies(a):
        cps = []
        lo, hi = a * HR, (a + 1) * HR
        while lo < hi:
            sec = lo // D
            nxt = min(hi, (sec + 1) * D)
            cps.append(pltpu.make_async_copy(
                wqkv_hbm.at[pl.ds(lo - sec * D, nxt - lo), pl.ds(sec * D, D)],
                wq_raw.at[a, pl.ds(lo - a * HR, nxt - lo), :],
                sems.at[SQ + a]))
            lo = nxt
        return cps

    def wq_wait(a):
        pltpu.make_async_copy(
            wq_raw.at[a], wq_raw.at[a], sems.at[SQ + a]).wait()

    def wo_copy(n):
        lo = n * WOC
        if not isinstance(n, int):
            lo = pl.multiple_of(lo, LANES)
        return pltpu.make_async_copy(
            wo_hbm.at[:, pl.ds(lo, WOC)], wo_raw.at[n], sems.at[SO + n])

    def ffn_copies():
        sem = sems.at[SR]
        f1 = pl.ds(F0, F1)
        return (
            pltpu.make_async_copy(wg_hbm.at[:, f1], wg, sem),
            pltpu.make_async_copy(wu_hbm.at[:, f1], wu, sem),
            pltpu.make_async_copy(wd_hbm.at[f1, :], wd, sem),
        )

    def out_copy(r, i):
        r0, r1, c0, c1 = out_pieces[i]
        return pltpu.make_async_copy(
            out_st[i].at[r],
            out_hbm.at[pl.ds(r * TM + r0, r1 - r0), pl.ds(c0, c1 - c0)],
            sem_out.at[i])

    for i in range(len(START_LOADS)):
        start_copy(i).start()
    for t in range(1, NP0):
        if t < NR0:
            x_copy(t).start()
        if t % NR0 == 0:
            for cp in group_copies(t // NR0):
                cp.start()
        if t >= NP0 - NSL:
            for cp in wq_copies(t - (NP0 - NSL)):
                cp.start()
        if t >= NP0 - NWO:
            wo_copy(t - (NP0 - NWO)).start()
    gw_copy().start()
    for cp in ffn_copies():
        cp.start()

    zeros_halo = jnp.zeros((HALO, LANES), _F32)
    for j in range(NT):
        k_s[j, pl.ds(0, HALO), :] = zeros_halo
        v_s[j, pl.ds(0, HALO), :] = zeros_halo

    n_clear = 16

    def clear(i, carry):
        n = HR // n_clear
        wq_raw[NSL, pl.ds(pl.multiple_of(i * n, 16), n), :] = (
            jnp.zeros((n, D), _BF16))
        n = D // n_clear
        wo_raw[NWO, pl.ds(pl.multiple_of(i * n, 16), n), :] = (
            jnp.zeros((n, WOC), _BF16))
        n = (S - TM0) // n_clear
        acc[pl.ds(pl.multiple_of(TM0 + i * n, 8), n), :] = (
            jnp.zeros((n, D), _F32))
        return carry

    lax.fori_loop(0, n_clear, clear, 0)

    def permute_wqkv(a):
        lane = lax.broadcasted_iota(jnp.int32, (PB * 8, LANES), 1)
        bits = [((lane >> (2 + b)) & 1) == 1 for b in range(3)]
        swap = ((lane & 3) << 5) | (lane & 28) | (lane >> 5)
        for g in range(HR // (16 * PB)):
            z = []
            for i in range(NT):
                w = pltpu.bitcast(
                    wq_raw[a, pl.ds(g * 16 * PB, 16 * PB),
                           pl.ds(i * LANES, LANES)], jnp.uint32)
                w = jnp.take_along_axis(w, swap, axis=1)
                z.append(w if i == 0 else pltpu.roll(w, 4 * i, 1))
            for b in range(3):
                z = [jnp.where(bits[b], z[(k + (1 << b)) % NT], z[k])
                     for k in range(NT)]
            for j in range(NT):
                y = z[(-j) % NT]
                wq_p[a, pl.ds(g * 8 * PB, 8 * PB), pl.ds(j * LANES, LANES)] = (
                    y if j == 0 else pltpu.roll(y, LANES - 4 * j, 1))

    def permute_wo(n, never, pace1, pace2):
        nj = WOC // LANES
        i = 0
        for h in range(H):
            blk = wo_raw[n, pl.ds(h * DH, DH), :].astype(_F32)
            for a in range(DH // 8):
                for j in range(nj):
                    pc = blk[a * 8:(a + 1) * 8, j * LANES:(j + 1) * LANES]
                    wo_f[a * nj + j][pl.ds(h * WOP, 8), :] = jnp.where(
                        never, pace1[i], pc)
                    i += 1
        i = 0
        for d in range(DH):
            for b in range(H // 8):
                rws = []
                for j in range(nj):
                    pc = wo_f[(d // 8) * nj + j][
                        pl.ds(b * 8 * WOP + d % 8, 8, stride=WOP), :]
                    rws.append(jnp.where(never, pace2[i], pc))
                    i += 1
                wo_p[n, pl.ds(d * H + b * 8, 8), :] = jnp.concatenate(
                    rws, axis=1).astype(_BF16)

    def assemble(pcs):
        return jnp.concatenate(
            [jnp.concatenate([pcs[k] for k in sorted(pcs) if k[0] == r0],
                             axis=1)
             for r0 in sorted({k[0] for k in pcs})], axis=0)

    waited = 0
    parts = {"g": {}, "u": {}}
    for nwait, work in START_STAGES:
        for i in range(waited, waited + nwait):
            start_copy(i).wait()
        waited += nwait
        for kind, r0, r1, c0, c1 in work:
            cols = pl.ds(c0, c1 - c0)
            if kind != "d":
                wref = wg0 if kind == "g" else wu0
                res = _dot(x_v[pl.ds(r0, r1 - r0), :], wref[0, :, cols])
                for rr in range(r0, r1, START_ROWS):
                    for cc in range(c0, c1, LANES):
                        parts[kind][(rr, cc)] = res[
                            rr - r0:rr - r0 + START_ROWS,
                            cc - c0:cc - c0 + LANES]
            else:
                sel = {kd: {k: v for k, v in parts[kd].items()
                            if r0 <= k[0] < r1} for kd in parts}
                hh0 = (jnp.maximum(assemble(sel["g"]), 0.0)
                       * assemble(sel["u"])).astype(_BF16)
                acc[pl.ds(r0, r1 - r0), cols] = _dot(hh0, wd0[0, :, cols])

    def phase0(t, carry):
        gi = lax.shift_right_logical(t, 1)
        r = t & 1

        @pl.when(r == 0)
        def _():
            for cp in group_copies(gi):
                cp.wait()

        @pl.when(t < NR0)
        def _():
            x_copy(r).wait()

        real_q = t >= NP0 - NSL

        @pl.when(real_q)
        def _():
            wq_wait(t - (NP0 - NSL))

        real_o = t >= NP0 - NWO

        @pl.when(real_o)
        def _():
            wo_copy(t - (NP0 - NWO)).wait()

        rows = pl.ds(pl.multiple_of(r * TM0, TM0), TM0)
        xv = x_v[rows, :]
        gt = _dot(xv, wg0[gi])
        up = _dot(xv, wu0[gi])
        hh = (jnp.maximum(gt, 0.0) * up).astype(_BF16)
        dn = _dot(hh, wd0[gi, :, dc])
        acc[rows, :] += dn
        permute_wqkv(jnp.where(real_q, t - (NP0 - NSL), NSL))
        never = lax.broadcasted_iota(jnp.int32, (8, LANES), 1) < -1 - t
        npc = D * WOC // (8 * LANES)
        p1 = _vregs(gt) + _vregs(up)
        p1 = [p1[i * len(p1) // npc] for i in range(npc)]
        p2 = _vregs(dn)
        p2 = [p2[i * 3 * len(p2) // (4 * npc)] for i in range(npc)]
        permute_wo(jnp.where(real_o, t - (NP0 - NWO), NWO), never, p1, p2)
        return carry

    lax.fori_loop(1, NP0, phase0, 0)
    gw_copy().wait()
    for cp in ffn_copies():
        cp.wait()

    scale = DH ** -0.5
    c_exp = scale * math.log2(math.e)
    neg = -1e9 / scale

    def attn_unit(r, row0, gw, never, link, masked):
        def tie(a, b):
            return a if b is None else jnp.where(never, b, a)

        base = r * TM + row0
        qs = [q_s[j, pl.ds(row0, UNIT), :] for j in range(NT)]
        xr = x_v[pl.ds(pl.multiple_of(base, UNIT), UNIT), :].astype(_F32)
        xg = xr[:, 0:LANES] * gw[:, 0:LANES]
        for j in range(1, NT):
            cols = slice(j * LANES, (j + 1) * LANES)
            xg = xg + xr[:, cols] * gw[:, cols]
        logits = []
        for w in range(W):
            st = base + (HALO - DIL * w)
            s = tie(qs[0], link) * k_s[0, pl.ds(st, UNIT), :]
            for j in range(1, NT):
                s = s + qs[j] * k_s[j, pl.ds(st, UNIT), :]
            link = s
            s = s + pltpu.roll(s, 64, 1)
            s = s + pltpu.roll(s, 32, 1)
            if masked and w > 0:
                pos = base + lax.broadcasted_iota(jnp.int32, (UNIT, LANES), 0)
                s = jnp.where(pos >= DIL * w, s, neg)
            logits.append(s)
        m = logits[0]
        for w in range(1, W):
            m = jnp.maximum(m, logits[w])
        ps = [jnp.exp2((logits[w] - m) * c_exp) for w in range(W)]
        den = ps[0]
        for w in range(1, W):
            den = den + ps[w]
        gate = jax.nn.sigmoid(jnp.sum(xg, axis=-1, keepdims=True))
        gate = jnp.broadcast_to(gate, (UNIT, LANES))
        g_s[pl.ds(row0, UNIT), :] = 1.0 - gate
        rinv = gate / den
        link = gate
        for j in range(NT):
            o = tie(ps[0], link) * v_s[j, pl.ds(base + HALO, UNIT), :]
            for w in range(1, W):
                o = o + ps[w] * v_s[j, pl.ds(base + (HALO - DIL * w), UNIT), :]
            link = o
            o_s[pl.ds(row0, UNIT), pl.ds(j * LANES, LANES)] = (
                (o * rinv).astype(_BF16))
        return link

    def row_block(r, carry):
        rows = pl.ds(pl.multiple_of(r * TM, TM), TM)
        krows = pl.ds(pl.multiple_of(r * TM + HALO, HALO), TM)
        xv = x_v[rows, :]
        for sec, dst in enumerate((q_s, k_s, v_s)):
            pcs = []
            lo, hi = sec * D, (sec + 1) * D
            while lo < hi:
                a = lo // HR
                nxt = min(hi, (a + 1) * HR)
                pcs.append(
                    wq_p[a, pl.ds((lo - a * HR) // 2, (nxt - lo) // 2), dc])
                lo = nxt
            res = _dot(xv, pltpu.bitcast(jnp.concatenate(pcs, axis=0), _BF16))
            for j in range(NT):
                piece = res[:, j * LANES:(j + 1) * LANES]
                if sec == 0:
                    dst[j] = piece
                else:
                    dst[j, krows, :] = piece

        gw = gw_ref[...].astype(_F32).reshape(1, D)
        never = lax.broadcasted_iota(jnp.int32, (UNIT, LANES), 1) < -1 - r
        link = None
        for un in range(TM // UNIT):
            link = attn_unit(r, un * UNIT, gw, never, link,
                             masked=(un * UNIT < HALO))

        gt = _dot(xv, wg[...])
        up = _dot(xv, wu[...])
        hh = (jnp.maximum(gt, 0.0) * up).astype(_BF16)
        acc[rows, :] += _dot(hh, wd[...])

        ov = o_s[...]
        g1 = jnp.concatenate([g_s[...]] * (WOC // LANES), axis=1)
        for n in range(NWO):
            res = (_dot(ov, wo_p[n])
                   + g1 * acc[rows, pl.ds(n * WOC, WOC)]).astype(_BF16)
            for i, (r0, r1, c0, c1) in enumerate(out_pieces):
                if c0 // WOC == n:
                    out_st[i][r] = res[r0:r1, c0 - n * WOC:c1 - n * WOC]
                    out_copy(r, i).start()
        return carry

    lax.fori_loop(0, NR, row_block, 0)
    for i in range(len(out_pieces)):
        for r in range(NR):
            out_copy(r, i).wait()


@jax.jit
def pallas_gated_mix__sliding_local_dilated__glu_gated_reglu__prompt_kernel(
    A_x: jax.Array,
    A_wqkv: jax.Array,
    A_wo: jax.Array,
    B_x: jax.Array,
    B_W_gate: jax.Array,
    B_W_up: jax.Array,
    B_W_down: jax.Array,
    gate_w: jax.Array,
):
    del B_x
    B, S, D = A_x.shape
    F = B_W_gate.shape[1]
    assert B == 1 and D == H * DH == NT * LANES
    assert S % TM == 0 and S == 2 * TM0 and F > F0 and F % LANES == 0
    NR = S // TM
    F1 = F - F0
    HR = 3 * D // NSL
    NWO = D // WOC
    out_pieces = _out_pieces()
    n_sems = len(START_LOADS) + S // TM0 + NG - 1 + NSL + NWO + 1

    any_spec = pl.BlockSpec(memory_space=pl.ANY)
    out = pl.pallas_call(
        functools.partial(_kernel, S=S, D=D, F=F),
        out_shape=jax.ShapeDtypeStruct((S, D), _BF16),
        in_specs=[any_spec] * 7,
        out_specs=any_spec,
        scratch_shapes=[
            pltpu.VMEM((S, D), _BF16),
            pltpu.VMEM((NSL + 1, HR, D), _BF16),
            pltpu.VMEM((NSL + 1, HR // 2, D + PAD), jnp.uint32),
            pltpu.VMEM((NWO + 1, D, WOC), _BF16),
            [pltpu.VMEM((H * (WOP + 1), LANES), _F32)
             for _ in range(WOC // LANES * DH // 8)],
            pltpu.VMEM((NWO + 1, D, WOC), _BF16),
            pltpu.VMEM((NG, D, FH), _BF16),
            pltpu.VMEM((NG, D, FH), _BF16),
            pltpu.VMEM((NG, FH, D + PAD), _BF16),
            pltpu.VMEM((D, F1), _BF16),
            pltpu.VMEM((D, F1), _BF16),
            pltpu.VMEM((F1, D), _BF16),
            pltpu.VMEM((S, D), _F32),
            pltpu.VMEM((NT, TM, LANES), _F32),
            pltpu.VMEM((NT, HALO + S, LANES), _F32),
            pltpu.VMEM((NT, HALO + S, LANES), _F32),
            pltpu.VMEM((TM, LANES), _F32),
            pltpu.VMEM((TM, D), _BF16),
            [pltpu.VMEM((NR, r1 - r0, c1 - c0), _BF16)
             for r0, r1, c0, c1 in out_pieces],
            pltpu.VMEM((D,), _BF16),
            pltpu.SemaphoreType.DMA((n_sems,)),
            pltpu.SemaphoreType.DMA((len(out_pieces),)),
        ],
        compiler_params=pltpu.CompilerParams(
            vmem_limit_bytes=120 * 1024 * 1024,
            disable_bounds_checks=True,
            disable_semaphore_checks=True),
        name="gated_mix",
    )(A_x.reshape(S, D), A_wqkv, A_wo, B_W_gate, B_W_up, B_W_down, gate_w)
    return out.reshape(B, S, D)
```

```python
import functools
import math

import jax
import jax.numpy as jnp
from jax import lax
import jax.experimental.pallas as pl
import jax.experimental.pallas.tpu as pltpu

H = 32
DH = 32
W = 8
DIL = 2

LANES = 128
NT = 8
HALO = 16

TM = 256
TM0 = 1024
FH = 256
NG = 3
F0 = NG * FH
UNIT = 8
NSL = 4
PB = 4
WOC = 256
WOP = 9
PAD = 128

START_K = (128, 128, 256, 256, 256)

_F32 = jnp.float32
_BF16 = jnp.bfloat16


def _out_pieces():
    return ((0, TM, 0, 256), (0, TM, 256, 512), (0, TM, 512, 768),
            (0, TM, 768, 896), (0, TM // 2, 896, 1024),
            (TM // 2, TM, 896, 1024))


def _dot(a, b):
    return jnp.dot(a, b, preferred_element_type=_F32)


def _vregs(v):
    return [v[i * 8:(i + 1) * 8, n * LANES:(n + 1) * LANES]
            for n in range(v.shape[1] // LANES)
            for i in range(v.shape[0] // 8)]


def _kernel(x_hbm, wqkv_hbm, wo_hbm, wg_hbm, wu_hbm, wd_hbm, gw_hbm, out_hbm,
            x_v, wq_raw, wq_p, wo_raw, wo_f, wo_p, wg0, wu0, wd0, wg, wu, wd,
            acc, gu_s, q_s, k_s, v_s, g_s, o_s, out_st, gw_ref,
            sems, sem_out,
            *, S, D, F):
    NR = S // TM
    NR0 = S // TM0
    NP0 = NG * NR0
    F1 = F - F0
    HR = 3 * D // NSL
    NWO = D // WOC
    out_pieces = _out_pieces()
    dc = pl.ds(0, D)

    SW0 = 0
    SX = SW0 + len(START_K)
    SW1 = SX + NR0 - 1
    SG = SW1 + NG - 1
    SQ = SG + 1
    SO = SQ + NSL
    SR = SO + NWO

    def start_copies(i):
        ks = pl.ds(sum(START_K[:i]), START_K[i])
        sem = sems.at[SW0 + i]
        rows = pl.ds(0, TM0)
        fs = pl.ds(0, FH)
        cps = [
            pltpu.make_async_copy(wg_hbm.at[ks, fs], wg0.at[0, ks, :], sem),
            pltpu.make_async_copy(wu_hbm.at[ks, fs], wu0.at[0, ks, :], sem),
            pltpu.make_async_copy(x_hbm.at[rows, ks], x_v.at[rows, ks], sem),
        ]
        if i == len(START_K) - 1:
            cps.append(pltpu.make_async_copy(
                wd_hbm.at[fs, :], wd0.at[0, :, dc], sem))
        return cps

    def x_copy(r):
        rows = pl.ds(r * TM0, TM0)
        return pltpu.make_async_copy(
            x_hbm.at[rows, :], x_v.at[rows, :], sems.at[SX + r - 1])

    def group_copies(gi):
        sem = sems.at[SW1 + gi - 1]
        lo = gi * FH
        if not isinstance(gi, int):
            lo = pl.multiple_of(lo, LANES)
        fs = pl.ds(lo, FH)
        return (
            pltpu.make_async_copy(wg_hbm.at[:, fs], wg0.at[gi], sem),
            pltpu.make_async_copy(wu_hbm.at[:, fs], wu0.at[gi], sem),
            pltpu.make_async_copy(wd_hbm.at[fs, :], wd0.at[gi, :, dc], sem),
        )

    def gw_copy():
        return pltpu.make_async_copy(gw_hbm, gw_ref, sems.at[SG])

    def wq_copies(a):
        cps = []
        lo, hi = a * HR, (a + 1) * HR
        while lo < hi:
            sec = lo // D
            nxt = min(hi, (sec + 1) * D)
            cps.append(pltpu.make_async_copy(
                wqkv_hbm.at[pl.ds(lo - sec * D, nxt - lo), pl.ds(sec * D, D)],
                wq_raw.at[a, pl.ds(lo - a * HR, nxt - lo), :],
                sems.at[SQ + a]))
            lo = nxt
        return cps

    def wq_wait(a):
        pltpu.make_async_copy(
            wq_raw.at[a], wq_raw.at[a], sems.at[SQ + a]).wait()

    def wo_copy(n):
        lo = n * WOC
        if not isinstance(n, int):
            lo = pl.multiple_of(lo, LANES)
        return pltpu.make_async_copy(
            wo_hbm.at[:, pl.ds(lo, WOC)], wo_raw.at[n], sems.at[SO + n])

    def ffn_copies():
        sem = sems.at[SR]
        f1 = pl.ds(F0, F1)
        return (
            pltpu.make_async_copy(wg_hbm.at[:, f1], wg, sem),
            pltpu.make_async_copy(wu_hbm.at[:, f1], wu, sem),
            pltpu.make_async_copy(wd_hbm.at[f1, :], wd, sem),
        )

    def out_copy(r, i):
        r0, r1, c0, c1 = out_pieces[i]
        return pltpu.make_async_copy(
            out_st[i].at[r],
            out_hbm.at[pl.ds(r * TM + r0, r1 - r0), pl.ds(c0, c1 - c0)],
            sem_out.at[i])

    for i in range(len(START_K)):
        for cp in start_copies(i):
            cp.start()
    for t in range(1, NP0):
        if t < NR0:
            x_copy(t).start()
        if t % NR0 == 0:
            for cp in group_copies(t // NR0):
                cp.start()
        if t >= NP0 - NSL:
            for cp in wq_copies(t - (NP0 - NSL)):
                cp.start()
        if t >= NP0 - NWO:
            wo_copy(t - (NP0 - NWO)).start()
    gw_copy().start()
    for cp in ffn_copies():
        cp.start()

    zeros_halo = jnp.zeros((HALO, LANES), _F32)
    for j in range(NT):
        k_s[j, pl.ds(0, HALO), :] = zeros_halo
        v_s[j, pl.ds(0, HALO), :] = zeros_halo

    n_clear = 16

    def clear(i, carry):
        n = HR // n_clear
        wq_raw[NSL, pl.ds(pl.multiple_of(i * n, 16), n), :] = (
            jnp.zeros((n, D), _BF16))
        n = D // n_clear
        wo_raw[NWO, pl.ds(pl.multiple_of(i * n, 16), n), :] = (
            jnp.zeros((n, WOC), _BF16))
        return carry

    lax.fori_loop(0, n_clear, clear, 0)

    def permute_wqkv(a):
        lane = lax.broadcasted_iota(jnp.int32, (PB * 8, LANES), 1)
        bits = [((lane >> (2 + b)) & 1) == 1 for b in range(3)]
        swap = ((lane & 3) << 5) | (lane & 28) | (lane >> 5)
        for g in range(HR // (16 * PB)):
            z = []
            for i in range(NT):
                w = pltpu.bitcast(
                    wq_raw[a, pl.ds(g * 16 * PB, 16 * PB),
                           pl.ds(i * LANES, LANES)], jnp.uint32)
                w = jnp.take_along_axis(w, swap, axis=1)
                z.append(w if i == 0 else pltpu.roll(w, 4 * i, 1))
            for b in range(3):
                z = [jnp.where(bits[b], z[(k + (1 << b)) % NT], z[k])
                     for k in range(NT)]
            for j in range(NT):
                y = z[(-j) % NT]
                wq_p[a, pl.ds(g * 8 * PB, 8 * PB), pl.ds(j * LANES, LANES)] = (
                    y if j == 0 else pltpu.roll(y, LANES - 4 * j, 1))

    def permute_wo(n, never, pace1, pace2):
        nj = WOC // LANES
        i = 0
        for h in range(H):
            blk = wo_raw[n, pl.ds(h * DH, DH), :].astype(_F32)
            for a in range(DH // 8):
                for j in range(nj):
                    pc = blk[a * 8:(a + 1) * 8, j * LANES:(j + 1) * LANES]
                    wo_f[a * nj + j][pl.ds(h * WOP, 8), :] = jnp.where(
                        never, pace1[i], pc)
                    i += 1
        i = 0
        for d in range(DH):
            for b in range(H // 8):
                rws = []
                for j in range(nj):
                    pc = wo_f[(d // 8) * nj + j][
                        pl.ds(b * 8 * WOP + d % 8, 8, stride=WOP), :]
                    rws.append(jnp.where(never, pace2[i], pc))
                    i += 1
                wo_p[n, pl.ds(d * H + b * 8, 8), :] = jnp.concatenate(
                    rws, axis=1).astype(_BF16)

    for i in range(len(START_K)):
        for cp in start_copies(i):
            cp.wait()
        ks = pl.ds(sum(START_K[:i]), START_K[i])
        part = _dot(x_v[pl.ds(0, TM0), ks],
                    jnp.concatenate([wg0[0, ks, :], wu0[0, ks, :]], axis=1))
        gu = part if i == 0 else part + gu_s[...]
        if i < len(START_K) - 1:
            gu_s[...] = gu
    hh0 = (jnp.maximum(gu[:, :FH], 0.0) * gu[:, FH:]).astype(_BF16)
    acc[pl.ds(0, TM0), :] = _dot(hh0, wd0[0, :, dc])

    def phase0(t, carry):
        gi = lax.shift_right_logical(t, 1)
        r = t & 1

        @pl.when(r == 0)
        def _():
            for cp in group_copies(gi):
                cp.wait()

        @pl.when(t < NR0)
        def _():
            x_copy(r).wait()

        real_q = t >= NP0 - NSL

        @pl.when(real_q)
        def _():
            wq_wait(t - (NP0 - NSL))

        real_o = t >= NP0 - NWO

        @pl.when(real_o)
        def _():
            wo_copy(t - (NP0 - NWO)).wait()

        rows = pl.ds(pl.multiple_of(r * TM0, TM0), TM0)
        xv = x_v[rows, :]
        gt = _dot(xv, wg0[gi])
        up = _dot(xv, wu0[gi])
        hh = (jnp.maximum(gt, 0.0) * up).astype(_BF16)
        dn = _dot(hh, wd0[gi, :, dc])
        acc[rows, :] = dn + jnp.where(t >= NR0, acc[rows, :], 0.0)
        permute_wqkv(jnp.where(real_q, t - (NP0 - NSL), NSL))
        never = lax.broadcasted_iota(jnp.int32, (8, LANES), 1) < -1 - t
        npc = D * WOC // (8 * LANES)
        p1 = _vregs(gt) + _vregs(up)
        p1 = [p1[i * len(p1) // npc] for i in range(npc)]
        p2 = _vregs(dn)
        p2 = [p2[i * 3 * len(p2) // (4 * npc)] for i in range(npc)]
        permute_wo(jnp.where(real_o, t - (NP0 - NWO), NWO), never, p1, p2)
        return carry

    lax.fori_loop(1, NP0, phase0, 0)
    gw_copy().wait()
    for cp in ffn_copies():
        cp.wait()

    scale = DH ** -0.5
    c_exp = scale * math.log2(math.e)
    neg = -1e9 / scale

    def attn_unit(r, row0, gw, never, link, masked):
        def tie(a, b):
            return a if b is None else jnp.where(never, b, a)

        base = r * TM + row0
        qs = [q_s[j, pl.ds(row0, UNIT), :] for j in range(NT)]
        xr = x_v[pl.ds(pl.multiple_of(base, UNIT), UNIT), :].astype(_F32)
        xg = xr[:, 0:LANES] * gw[:, 0:LANES]
        for j in range(1, NT):
            cols = slice(j * LANES, (j + 1) * LANES)
            xg = xg + xr[:, cols] * gw[:, cols]
        logits = []
        for w in range(W):
            st = base + (HALO - DIL * w)
            s = tie(qs[0], link) * k_s[0, pl.ds(st, UNIT), :]
            for j in range(1, NT):
                s = s + qs[j] * k_s[j, pl.ds(st, UNIT), :]
            link = s
            s = s + pltpu.roll(s, 64, 1)
            s = s + pltpu.roll(s, 32, 1)
            if masked and w > 0:
                pos = base + lax.broadcasted_iota(jnp.int32, (UNIT, LANES), 0)
                s = jnp.where(pos >= DIL * w, s, neg)
            logits.append(s)
        m = logits[0]
        for w in range(1, W):
            m = jnp.maximum(m, logits[w])
        ps = [jnp.exp2((logits[w] - m) * c_exp) for w in range(W)]
        den = ps[0]
        for w in range(1, W):
            den = den + ps[w]
        gate = jax.nn.sigmoid(jnp.sum(xg, axis=-1, keepdims=True))
        gate = jnp.broadcast_to(gate, (UNIT, LANES))
        g_s[pl.ds(row0, UNIT), :] = 1.0 - gate
        rinv = gate / den
        link = gate
        for j in range(NT):
            o = tie(ps[0], link) * v_s[j, pl.ds(base + HALO, UNIT), :]
            for w in range(1, W):
                o = o + ps[w] * v_s[j, pl.ds(base + (HALO - DIL * w), UNIT), :]
            link = o
            o_s[pl.ds(row0, UNIT), pl.ds(j * LANES, LANES)] = (
                (o * rinv).astype(_BF16))
        return link

    def row_block(r, carry):
        rows = pl.ds(pl.multiple_of(r * TM, TM), TM)
        krows = pl.ds(pl.multiple_of(r * TM + HALO, HALO), TM)
        xv = x_v[rows, :]
        for sec, dst in enumerate((q_s, k_s, v_s)):
            pcs = []
            lo, hi = sec * D, (sec + 1) * D
            while lo < hi:
                a = lo // HR
                nxt = min(hi, (a + 1) * HR)
                pcs.append(
                    wq_p[a, pl.ds((lo - a * HR) // 2, (nxt - lo) // 2), dc])
                lo = nxt
            res = _dot(xv, pltpu.bitcast(jnp.concatenate(pcs, axis=0), _BF16))
            for j in range(NT):
                piece = res[:, j * LANES:(j + 1) * LANES]
                if sec == 0:
                    dst[j] = piece
                else:
                    dst[j, krows, :] = piece

        gw = gw_ref[...].astype(_F32).reshape(1, D)
        never = lax.broadcasted_iota(jnp.int32, (UNIT, LANES), 1) < -1 - r
        link = None
        for un in range(TM // UNIT):
            link = attn_unit(r, un * UNIT, gw, never, link,
                             masked=(un * UNIT < HALO))

        gt = _dot(xv, wg[...])
        up = _dot(xv, wu[...])
        hh = (jnp.maximum(gt, 0.0) * up).astype(_BF16)
        acc[rows, :] += _dot(hh, wd[...])

        ov = o_s[...]
        g1 = jnp.concatenate([g_s[...]] * (WOC // LANES), axis=1)
        for n in range(NWO):
            res = (_dot(ov, wo_p[n])
                   + g1 * acc[rows, pl.ds(n * WOC, WOC)]).astype(_BF16)
            for i, (r0, r1, c0, c1) in enumerate(out_pieces):
                if c0 // WOC == n:
                    out_st[i][r] = res[r0:r1, c0 - n * WOC:c1 - n * WOC]
                    out_copy(r, i).start()
        return carry

    lax.fori_loop(0, NR, row_block, 0)
    for i in range(len(out_pieces)):
        for r in range(NR):
            out_copy(r, i).wait()


@jax.jit
def pallas_gated_mix__sliding_local_dilated__glu_gated_reglu__prompt_kernel(
    A_x: jax.Array,
    A_wqkv: jax.Array,
    A_wo: jax.Array,
    B_x: jax.Array,
    B_W_gate: jax.Array,
    B_W_up: jax.Array,
    B_W_down: jax.Array,
    gate_w: jax.Array,
):
    del B_x
    B, S, D = A_x.shape
    F = B_W_gate.shape[1]
    assert B == 1 and D == H * DH == NT * LANES
    assert sum(START_K) == D
    assert S % TM == 0 and S == 2 * TM0 and F > F0 and F % LANES == 0
    NR = S // TM
    F1 = F - F0
    HR = 3 * D // NSL
    NWO = D // WOC
    out_pieces = _out_pieces()
    n_sems = len(START_K) + S // TM0 + NG - 1 + NSL + NWO + 1

    any_spec = pl.BlockSpec(memory_space=pl.ANY)
    out = pl.pallas_call(
        functools.partial(_kernel, S=S, D=D, F=F),
        out_shape=jax.ShapeDtypeStruct((S, D), _BF16),
        in_specs=[any_spec] * 7,
        out_specs=any_spec,
        scratch_shapes=[
            pltpu.VMEM((S, D), _BF16),
            pltpu.VMEM((NSL + 1, HR, D), _BF16),
            pltpu.VMEM((NSL + 1, HR // 2, D + PAD), jnp.uint32),
            pltpu.VMEM((NWO + 1, D, WOC), _BF16),
            [pltpu.VMEM((H * (WOP + 1), LANES), _F32)
             for _ in range(WOC // LANES * DH // 8)],
            pltpu.VMEM((NWO + 1, D, WOC), _BF16),
            pltpu.VMEM((NG, D, FH), _BF16),
            pltpu.VMEM((NG, D, FH), _BF16),
            pltpu.VMEM((NG, FH, D + PAD), _BF16),
            pltpu.VMEM((D, F1), _BF16),
            pltpu.VMEM((D, F1), _BF16),
            pltpu.VMEM((F1, D), _BF16),
            pltpu.VMEM((S, D), _F32),
            pltpu.VMEM((TM0, 2 * FH), _F32),
            pltpu.VMEM((NT, TM, LANES), _F32),
            pltpu.VMEM((NT, HALO + S, LANES), _F32),
            pltpu.VMEM((NT, HALO + S, LANES), _F32),
            pltpu.VMEM((TM, LANES), _F32),
            pltpu.VMEM((TM, D), _BF16),
            [pltpu.VMEM((NR, r1 - r0, c1 - c0), _BF16)
             for r0, r1, c0, c1 in out_pieces],
            pltpu.VMEM((D,), _BF16),
            pltpu.SemaphoreType.DMA((n_sems,)),
            pltpu.SemaphoreType.DMA((len(out_pieces),)),
        ],
        compiler_params=pltpu.CompilerParams(
            vmem_limit_bytes=120 * 1024 * 1024,
            disable_bounds_checks=True,
            disable_semaphore_checks=True),
        name="gated_mix",
    )(A_x.reshape(S, D), A_wqkv, A_wo, B_W_gate, B_W_up, B_W_down, gate_w)
    return out.reshape(B, S, D)
```

```python
import functools
import math

import jax
import jax.numpy as jnp
from jax import lax
import jax.experimental.pallas as pl
import jax.experimental.pallas.tpu as pltpu

H = 32
DH = 32
W = 8
DIL = 2

LANES = 128
NT = 8
HALO = 16

TM = 256
TM0 = 1024
FH = 256
NG = 3
F0 = NG * FH
UNIT = 8
NSL = 4
PB = 4
WOC = 256
WOP = 9
PAD = 128

START_K = (128, 128, 256, 256, 256)

_F32 = jnp.float32
_BF16 = jnp.bfloat16


def _out_pieces():
    return ((0, TM, 0, 256), (0, TM, 256, 512), (0, TM, 512, 768),
            (0, TM, 768, 896), (0, TM // 2, 896, 1024),
            (TM // 2, TM, 896, 1024))


def _dot(a, b):
    return jnp.dot(a, b, preferred_element_type=_F32)


def _vregs(v):
    return [v[i * 8:(i + 1) * 8, n * LANES:(n + 1) * LANES]
            for n in range(v.shape[1] // LANES)
            for i in range(v.shape[0] // 8)]


def _kernel(x_hbm, wqkv_hbm, wo_hbm, wg_hbm, wu_hbm, wd_hbm, gw_hbm, out_hbm,
            x_v, wq_raw, wq_p, wo_raw, wo_f, wo_p, wg0, wu0, wd0, wg, wu, wd,
            acc, gu_s, q_s, k_s, v_s, g_s, o_s, out_st, gw_ref,
            sems, sem_out,
            *, S, D, F):
    NR = S // TM
    NR0 = S // TM0
    NP0 = NG * NR0
    F1 = F - F0
    HR = 3 * D // NSL
    NWO = D // WOC
    out_pieces = _out_pieces()
    dc = pl.ds(0, D)

    SW0 = 0
    SX = SW0 + len(START_K)
    SW1 = SX + NR0 - 1
    SG = SW1 + NG - 1
    SQ = SG + 1
    SR = SQ + NSL

    def start_copies(i):
        ks = pl.ds(sum(START_K[:i]), START_K[i])
        sem = sems.at[SW0 + i]
        rows = pl.ds(0, TM0)
        fs = pl.ds(0, FH)
        cps = [
            pltpu.make_async_copy(wg_hbm.at[ks, fs], wg0.at[0, ks, :], sem),
            pltpu.make_async_copy(wu_hbm.at[ks, fs], wu0.at[0, ks, :], sem),
            pltpu.make_async_copy(x_hbm.at[rows, ks], x_v.at[rows, ks], sem),
        ]
        if i == len(START_K) - 1:
            cps.append(pltpu.make_async_copy(
                wd_hbm.at[fs, :], wd0.at[0, :, dc], sem))
        return cps

    def x_copy(r):
        rows = pl.ds(r * TM0, TM0)
        return pltpu.make_async_copy(
            x_hbm.at[rows, :], x_v.at[rows, :], sems.at[SX + r - 1])

    def group_copies(gi):
        sem = sems.at[SW1 + gi - 1]
        lo = gi * FH
        if not isinstance(gi, int):
            lo = pl.multiple_of(lo, LANES)
        fs = pl.ds(lo, FH)
        return (
            pltpu.make_async_copy(wg_hbm.at[:, fs], wg0.at[gi], sem),
            pltpu.make_async_copy(wu_hbm.at[:, fs], wu0.at[gi], sem),
            pltpu.make_async_copy(wd_hbm.at[fs, :], wd0.at[gi, :, dc], sem),
        )

    def gw_copy():
        return pltpu.make_async_copy(gw_hbm, gw_ref, sems.at[SG])

    def wq_copies(a):
        cps = []
        lo, hi = a * HR, (a + 1) * HR
        while lo < hi:
            sec = lo // D
            nxt = min(hi, (sec + 1) * D)
            cps.append(pltpu.make_async_copy(
                wqkv_hbm.at[pl.ds(lo - sec * D, nxt - lo), pl.ds(sec * D, D)],
                wq_raw.at[a, pl.ds(lo - a * HR, nxt - lo), :],
                sems.at[SQ + a]))
            lo = nxt
        return cps

    def wq_wait(a):
        pltpu.make_async_copy(
            wq_raw.at[a], wq_raw.at[a], sems.at[SQ + a]).wait()

    def wo_copy(n):
        lo = n * WOC
        if not isinstance(n, int):
            lo = pl.multiple_of(lo, LANES)
        return pltpu.make_async_copy(
            wo_hbm.at[:, pl.ds(lo, WOC)], wo_raw.at[n], sems.at[SQ + n])

    def ffn_copies():
        sem = sems.at[SR]
        f1 = pl.ds(F0, F1)
        return (
            pltpu.make_async_copy(wg_hbm.at[:, f1], wg, sem),
            pltpu.make_async_copy(wu_hbm.at[:, f1], wu, sem),
            pltpu.make_async_copy(wd_hbm.at[f1, :], wd, sem),
        )

    def out_copy(r, i):
        r0, r1, c0, c1 = out_pieces[i]
        return pltpu.make_async_copy(
            out_st[i].at[r],
            out_hbm.at[pl.ds(r * TM + r0, r1 - r0), pl.ds(c0, c1 - c0)],
            sem_out.at[i])

    for i in range(len(START_K)):
        for cp in start_copies(i):
            cp.start()
    for t in range(1, NP0):
        if t < NR0:
            x_copy(t).start()
        if t % NR0 == 0:
            for cp in group_copies(t // NR0):
                cp.start()
        if t >= NP0 - NSL:
            for cp in wq_copies(t - (NP0 - NSL)):
                cp.start()
            wo_copy(t - (NP0 - NSL)).start()
    gw_copy().start()
    for cp in ffn_copies():
        cp.start()

    zeros_halo = jnp.zeros((HALO, LANES), _F32)
    for j in range(NT):
        k_s[j, pl.ds(0, HALO), :] = zeros_halo
        v_s[j, pl.ds(0, HALO), :] = zeros_halo

    n_clear = 16

    def clear(i, carry):
        n = HR // n_clear
        wq_raw[NSL, pl.ds(pl.multiple_of(i * n, 16), n), :] = (
            jnp.zeros((n, D), _BF16))
        n = D // n_clear
        wo_raw[NWO, pl.ds(pl.multiple_of(i * n, 16), n), :] = (
            jnp.zeros((n, WOC), _BF16))
        return carry

    lax.fori_loop(0, n_clear, clear, 0)

    def permute_wqkv(a):
        lane = lax.broadcasted_iota(jnp.int32, (PB * 8, LANES), 1)
        bits = [((lane >> (2 + b)) & 1) == 1 for b in range(3)]
        swap = ((lane & 3) << 5) | (lane & 28) | (lane >> 5)
        for g in range(HR // (16 * PB)):
            z = []
            for i in range(NT):
                w = pltpu.bitcast(
                    wq_raw[a, pl.ds(g * 16 * PB, 16 * PB),
                           pl.ds(i * LANES, LANES)], jnp.uint32)
                w = jnp.take_along_axis(w, swap, axis=1)
                z.append(w if i == 0 else pltpu.roll(w, 4 * i, 1))
            for b in range(3):
                z = [jnp.where(bits[b], z[(k + (1 << b)) % NT], z[k])
                     for k in range(NT)]
            for j in range(NT):
                y = z[(-j) % NT]
                wq_p[a, pl.ds(g * 8 * PB, 8 * PB), pl.ds(j * LANES, LANES)] = (
                    y if j == 0 else pltpu.roll(y, LANES - 4 * j, 1))

    def permute_wo(n, never, pace1, pace2):
        nj = WOC // LANES
        i = 0
        for h in range(H):
            blk = wo_raw[n, pl.ds(h * DH, DH), :].astype(_F32)
            for a in range(DH // 8):
                for j in range(nj):
                    pc = blk[a * 8:(a + 1) * 8, j * LANES:(j + 1) * LANES]
                    wo_f[a * nj + j][pl.ds(h * WOP, 8), :] = jnp.where(
                        never, pace1[i], pc)
                    i += 1
        i = 0
        for d in range(DH):
            for b in range(H // 8):
                rws = []
                for j in range(nj):
                    pc = wo_f[(d // 8) * nj + j][
                        pl.ds(b * 8 * WOP + d % 8, 8, stride=WOP), :]
                    rws.append(jnp.where(never, pace2[i], pc))
                    i += 1
                wo_p[n, pl.ds(d * H + b * 8, 8), :] = jnp.concatenate(
                    rws, axis=1).astype(_BF16)

    for i in range(len(START_K)):
        for cp in start_copies(i):
            cp.wait()
        ks = pl.ds(sum(START_K[:i]), START_K[i])
        part = _dot(x_v[pl.ds(0, TM0), ks],
                    jnp.concatenate([wg0[0, ks, :], wu0[0, ks, :]], axis=1))
        gu = part if i == 0 else part + gu_s[...]
        if i < len(START_K) - 1:
            gu_s[...] = gu
    hh0 = (jnp.maximum(gu[:, :FH], 0.0) * gu[:, FH:]).astype(_BF16)
    acc[pl.ds(0, TM0), :] = _dot(hh0, wd0[0, :, dc])

    def phase0(t, carry):
        gi = lax.shift_right_logical(t, 1)
        r = t & 1

        @pl.when(r == 0)
        def _():
            for cp in group_copies(gi):
                cp.wait()

        real = t >= NP0 - NSL

        @pl.when(real)
        def _():
            wq_wait(t - (NP0 - NSL))
            wo_copy(t - (NP0 - NSL)).wait()

        rows = pl.ds(pl.multiple_of(r * TM0, TM0), TM0)
        xv = x_v[rows, :]
        gt = _dot(xv, wg0[gi])
        up = _dot(xv, wu0[gi])
        hh = (jnp.maximum(gt, 0.0) * up).astype(_BF16)
        dn = _dot(hh, wd0[gi, :, dc])
        acc[rows, :] = dn + jnp.where(t >= NR0, acc[rows, :], 0.0)
        sl = jnp.where(real, t - (NP0 - NSL), NSL)
        permute_wqkv(sl)
        never = lax.broadcasted_iota(jnp.int32, (8, LANES), 1) < -1 - t
        npc = D * WOC // (8 * LANES)
        p1 = _vregs(gt) + _vregs(up)
        p1 = [p1[i * len(p1) // npc] for i in range(npc)]
        p2 = _vregs(dn)
        p2 = [p2[i * 3 * len(p2) // (4 * npc)] for i in range(npc)]
        permute_wo(sl, never, p1, p2)
        return carry

    x_copy(1).wait()
    lax.fori_loop(1, NP0, phase0, 0)
    gw_copy().wait()
    for cp in ffn_copies():
        cp.wait()

    scale = DH ** -0.5
    c_exp = scale * math.log2(math.e)
    neg = -1e9 / scale

    def attn_unit(r, row0, gw, never, link, masked):
        def tie(a, b):
            return a if b is None else jnp.where(never, b, a)

        base = r * TM + row0
        qs = [q_s[j, pl.ds(row0, UNIT), :] for j in range(NT)]
        xr = x_v[pl.ds(pl.multiple_of(base, UNIT), UNIT), :].astype(_F32)
        xg = xr[:, 0:LANES] * gw[:, 0:LANES]
        for j in range(1, NT):
            cols = slice(j * LANES, (j + 1) * LANES)
            xg = xg + xr[:, cols] * gw[:, cols]
        logits = []
        for w in range(W):
            st = base + (HALO - DIL * w)
            s = tie(qs[0], link) * k_s[0, pl.ds(st, UNIT), :]
            for j in range(1, NT):
                s = s + qs[j] * k_s[j, pl.ds(st, UNIT), :]
            link = s
            s = s + pltpu.roll(s, 64, 1)
            s = s + pltpu.roll(s, 32, 1)
            if masked and w > 0:
                pos = base + lax.broadcasted_iota(jnp.int32, (UNIT, LANES), 0)
                s = jnp.where(pos >= DIL * w, s, neg)
            logits.append(s)
        m = logits[0]
        for w in range(1, W):
            m = jnp.maximum(m, logits[w])
        ps = [jnp.exp2((logits[w] - m) * c_exp) for w in range(W)]
        den = ps[0]
        for w in range(1, W):
            den = den + ps[w]
        gate = jax.nn.sigmoid(jnp.sum(xg, axis=-1, keepdims=True))
        gate = jnp.broadcast_to(gate, (UNIT, LANES))
        g_s[pl.ds(row0, UNIT), :] = 1.0 - gate
        rinv = gate / den
        link = gate
        for j in range(NT):
            o = tie(ps[0], link) * v_s[j, pl.ds(base + HALO, UNIT), :]
            for w in range(1, W):
                o = o + ps[w] * v_s[j, pl.ds(base + (HALO - DIL * w), UNIT), :]
            link = o
            o_s[pl.ds(row0, UNIT), pl.ds(j * LANES, LANES)] = (
                (o * rinv).astype(_BF16))
        return link

    def row_block(r, carry):
        rows = pl.ds(pl.multiple_of(r * TM, TM), TM)
        krows = pl.ds(pl.multiple_of(r * TM + HALO, HALO), TM)
        xv = x_v[rows, :]
        for sec, dst in enumerate((q_s, k_s, v_s)):
            pcs = []
            lo, hi = sec * D, (sec + 1) * D
            while lo < hi:
                a = lo // HR
                nxt = min(hi, (a + 1) * HR)
                pcs.append(
                    wq_p[a, pl.ds((lo - a * HR) // 2, (nxt - lo) // 2), dc])
                lo = nxt
            res = _dot(xv, pltpu.bitcast(jnp.concatenate(pcs, axis=0), _BF16))
            for j in range(NT):
                piece = res[:, j * LANES:(j + 1) * LANES]
                if sec == 0:
                    dst[j] = piece
                else:
                    dst[j, krows, :] = piece

        gw = gw_ref[...].astype(_F32).reshape(1, D)
        never = lax.broadcasted_iota(jnp.int32, (UNIT, LANES), 1) < -1 - r
        link = None
        for un in range(TM // UNIT):
            link = attn_unit(r, un * UNIT, gw, never, link,
                             masked=(un * UNIT < HALO))

        gt = _dot(xv, wg[...])
        up = _dot(xv, wu[...])
        hh = (jnp.maximum(gt, 0.0) * up).astype(_BF16)
        acc[rows, :] += _dot(hh, wd[...])

        ov = o_s[...]
        g1 = jnp.concatenate([g_s[...]] * (WOC // LANES), axis=1)
        for n in range(NWO):
            res = (_dot(ov, wo_p[n])
                   + g1 * acc[rows, pl.ds(n * WOC, WOC)]).astype(_BF16)
            for i, (r0, r1, c0, c1) in enumerate(out_pieces):
                if c0 // WOC == n:
                    out_st[i][r] = res[r0:r1, c0 - n * WOC:c1 - n * WOC]
                    out_copy(r, i).start()
        return carry

    lax.fori_loop(0, NR, row_block, 0)
    for i in range(len(out_pieces)):
        for r in range(NR):
            out_copy(r, i).wait()


@jax.jit
def pallas_gated_mix__sliding_local_dilated__glu_gated_reglu__prompt_kernel(
    A_x: jax.Array,
    A_wqkv: jax.Array,
    A_wo: jax.Array,
    B_x: jax.Array,
    B_W_gate: jax.Array,
    B_W_up: jax.Array,
    B_W_down: jax.Array,
    gate_w: jax.Array,
):
    del B_x
    B, S, D = A_x.shape
    F = B_W_gate.shape[1]
    assert B == 1 and D == H * DH == NT * LANES
    assert sum(START_K) == D
    assert S % TM == 0 and S == 2 * TM0 and F > F0 and F % LANES == 0
    NR = S // TM
    F1 = F - F0
    HR = 3 * D // NSL
    NWO = D // WOC
    assert NWO == NSL
    out_pieces = _out_pieces()
    n_sems = len(START_K) + S // TM0 + NG - 1 + NSL + 1

    any_spec = pl.BlockSpec(memory_space=pl.ANY)
    out = pl.pallas_call(
        functools.partial(_kernel, S=S, D=D, F=F),
        out_shape=jax.ShapeDtypeStruct((S, D), _BF16),
        in_specs=[any_spec] * 7,
        out_specs=any_spec,
        scratch_shapes=[
            pltpu.VMEM((S, D), _BF16),
            pltpu.VMEM((NSL + 1, HR, D), _BF16),
            pltpu.VMEM((NSL + 1, HR // 2, D + PAD), jnp.uint32),
            pltpu.VMEM((NWO + 1, D, WOC), _BF16),
            [pltpu.VMEM((H * (WOP + 1), LANES), _F32)
             for _ in range(WOC // LANES * DH // 8)],
            pltpu.VMEM((NWO + 1, D, WOC), _BF16),
            pltpu.VMEM((NG, D, FH), _BF16),
            pltpu.VMEM((NG, D, FH), _BF16),
            pltpu.VMEM((NG, FH, D + PAD), _BF16),
            pltpu.VMEM((D, F1), _BF16),
            pltpu.VMEM((D, F1), _BF16),
            pltpu.VMEM((F1, D), _BF16),
            pltpu.VMEM((S, D), _F32),
            pltpu.VMEM((TM0, 2 * FH), _F32),
            pltpu.VMEM((NT, TM, LANES), _F32),
            pltpu.VMEM((NT, HALO + S, LANES), _F32),
            pltpu.VMEM((NT, HALO + S, LANES), _F32),
            pltpu.VMEM((TM, LANES), _F32),
            pltpu.VMEM((TM, D), _BF16),
            [pltpu.VMEM((NR, r1 - r0, c1 - c0), _BF16)
             for r0, r1, c0, c1 in out_pieces],
            pltpu.VMEM((D,), _BF16),
            pltpu.SemaphoreType.DMA((n_sems,)),
            pltpu.SemaphoreType.DMA((len(out_pieces),)),
        ],
        compiler_params=pltpu.CompilerParams(
            vmem_limit_bytes=120 * 1024 * 1024,
            disable_bounds_checks=True,
            disable_semaphore_checks=True),
        name="gated_mix",
    )(A_x.reshape(S, D), A_wqkv, A_wo, B_W_gate, B_W_up, B_W_down, gate_w)
    return out.reshape(B, S, D)
```
